```python
import jax
import jax.numpy as jnp

def _softmax(x, axis=-1):
    return jax.nn.softmax(x, axis=axis)
def _gelu(x):
    return jax.nn.gelu(x, approximate=True)
def _silu(x):
    return jax.nn.silu(x)
def _sigmoid(x):
    return jax.nn.sigmoid(x)
def _layernorm(x, axis=-1, eps=1e-5):
    m = jnp.mean(x, axis=axis, keepdims=True)
    v = jnp.var(x, axis=axis, keepdims=True)
    return (x - m) / jnp.sqrt(v + eps)
def _scatter_add(tgt, idx, src, axis=0):
    return tgt.at[idx].add(src)
def _segment_sum(src, seg, n):
    return jax.ops.segment_sum(src, seg, n)
class _Rng:
    def __init__(self, key):
        self._k = key
    def _next(self):
        self._k, sub = jax.random.split(self._k)
        return sub
    def normal(self, shape):
        return jax.random.normal(self._next(), shape, dtype=jnp.bfloat16)
    def randint(self, lo, hi, shape):
        return jax.random.randint(self._next(), shape, lo, hi, dtype=jnp.int32)
    def uniform(self, shape, lo=0.0, hi=1.0):
        return jax.random.uniform(self._next(), shape, jnp.bfloat16, lo, hi)
    def permutation(self, n):
        return jax.random.permutation(self._next(), n)


kernel_name = 'gated_mix__compressed_kv_cla__ssm_conv_h3__prompt'

def setup_inputs():
    _rng = _Rng(jax.random.key(int.from_bytes(__import__("os").urandom(4), "little")))
    _w = (lambda a: (lambda t: t.astype(jnp.bfloat16) if jnp.issubdtype(t.dtype, jnp.floating) else t)(jnp.asarray(a)))
    def _A_setup():
        B, H, Sq, Sk, D, M = 1, 32, 2048, 2048, 128, 1024
        Dc = 4 * D
        return {
            "x": _w((lambda *s: _rng.normal(s) * 0.05)(B, Sq, M)),
            "c_kv": _w((lambda *s: _rng.normal(s) * 0.05)(B, Sk, Dc)),
            "w_q": _w((lambda *s: _rng.normal(s) * 0.05)(M, H, D) * (M ** -0.5)),
            "w_uk": _w((lambda *s: _rng.normal(s) * 0.05)(Dc, H, D) * (Dc ** -0.5)),
            "w_uv": _w((lambda *s: _rng.normal(s) * 0.05)(Dc, H, D) * (Dc ** -0.5)),
            "w_o": _w((lambda *s: _rng.normal(s) * 0.05)(H, D, M) * ((H * D) ** -0.5)),
        }
    _A_in = _A_setup()

    def _B_setup():
        B, S, D = 1, 2048, 1024
        ks = 4
        return {
            "q": _w((lambda *s: _rng.normal(s) * 0.05)(B, S, D)),
            "k": _w((lambda *s: _rng.normal(s) * 0.05)(B, S, D)),
            "v": _w((lambda *s: _rng.normal(s) * 0.05)(B, S, D)),
            "shift_k": _w((lambda *s: _rng.normal(s) * 0.05)(D, ks) * 0.5),
            "ssm_k": _w((lambda *s: _rng.normal(s) * 0.05)(D, S) * (1.0 / S ** 0.5)),
            "ssm_D": _w((lambda *s: _rng.normal(s) * 0.05)(D)),
        }
    _B_in = _B_setup()

    return {
        "A_x": _A_in["x"],
        "A_c_kv": _A_in["c_kv"],
        "A_w_q": _A_in["w_q"],
        "A_w_uk": _A_in["w_uk"],
        "A_w_uv": _A_in["w_uv"],
        "A_w_o": _A_in["w_o"],
        "B_q": _B_in["q"],
        "B_k": _B_in["k"],
        "B_v": _B_in["v"],
        "B_shift_k": _B_in["shift_k"],
        "B_ssm_k": _B_in["ssm_k"],
        "B_ssm_D": _B_in["ssm_D"],
        "gate_w": _w((lambda *s: _rng.normal(s) * 0.05)(1024)),
    }

def reference(A_x, A_c_kv, A_w_q, A_w_uk, A_w_uv, A_w_o, B_q, B_k, B_v, B_shift_k, B_ssm_k, B_ssm_D, gate_w):
    def _A_ref(x, c_kv, w_q, w_uk, w_uv, w_o):
        B, Sq, M = x.shape[0], x.shape[1], x.shape[2]
        Sk = c_kv.shape[1]
        H, D = w_q.shape[1], w_q.shape[2]
        q = jnp.einsum("bqm,mhd->bhqd", x, w_q)
        k = jnp.einsum("bkc,chd->bhkd", c_kv, w_uk)
        v = jnp.einsum("bkc,chd->bhkd", c_kv, w_uv)
        scores = jnp.einsum("bhqd,bhkd->bhqk", q, k) * (D ** -0.5)
        off = Sk - Sq
        qi = jnp.arange(Sq)[:, None]
        kj = jnp.arange(Sk)[None, :]
        cmask = kj <= (qi + off)
        scores = jnp.where(cmask[None, None], scores, -1e9)
        p = _softmax(scores, axis=-1)
        ctx = jnp.einsum("bhqk,bhkd->bhqd", p, v)
        return jnp.einsum("bhqd,hdm->bqm", ctx, w_o)

    def _B_ref(q, k, v, shift_k, ssm_k, ssm_D):
        B, S, D = q.shape
        ks = shift_k.shape[-1]
        k_pad = jnp.pad(k, ((0, 0), (ks - 1, 0), (0, 0)))
        k_shift = jnp.zeros_like(k)
        for t in range(ks):
            k_shift = k_shift + k_pad[:, t:t + S, :] * shift_k[:, ks - 1 - t][None, None, :]
        kv = k_shift * v
        L = 2 * S
        kv_pad = jnp.pad(kv, ((0, 0), (0, S), (0, 0)))
        kf_pad = jnp.pad(ssm_k, ((0, 0), (0, S)))
        kv_f = (lambda x, axes=(-2,-1): jnp.fft.rfft2(x.astype(jnp.float32), axes=axes))(kv_pad[:, None, :, :], axes=(1, 2))
        kf_f = (lambda x, axes=(-2,-1): jnp.fft.rfft2(x.astype(jnp.float32), axes=axes))(kf_pad[:, None, :], axes=(1, 2))
        kf_f = (lambda x, *d: x.transpose(*d))(kf_f, 1, 2, 0)
        y_f = kv_f * kf_f[None, :, :, :]
        y = (lambda x, s, axes=(-2,-1): jnp.fft.irfft2(x, s=s, axes=axes).astype(jnp.bfloat16))(y_f, (1, L), axes=(1, 2))[:, 0, :S, :]
        y = y + kv * ssm_D[None, None, :]
        return q * y

    x = A_x
    g = _sigmoid((x * gate_w).sum(-1, keepdims=True))
    a = _A_ref(x, A_c_kv, A_w_q, A_w_uk, A_w_uv, A_w_o)
    b = _B_ref(x, B_k, B_v, B_shift_k, B_ssm_k, B_ssm_D)
    return g * a + (1 - g) * b
```

```python
import math

import jax
import jax.numpy as jnp
import numpy as np
import jax.experimental.pallas as pl
import jax.experimental.pallas.tpu as pltpu

f32 = jnp.float32
bf16 = jnp.bfloat16
u32 = jnp.uint32

S = 2048
M = 1024
DC = 512
H = 32
D = 128
T = 128
BQ = 512
NQ = S // BQ
NSUB = BQ // T
RC = 32
DEP_LAG = 2
C = 128
NCH = S // C
HALF = M // 2
KS = 4
RE = 128
NE = S // RE

QSCALE = (D ** -0.5) * math.log2(math.e)
NEG = -1e30
NT = (((1,), (1,)), ((), ()))


def _dft_matrices():
    freqs = np.concatenate([np.arange(0, C, 2), np.arange(1, C, 2)])
    t = np.arange(C)
    n = ((2 * freqs[:, None] + 1) * t[None, :]) % (4 * C)
    ang = np.pi * n / (2 * C)
    fwd = np.concatenate([np.cos(ang), -np.sin(ang)], axis=0)
    inv = fwd.T / C
    return fwd.astype(np.float32), inv.astype(np.float32)


def _iota(shape, dim):
    return jax.lax.broadcasted_iota(jnp.int32, shape, dim)


def _pk(v):
    return pltpu.bitcast(v, u32)


def _ld(ref, r0, r1, cols=slice(None)):
    return pltpu.bitcast(ref[r0 // 2: r1 // 2, cols], bf16)


def _kernel(x_ref, c_ref, wq_hbm, wk_hbm, wv_hbm, wo_hbm, k_ref, v_ref, sh_ref, sk_ref,
            sd_ref, gw_ref, fw_ref, iv_ref, o_ref,
            q_s, k_s, v_s, ctx_s, wo_s, wqb, wkb, wvb, wq_s, wk_s, wv_s, sem, wo_sem,
            xf, kf, yf, kprev, khalo, kv_s, g_s):
    h = pl.program_id(0)

    def w_copies(pair, slot):
        return [
            pltpu.make_async_copy(src.bitcast(u32).at[:, pair, :], dst.at[slot], sem.at[slot, n])
            for n, (src, dst) in enumerate(((wq_hbm, wqb), (wk_hbm, wkb), (wv_hbm, wvb)))
        ]

    def wo_copy():
        return pltpu.make_async_copy(wo_hbm, wo_s, wo_sem.at[0])

    def unpack_weights(slot, parity):
        sh = (16 * (1 - parity)).astype(u32)
        for src, dst in ((wqb, wq_s), (wkb, wk_s), (wvb, wv_s)):
            u = (src[slot] << sh) & jnp.uint32(0xFFFF0000)
            dst[...] = _pk(pltpu.bitcast(u, f32).astype(bf16))

    def q_proj(r0, r1):
        q = jnp.dot(x_ref[r0:r1, :], _ld(wq_s, 0, M), preferred_element_type=f32)
        q_s[r0 // 2: r1 // 2, :] = _pk((q * QSCALE).astype(bf16))

    def k_proj(r0, r1):
        k = jnp.dot(c_ref[r0:r1, :], _ld(wk_s, 0, DC), preferred_element_type=f32)
        k_s[r0 // 2: r1 // 2, :] = _pk(k.astype(bf16))

    def v_proj(r0, r1):
        v = jnp.dot(c_ref[r0:r1, :], _ld(wv_s, 0, DC), preferred_element_type=f32)
        v_s[r0 // 2: r1 // 2, :] = _pk(v.astype(bf16))

    st = {}

    def scores(i, g):
        base = i * BQ
        q = _ld(q_s, base, base + BQ)
        if g < i:
            st["s", i, g] = jax.lax.dot_general(q, _ld(k_s, g * BQ, (g + 1) * BQ), NT,
                                                preferred_element_type=f32)
            return
        tri = _iota((T, T), 1) <= _iota((T, T), 0)
        sd = []
        for t in range(NSUB):
            s = jax.lax.dot_general(q[t * T:, :], _ld(k_s, base + t * T, base + (t + 1) * T), NT,
                                    preferred_element_type=f32)
            top = jnp.where(tri, s[:T], NEG)
            sd.append(top if t == NSUB - 1 else jnp.concatenate([top, s[T:]], axis=0))
        st["s", i, i] = sd

    def group_tiles(i, g, r0):
        s = st["s", i, g]
        if g < i:
            return [s[r0:r0 + RC, cc * T:(cc + 1) * T] for cc in range(NSUB)]
        return [s[t][r0 - t * T: r0 - t * T + RC] for t in range(r0 // T + 1)]

    def tree(op, xs):
        while len(xs) > 1:
            xs = [op(xs[n], xs[n + 1]) if n + 1 < len(xs) else xs[n] for n in range(0, len(xs), 2)]
        return xs[0]

    chunks = list(range(0, BQ, RC))

    def row_max(i):
        mel = {}
        for g in range(i + 1):
            for r0 in chunks:
                pm = tree(jnp.maximum, group_tiles(i, g, r0))
                mel[r0] = pm if g == 0 else jnp.maximum(mel[r0], pm)
        st["m", i] = {r0: jnp.broadcast_to(jnp.max(mel[r0], axis=1, keepdims=True), (RC, T))
                      for r0 in chunks}

    def context(i):
        base = i * BQ
        mb = st.pop(("m", i))
        lsum = {}
        acc = None
        deps = []
        for g in range(i + 1):
            ps = {}
            for r0 in chunks:
                m = mb[r0]
                if len(deps) >= DEP_LAG:
                    m = jnp.concatenate([m[:8] + deps[-DEP_LAG], m[8:]], axis=0)
                p = [jnp.exp2(t - m) for t in group_tiles(i, g, r0)]
                part = tree(jnp.add, p)
                lsum[r0] = part if g == 0 else lsum[r0] + part
                deps.append(tree(jnp.add, [lsum[r0][n:n + 8] for n in range(0, RC, 8)]) * 0.0)
                ps[r0] = p
            if g < i:
                pg = jnp.concatenate([jnp.concatenate(ps[r0], axis=1) for r0 in chunks], axis=0)
                pv = jnp.dot(pg.astype(bf16), _ld(v_s, g * BQ, (g + 1) * BQ),
                             preferred_element_type=f32)
                acc = pv if acc is None else acc + pv
            else:
                parts = [None] * NSUB
                for t in range(NSUB):
                    pt = jnp.concatenate([ps[r0][t] for r0 in chunks if r0 >= t * T], axis=0)
                    pv = jnp.dot(pt.astype(bf16), _ld(v_s, base + t * T, base + (t + 1) * T),
                                 preferred_element_type=f32)
                    for r in range(t, NSUB):
                        piece = pv[(r - t) * T:(r - t + 1) * T]
                        parts[r] = piece if parts[r] is None else parts[r] + piece
                diag = jnp.concatenate(parts, axis=0)
                acc = diag if acc is None else acc + diag
            st.pop(("s", i, g))
        for r0 in chunks:
            l = jnp.sum(lsum[r0], axis=1, keepdims=True)
            inv = pl.reciprocal(l, approx=True)
            inv = inv * (2.0 - l * inv)
            ctx_s[h, (base + r0) // 2: (base + r0 + RC) // 2, :] = _pk(
                (acc[r0:r0 + RC] * inv).astype(bf16))

    def conv_forward_x(j):
        r0 = pl.multiple_of(j * C, C)
        w = sh_ref[...].astype(f32)
        kc = k_ref[...].astype(f32)
        ext = jnp.concatenate([khalo[...], kc], axis=0)
        ks = kc * w[0:1]
        for lag in range(1, KS):
            ks = ks + ext[8 - lag: 8 + C - lag] * w[lag:lag + 1]
        khalo[...] = kc[C - 8:]
        kvc = (ks * v_ref[...].astype(f32)).astype(bf16)
        kv_s[pl.ds(pl.multiple_of(j * (C // 2), C // 2), C // 2), :] = _pk(kvc)
        xs = jnp.dot(fw_ref[...], kvc, preferred_element_type=f32)
        xf[j, 0] = xs[:, :HALF]
        xf[j, 1] = xs[:, HALF:]
        xg = x_ref[pl.ds(r0, C), :].astype(f32) * gw_ref[...].astype(f32).reshape(1, M)
        g_s[pl.ds(r0, C), :] = jax.nn.sigmoid(jnp.sum(xg, axis=1, keepdims=True))

    def conv_forward_k(j):
        kn = jax.lax.dot_general(fw_ref[...], sk_ref[...], NT, preferred_element_type=f32)
        q4 = C // 2
        kp = kprev[...]
        kw = jnp.concatenate([
            kn[0:q4] - kp[2 * q4:3 * q4],
            kn[q4:2 * q4] + kp[3 * q4:4 * q4],
            kn[2 * q4:3 * q4] + kp[0:q4],
            kn[3 * q4:4 * q4] - kp[q4:2 * q4],
        ], axis=0)
        kprev[...] = kn
        kf[j, 0] = kw[:, :HALF]
        kf[j, 1] = kw[:, HALF:]

    def conv_block(n, outs):
        half = n % 2
        re = pl.ds(pl.multiple_of((n // 2) * 16, 16), 16)
        im = pl.ds(pl.multiple_of(C + (n // 2) * 16, 16), 16)
        pre = pl.ds(pl.multiple_of((n // 2) * 8, 8), 8)
        pim = pl.ds(pl.multiple_of(C // 2 + (n // 2) * 8, 8), 8)
        for i in outs:
            yr = yi = None
            for a in range(i + 1):
                xr, xi = xf[i - a, half, re, :], xf[i - a, half, im, :]
                kr, ki = kf[a, half, re, :], kf[a, half, im, :]
                pr = xr * kr - xi * ki
                pi = xr * ki + xi * kr
                yr = pr if yr is None else yr + pr
                yi = pi if yi is None else yi + pi
            yf[i, half, pre, :] = _pk(yr.astype(bf16))
            yf[i, half, pim, :] = _pk(yi.astype(bf16))

    def conv_block_fill(n):
        return {"P%d" % m: (lambda m=m: conv_block(n, (NCH - 1 - m, m))) for m in range(NCH // 2)}

    def conv_inverse(j):
        dvec = sd_ref[...].astype(f32).reshape(1, M)
        r = pl.ds(pl.multiple_of(j * C, C), C)
        pr = pl.ds(pl.multiple_of(j * (C // 2), C // 2), C // 2)
        y = jnp.concatenate(
            [jnp.dot(iv_ref[...], pltpu.bitcast(yf[j, hh], bf16), preferred_element_type=f32)
             for hh in range(2)], axis=1)
        y = y + pltpu.bitcast(kv_s[pr, :], bf16).astype(f32) * dvec
        return x_ref[r, :].astype(f32) * y

    @pl.when(h == 0)
    def _():
        for cp in w_copies(0, 0):
            cp.start()
        wo_copy().start()
        kprev[...] = jnp.zeros(kprev.shape, f32)
        khalo[...] = jnp.zeros(khalo.shape, f32)
        for cp in w_copies(0, 0):
            cp.wait()
        unpack_weights(0, h * 0)

        def body(i, carry):
            r = pl.ds(pl.multiple_of(i * BQ, BQ), BQ)
            pr = pl.ds(pl.multiple_of(i * (BQ // 2), BQ // 2), BQ // 2)
            cc = c_ref[r, :]
            k_s[pr, :] = _pk(jnp.dot(cc, _ld(wk_s, 0, DC), preferred_element_type=f32).astype(bf16))
            v_s[pr, :] = _pk(jnp.dot(cc, _ld(wv_s, 0, DC), preferred_element_type=f32).astype(bf16))
            q = jnp.dot(x_ref[r, :], _ld(wq_s, 0, M), preferred_element_type=f32)
            q_s[pr, :] = _pk((q * QSCALE).astype(bf16))
            return carry

        jax.lax.fori_loop(0, NQ, body, 0)

    slot = h % 2

    @pl.when(jnp.logical_and(h > 0, h < H - 1))
    def _():
        for cp in w_copies((h + 1) // 2, slot):
            cp.wait()

    @pl.when(h < H - 2)
    def _():
        for cp in w_copies((h + 2) // 2, 1 - slot):
            cp.start()

    HB = BQ // 2

    def head_step(fill):
        def run(*names):
            for name in names:
                if name in fill:
                    fill[name]()
        scores(3, 0); run("P0"); scores(3, 1); scores(3, 2); run("P1"); scores(3, 3)
        row_max(3)
        run("K3")
        context(3)
        run("V3", "P2")
        scores(2, 0); scores(2, 1); run("P3"); scores(2, 2)
        row_max(2)
        run("Q3a", "Q3b")
        context(2)
        run("V2", "P4")
        scores(1, 0); scores(1, 1)
        row_max(1)
        run("K2", "P5", "Q2a", "Q2b")
        context(1)
        run("V1")
        scores(0, 0)
        row_max(0)
        run("K1", "P6", "Q1a", "Q1b", "E0", "E1")
        context(0)
        run("V0", "P7", "K0", "Q0a", "Q0b")

    def proj_fill():
        fill = {}
        for i in range(NQ):
            fill["K%d" % i] = lambda i=i: k_proj(i * BQ, (i + 1) * BQ)
            fill["V%d" % i] = lambda i=i: v_proj(i * BQ, (i + 1) * BQ)
            fill["Q%da" % i] = lambda i=i: q_proj(i * BQ, i * BQ + HB)
            fill["Q%db" % i] = lambda i=i: q_proj(i * BQ + HB, (i + 1) * BQ)
        return fill

    @pl.when(h < NCH)
    def _():
        unpack_weights(slot, (h + 1) % 2)
        fill = proj_fill()
        fill["E0"] = lambda: conv_forward_x(h)
        fill["E1"] = lambda: conv_forward_k(h)
        head_step(fill)

    @pl.when(jnp.logical_and(h >= NCH, h < H - 1))
    def _():
        unpack_weights(slot, (h + 1) % 2)
        fill = proj_fill()
        fill.update(conv_block_fill(h - NCH))
        head_step(fill)

    @pl.when(h == H - 1)
    def _():
        head_step(conv_block_fill(NCH - 1))
        wo_copy().wait()

    @pl.when(h >= H)
    def _():
        e = h - H
        pr = pl.ds(pl.multiple_of(e * (RE // 2), RE // 2), RE // 2)
        r = pl.ds(pl.multiple_of(e * RE, RE), RE)
        ctx = jnp.concatenate([pltpu.bitcast(ctx_s[hh, pr, :], bf16) for hh in range(H)], axis=1)
        b = jnp.concatenate([conv_inverse(e * (RE // C) + j) for j in range(RE // C)], axis=0)
        a = jnp.dot(ctx, wo_s[...], preferred_element_type=f32)
        g = g_s[r, :]
        o_ref[...] = (b + g * (a - b)).astype(o_ref.dtype)


@jax.jit
def pallas_gated_mix__compressed_kv_cla__ssm_conv_h3__prompt_kernel(
    A_x: jax.Array,
    A_c_kv: jax.Array,
    A_w_q: jax.Array,
    A_w_uk: jax.Array,
    A_w_uv: jax.Array,
    A_w_o: jax.Array,
    B_q: jax.Array,
    B_k: jax.Array,
    B_v: jax.Array,
    B_shift_k: jax.Array,
    B_ssm_k: jax.Array,
    B_ssm_D: jax.Array,
    gate_w: jax.Array,
):
    fwd, inv = _dft_matrices()
    fwd = jnp.asarray(fwd, bf16)
    inv = jnp.asarray(inv, bf16)

    once = pl.Buffered(1)

    def whole(shape):
        return pl.BlockSpec(shape, lambda h: (0,) * len(shape), pipeline_mode=once)

    chunk = lambda h: (0, jnp.minimum(h, NCH - 1), 0)
    in_specs = [
        pl.BlockSpec((None, S, M), lambda h: (0, 0, 0), pipeline_mode=once),
        pl.BlockSpec((None, S, DC), lambda h: (0, 0, 0), pipeline_mode=once),
        pl.BlockSpec(memory_space=pl.ANY),
        pl.BlockSpec(memory_space=pl.ANY),
        pl.BlockSpec(memory_space=pl.ANY),
        pl.BlockSpec(memory_space=pl.ANY),
        pl.BlockSpec((None, C, M), chunk),
        pl.BlockSpec((None, C, M), chunk),
        whole((KS, M)),
        pl.BlockSpec((M, C), lambda h: (0, jnp.minimum(h, NCH - 1))),
        whole((M,)),
        whole((M,)),
        whole((2 * C, C)),
        whole((C, 2 * C)),
    ]
    scratch = [
        pltpu.VMEM((S // 2, D), u32), pltpu.VMEM((S // 2, D), u32), pltpu.VMEM((S // 2, D), u32),
        pltpu.VMEM((H, S // 2, D), u32),
        pltpu.VMEM((H * D, M), bf16),
        pltpu.VMEM((2, M, D), u32), pltpu.VMEM((2, DC, D), u32), pltpu.VMEM((2, DC, D), u32),
        pltpu.VMEM((M // 2, D), u32), pltpu.VMEM((DC // 2, D), u32), pltpu.VMEM((DC // 2, D), u32),
        pltpu.SemaphoreType.DMA((2, 3)),
        pltpu.SemaphoreType.DMA((1,)),
        pltpu.VMEM((NCH, 2, 2 * C, HALF), f32),
        pltpu.VMEM((NCH, 2, 2 * C, HALF), f32),
        pltpu.VMEM((NCH, 2, C, HALF), u32),
        pltpu.VMEM((2 * C, M), f32),
        pltpu.VMEM((8, M), f32),
        pltpu.VMEM((S // 2, M), u32),
        pltpu.VMEM((S, 1), f32),
    ]
    return pl.pallas_call(
        _kernel,
        grid=(H + NE,),
        in_specs=in_specs,
        out_specs=pl.BlockSpec((None, RE, M), lambda h: (0, jnp.maximum(h - H, 0), 0)),
        out_shape=jax.ShapeDtypeStruct((1, S, M), bf16),
        scratch_shapes=scratch,
        compiler_params=pltpu.CompilerParams(
            dimension_semantics=("arbitrary",),
            vmem_limit_bytes=126 * 1024 * 1024,
        ),
        name="gated_mix_kernel",
    )(A_x, A_c_kv, A_w_q, A_w_uk, A_w_uv, A_w_o.reshape(H * D, M), B_k, B_v, B_shift_k.T,
      B_ssm_k, B_ssm_D, gate_w, fwd, inv)
```

```python
import math

import jax
import jax.numpy as jnp
import numpy as np
import jax.experimental.pallas as pl
import jax.experimental.pallas.tpu as pltpu

f32 = jnp.float32
bf16 = jnp.bfloat16
u32 = jnp.uint32

S = 2048
M = 1024
DC = 512
H = 32
D = 128
T = 128
BQ = 512
NQ = S // BQ
NSUB = BQ // T
RC = 32
DEP_LAG = 2
GROUP = 2
C = 128
NCH = S // C
HALF = M // 2
KS = 4
RE = 128
NE = S // RE

QSCALE = (D ** -0.5) * math.log2(math.e)
NEG = -1e30
NT = (((1,), (1,)), ((), ()))


def _dft_matrices():
    freqs = np.concatenate([np.arange(0, C, 2), np.arange(1, C, 2)])
    t = np.arange(C)
    n = ((2 * freqs[:, None] + 1) * t[None, :]) % (4 * C)
    ang = np.pi * n / (2 * C)
    fwd = np.concatenate([np.cos(ang), -np.sin(ang)], axis=0)
    inv = fwd.T / C
    return fwd.astype(np.float32), inv.astype(np.float32)


def _iota(shape, dim):
    return jax.lax.broadcasted_iota(jnp.int32, shape, dim)


def _pk(v):
    return pltpu.bitcast(v, u32)


def _un(u):
    return pltpu.bitcast(u, bf16)


def _ld(ref, r0, r1, cols=slice(None)):
    return _un(ref[r0 // 2: r1 // 2, cols])


def _zero_of(t):
    return (pltpu.bitcast(t, u32) >> 31) & jnp.uint32(2)


class Hooks:
    def __init__(self, items=(), rate=1.0):
        self.items = list(items)
        self.rate = rate
        self.credit = 0.0

    def take(self):
        self.credit += self.rate
        if self.items and self.items[0][0] <= self.credit:
            cost, thunk = self.items.pop(0)
            self.credit -= cost
            return thunk()
        return None

    def flush(self):
        for _, thunk in self.items:
            thunk()
        self.items = []

    def lhs(self, u, tiles=(0,)):
        nrow = u.shape[0] // 8
        cols = [u[:, t * T:(t + 1) * T] for t in range(u.shape[1] // T)]
        for t in tiles:
            parts, start = [], 0
            for r in range(nrow):
                z = self.take()
                if z is not None:
                    if r * 8 > start:
                        parts.append(cols[t][start:r * 8])
                    parts.append(cols[t][r * 8:(r + 1) * 8] | z)
                    start = (r + 1) * 8
            if start < nrow * 8:
                parts.append(cols[t][start:])
            cols[t] = parts[0] if len(parts) == 1 else jnp.concatenate(parts, axis=0)
        return _un(cols[0] if len(cols) == 1 else jnp.concatenate(cols, axis=1))


def _kernel(x_hbm, c_hbm, wq_hbm, wk_hbm, wv_hbm, wo_hbm, k_hbm, v_hbm, sk_hbm,
            sh_ref, sd_ref, gw_ref, fw_ref, iv_ref, o_ref,
            x_s, c_s, wo_s, q_s, k_s, v_s, ctx_s, wqb, wkb, wvb, wq_s, wk_s, wv_s,
            kb, vb, skb, xf, kf, yf, kprev, khalo, kv_s, g_s,
            big_sem, w_sem, ch_sem):
    h = pl.program_id(0)

    def big_copy(n):
        src, dst = ((c_hbm.at[0], c_s), (x_hbm.at[0], x_s), (wo_hbm, wo_s))[n]
        return pltpu.make_async_copy(src.bitcast(u32), dst, big_sem.at[n])

    def w_copies(pair, slot):
        return [
            pltpu.make_async_copy(src.bitcast(u32).at[:, pair, :], dst.at[slot], w_sem.at[slot, n])
            for n, (src, dst) in enumerate(((wq_hbm, wqb), (wk_hbm, wkb), (wv_hbm, wvb)))
        ]

    def chunk_copies(j, slot):
        rows = pl.ds(pl.multiple_of(j * (C // 2), C // 2), C // 2)
        cols = pl.ds(pl.multiple_of(j * C, C), C)
        return [
            pltpu.make_async_copy(k_hbm.at[0].bitcast(u32).at[rows, :], kb.at[slot], ch_sem.at[slot, 0]),
            pltpu.make_async_copy(v_hbm.at[0].bitcast(u32).at[rows, :], vb.at[slot], ch_sem.at[slot, 1]),
            pltpu.make_async_copy(sk_hbm.bitcast(u32).at[:, cols], skb.at[slot], ch_sem.at[slot, 2]),
        ]

    def unpack_weights(slot, parity):
        sh = (16 * (1 - parity)).astype(u32)
        for src, dst in ((wqb, wq_s), (wkb, wk_s), (wvb, wv_s)):
            u = (src[slot] << sh) & jnp.uint32(0xFFFF0000)
            dst[...] = _pk(pltpu.bitcast(u, f32).astype(bf16))

    def q_proj(r0, r1, hk):
        lhs = hk.lhs(x_s[r0 // 2: r1 // 2, :], (0, 4))
        q = jnp.dot(lhs, _un(wq_s[...]), preferred_element_type=f32)
        q_s[r0 // 2: r1 // 2, :] = _pk((q * QSCALE).astype(bf16))

    def k_proj(r0, r1, hk):
        lhs = hk.lhs(c_s[r0 // 2: r1 // 2, :])
        k = jnp.dot(lhs, _un(wk_s[...]), preferred_element_type=f32)
        k_s[r0 // 2: r1 // 2, :] = _pk(k.astype(bf16))

    def v_proj(r0, r1, hk):
        lhs = hk.lhs(c_s[r0 // 2: r1 // 2, :])
        v = jnp.dot(lhs, _un(wv_s[...]), preferred_element_type=f32)
        v_s[r0 // 2: r1 // 2, :] = _pk(v.astype(bf16))

    st = {}

    def scores(i, g, hk):
        base = i * BQ
        qu = q_s[base // 2: (base + BQ) // 2, :]
        if g < i:
            st["s", i, g] = jax.lax.dot_general(hk.lhs(qu), _ld(k_s, g * BQ, (g + 1) * BQ), NT,
                                                preferred_element_type=f32)
            return
        q = _un(qu)
        tri = _iota((T, T), 1) <= _iota((T, T), 0)
        sd = []
        for t in range(NSUB):
            s = jax.lax.dot_general(q[t * T:, :], _ld(k_s, base + t * T, base + (t + 1) * T), NT,
                                    preferred_element_type=f32)
            top = jnp.where(tri, s[:T], NEG)
            sd.append(top if t == NSUB - 1 else jnp.concatenate([top, s[T:]], axis=0))
        st["s", i, i] = sd

    def group_tiles(i, g, r0):
        s = st["s", i, g]
        if g < i:
            return [s[r0:r0 + RC, cc * T:(cc + 1) * T] for cc in range(NSUB)]
        return [s[t][r0 - t * T: r0 - t * T + RC] for t in range(r0 // T + 1)]

    def tree(op, xs):
        while len(xs) > 1:
            xs = [op(xs[n], xs[n + 1]) if n + 1 < len(xs) else xs[n] for n in range(0, len(xs), 2)]
        return xs[0]

    chunks = list(range(0, BQ, RC))

    def row_max(i):
        mel = {}
        for g in range(i + 1):
            for r0 in chunks:
                pm = tree(jnp.maximum, group_tiles(i, g, r0))
                mel[r0] = pm if g == 0 else jnp.maximum(mel[r0], pm)
        st["m", i] = {r0: jnp.broadcast_to(jnp.max(mel[r0], axis=1, keepdims=True), (RC, T))
                      for r0 in chunks}

    def context(i):
        base = i * BQ
        mb = st.pop(("m", i))
        lsum = {}
        acc = None
        deps = []
        for g in range(i + 1):
            ps = {}
            for r0 in chunks:
                m = mb[r0]
                if len(deps) >= DEP_LAG:
                    m = jnp.concatenate([m[:8] + deps[-DEP_LAG], m[8:]], axis=0)
                p = [jnp.exp2(t - m) for t in group_tiles(i, g, r0)]
                part = tree(jnp.add, p)
                lsum[r0] = part if g == 0 else lsum[r0] + part
                deps.append(tree(jnp.add, [lsum[r0][n:n + 8] for n in range(0, RC, 8)]) * 0.0)
                ps[r0] = p
            if g < i:
                pg = jnp.concatenate([jnp.concatenate(ps[r0], axis=1) for r0 in chunks], axis=0)
                pv = jnp.dot(pg.astype(bf16), _ld(v_s, g * BQ, (g + 1) * BQ),
                             preferred_element_type=f32)
                acc = pv if acc is None else acc + pv
            else:
                parts = [None] * NSUB
                for t in range(NSUB):
                    pt = jnp.concatenate([ps[r0][t] for r0 in chunks if r0 >= t * T], axis=0)
                    pv = jnp.dot(pt.astype(bf16), _ld(v_s, base + t * T, base + (t + 1) * T),
                                 preferred_element_type=f32)
                    for r in range(t, NSUB):
                        piece = pv[(r - t) * T:(r - t + 1) * T]
                        parts[r] = piece if parts[r] is None else parts[r] + piece
                diag = jnp.concatenate(parts, axis=0)
                acc = diag if acc is None else acc + diag
            st.pop(("s", i, g))
        for r0 in chunks:
            l = jnp.sum(lsum[r0], axis=1, keepdims=True)
            inv = pl.reciprocal(l, approx=True)
            inv = inv * (2.0 - l * inv)
            ctx_s[h, (base + r0) // 2: (base + r0 + RC) // 2, :] = _pk(
                (acc[r0:r0 + RC] * inv).astype(bf16))

    def conv_forward_x(j, slot):
        pr = pl.ds(pl.multiple_of(j * (C // 2), C // 2), C // 2)
        r = pl.ds(pl.multiple_of(j * C, C), C)
        w = sh_ref[...].astype(f32)
        kc = _un(kb[slot]).astype(f32)
        ext = jnp.concatenate([khalo[...], kc], axis=0)
        ks = kc * w[0:1]
        for lag in range(1, KS):
            ks = ks + ext[8 - lag: 8 + C - lag] * w[lag:lag + 1]
        khalo[...] = kc[C - 8:]
        kvc = (ks * _un(vb[slot]).astype(f32)).astype(bf16)
        kv_s[pr, :] = _pk(kvc)
        xs = jnp.dot(fw_ref[...], kvc, preferred_element_type=f32)
        xf[j, 0] = xs[:, :HALF]
        xf[j, 1] = xs[:, HALF:]
        xg = _un(x_s[pr, :]).astype(f32) * gw_ref[...].astype(f32).reshape(1, M)
        g_s[r, :] = jax.nn.sigmoid(jnp.sum(xg, axis=1, keepdims=True))

    def conv_forward_k(j, slot):
        kn = jax.lax.dot_general(fw_ref[...], _un(skb[slot]), NT, preferred_element_type=f32)
        q4 = C // 2
        kp = kprev[...]
        kw = jnp.concatenate([
            kn[0:q4] - kp[2 * q4:3 * q4],
            kn[q4:2 * q4] + kp[3 * q4:4 * q4],
            kn[2 * q4:3 * q4] + kp[0:q4],
            kn[3 * q4:4 * q4] - kp[q4:2 * q4],
        ], axis=0)
        kprev[...] = kn
        kf[j, 0] = kw[:, :HALF]
        kf[j, 1] = kw[:, HALF:]

    def conv_block_items(n, group):
        half = n % 2
        re = pl.ds(pl.multiple_of((n // 2) * 16, 16), 16)
        im = pl.ds(pl.multiple_of(C + (n // 2) * 16, 16), 16)
        pre = pl.ds(pl.multiple_of((n // 2) * 8, 8), 8)
        pim = pl.ds(pl.multiple_of(C // 2 + (n // 2) * 8, 8), 8)

        acc = {}

        def some(lb, i, a0, a1):
            ln = slice(lb * T, (lb + 1) * T)
            yr, yi = acc.pop((lb, i), (None, None))
            for a in range(a0, a1):
                xr, xi = xf[i - a, half, re, ln], xf[i - a, half, im, ln]
                kr, ki = kf[a, half, re, ln], kf[a, half, im, ln]
                pr = xr * kr - xi * ki
                pi = xr * ki + xi * kr
                yr = pr if yr is None else yr + pr
                yi = pi if yi is None else yi + pi
            if a1 == i + 1:
                yr, yi = _pk(yr.astype(bf16)), _pk(yi.astype(bf16))
                yf[i, half, pre, ln] = yr
                yf[i, half, pim, ln] = yi
                return _zero_of(yr | yi)
            acc[lb, i] = (yr, yi)
            ur, ui = pltpu.bitcast(yr, u32), pltpu.bitcast(yi, u32)
            return _zero_of((ur[:8] | ur[8:]) | (ui[:8] | ui[8:]))

        return [(min(a0 + group, i + 1) - a0,
                 (lambda lb=lb, i=i, a0=a0: some(lb, i, a0, min(a0 + group, i + 1))))
                for lb in range(HALF // T) for i in range(NCH) for a0 in range(0, i + 1, group)]

    def conv_inverse(j):
        dvec = sd_ref[...].astype(f32).reshape(1, M)
        pr = pl.ds(pl.multiple_of(j * (C // 2), C // 2), C // 2)
        y = jnp.concatenate(
            [jnp.dot(iv_ref[...], _un(yf[j, hh]), preferred_element_type=f32)
             for hh in range(2)], axis=1)
        y = y + _un(kv_s[pr, :]).astype(f32) * dvec
        return _un(x_s[pr, :]).astype(f32) * y

    @pl.when(h == 0)
    def _():
        big_copy(0).start()
        for cp in w_copies(0, 0):
            cp.start()
        big_copy(1).start()
        for cp in chunk_copies(0, 0):
            cp.start()
        kprev[...] = jnp.zeros(kprev.shape, f32)
        khalo[...] = jnp.zeros(khalo.shape, f32)
        big_copy(0).wait()
        for cp in w_copies(0, 0):
            cp.wait()
        unpack_weights(0, h * 0)

        def kv_body(i, carry):
            pr = pl.ds(pl.multiple_of(i * (BQ // 2), BQ // 2), BQ // 2)
            cc = _un(c_s[pr, :])
            k_s[pr, :] = _pk(jnp.dot(cc, _un(wk_s[...]), preferred_element_type=f32).astype(bf16))
            v_s[pr, :] = _pk(jnp.dot(cc, _un(wv_s[...]), preferred_element_type=f32).astype(bf16))
            return carry

        jax.lax.fori_loop(0, NQ, kv_body, 0)
        big_copy(1).wait()
        big_copy(2).start()

        def q_body(i, carry):
            pr = pl.ds(pl.multiple_of(i * (BQ // 2), BQ // 2), BQ // 2)
            q = jnp.dot(_un(x_s[pr, :]), _un(wq_s[...]), preferred_element_type=f32)
            q_s[pr, :] = _pk((q * QSCALE).astype(bf16))
            return carry

        jax.lax.fori_loop(0, NQ, q_body, 0)

    slot = h % 2

    @pl.when(jnp.logical_and(h > 0, h < H - 1))
    def _():
        for cp in w_copies((h + 1) // 2, slot):
            cp.wait()

    @pl.when(h < H - 2)
    def _():
        for cp in w_copies((h + 2) // 2, 1 - slot):
            cp.start()

    @pl.when(h < NCH)
    def _():
        for cp in chunk_copies(h, slot):
            cp.wait()

    @pl.when(h < NCH - 1)
    def _():
        for cp in chunk_copies(h + 1, 1 - slot):
            cp.start()

    HB = BQ // 2

    def head_step(fill, hk):
        def run(*names):
            for name in names:
                if name in fill:
                    fill[name](hk)

        for g in range(4):
            scores(3, g, hk)
        row_max(3)
        run("K3")
        context(3)
        run("V3")
        for g in range(3):
            scores(2, g, hk)
        row_max(2)
        run("Q3a", "Q3b")
        context(2)
        run("V2")
        for g in range(2):
            scores(1, g, hk)
        row_max(1)
        run("K2", "Q2a", "Q2b")
        context(1)
        run("V1")
        scores(0, 0, hk)
        row_max(0)
        run("K1", "Q1a", "Q1b", "E0", "E1")
        context(0)
        run("V0", "K0", "Q0a", "Q0b")
        hk.flush()

    def proj_fill():
        fill = {}
        for i in range(NQ):
            fill["K%d" % i] = lambda hk, i=i: k_proj(i * BQ, (i + 1) * BQ, hk)
            fill["V%d" % i] = lambda hk, i=i: v_proj(i * BQ, (i + 1) * BQ, hk)
            fill["Q%da" % i] = lambda hk, i=i: q_proj(i * BQ, i * BQ + HB, hk)
            fill["Q%db" % i] = lambda hk, i=i: q_proj(i * BQ + HB, (i + 1) * BQ, hk)
        return fill

    @pl.when(h < NCH)
    def _():
        unpack_weights(slot, (h + 1) % 2)
        fill = proj_fill()
        fill["E0"] = lambda hk: conv_forward_x(h, slot)
        fill["E1"] = lambda hk: conv_forward_k(h, slot)
        head_step(fill, Hooks())

    @pl.when(jnp.logical_and(h >= NCH, h < H - 1))
    def _():
        unpack_weights(slot, (h + 1) % 2)
        head_step(proj_fill(), Hooks(conv_block_items(h - NCH, GROUP), rate=0.8))

    @pl.when(h == H - 1)
    def _():
        head_step({}, Hooks(conv_block_items(NCH - 1, 4), rate=3.0))
        big_copy(2).wait()

    @pl.when(h >= H)
    def _():
        e = h - H
        pr = pl.ds(pl.multiple_of(e * (RE // 2), RE // 2), RE // 2)
        r = pl.ds(pl.multiple_of(e * RE, RE), RE)
        ctx = jnp.concatenate([_un(ctx_s[hh, pr, :]) for hh in range(H)], axis=1)
        b = jnp.concatenate([conv_inverse(e * (RE // C) + j) for j in range(RE // C)], axis=0)
        a = jnp.dot(ctx, _un(wo_s[...]), preferred_element_type=f32)
        g = g_s[r, :]
        o_ref[...] = (b + g * (a - b)).astype(o_ref.dtype)


@jax.jit
def pallas_gated_mix__compressed_kv_cla__ssm_conv_h3__prompt_kernel(
    A_x: jax.Array,
    A_c_kv: jax.Array,
    A_w_q: jax.Array,
    A_w_uk: jax.Array,
    A_w_uv: jax.Array,
    A_w_o: jax.Array,
    B_q: jax.Array,
    B_k: jax.Array,
    B_v: jax.Array,
    B_shift_k: jax.Array,
    B_ssm_k: jax.Array,
    B_ssm_D: jax.Array,
    gate_w: jax.Array,
):
    fwd, inv = _dft_matrices()
    fwd = jnp.asarray(fwd, bf16)
    inv = jnp.asarray(inv, bf16)

    once = pl.Buffered(1)

    def whole(shape):
        return pl.BlockSpec(shape, lambda h: (0,) * len(shape), pipeline_mode=once)

    hbm = pl.BlockSpec(memory_space=pl.ANY)
    in_specs = [hbm] * 9 + [
        whole((KS, M)),
        whole((M,)),
        whole((M,)),
        whole((2 * C, C)),
        whole((C, 2 * C)),
    ]
    scratch = [
        pltpu.VMEM((S // 2, M), u32),
        pltpu.VMEM((S // 2, DC), u32),
        pltpu.VMEM((H * D // 2, M), u32),
        pltpu.VMEM((S // 2, D), u32), pltpu.VMEM((S // 2, D), u32), pltpu.VMEM((S // 2, D), u32),
        pltpu.VMEM((H, S // 2, D), u32),
        pltpu.VMEM((2, M, D), u32), pltpu.VMEM((2, DC, D), u32), pltpu.VMEM((2, DC, D), u32),
        pltpu.VMEM((M // 2, D), u32), pltpu.VMEM((DC // 2, D), u32), pltpu.VMEM((DC // 2, D), u32),
        pltpu.VMEM((2, C // 2, M), u32), pltpu.VMEM((2, C // 2, M), u32),
        pltpu.VMEM((2, M // 2, C), u32),
        pltpu.VMEM((NCH, 2, 2 * C, HALF), f32),
        pltpu.VMEM((NCH, 2, 2 * C, HALF), f32),
        pltpu.VMEM((NCH, 2, C, HALF), u32),
        pltpu.VMEM((2 * C, M), f32),
        pltpu.VMEM((8, M), f32),
        pltpu.VMEM((S // 2, M), u32),
        pltpu.VMEM((S, 1), f32),
        pltpu.SemaphoreType.DMA((3,)),
        pltpu.SemaphoreType.DMA((2, 3)),
        pltpu.SemaphoreType.DMA((2, 3)),
    ]
    return pl.pallas_call(
        _kernel,
        grid=(H + NE,),
        in_specs=in_specs,
        out_specs=pl.BlockSpec((None, RE, M), lambda h: (0, jnp.maximum(h - H, 0), 0)),
        out_shape=jax.ShapeDtypeStruct((1, S, M), bf16),
        scratch_shapes=scratch,
        compiler_params=pltpu.CompilerParams(
            dimension_semantics=("arbitrary",),
            vmem_limit_bytes=126 * 1024 * 1024,
        ),
        name="gated_mix_kernel",
    )(A_x, A_c_kv, A_w_q, A_w_uk, A_w_uv, A_w_o.reshape(H * D, M), B_k, B_v, B_ssm_k,
      B_shift_k.T, B_ssm_D, gate_w, fwd, inv)
```

```python
import math

import jax
import jax.numpy as jnp
import numpy as np
import jax.experimental.pallas as pl
import jax.experimental.pallas.tpu as pltpu

f32 = jnp.float32
bf16 = jnp.bfloat16
u32 = jnp.uint32

S = 2048
M = 1024
DC = 512
H = 32
D = 128
T = 128
BQ = 512
NQ = S // BQ
NSUB = BQ // T
RC = 32
DEP_LAG = 1
GROUP = 2
USE_GATE = False
GATE_K = 0.5
GATE_Q = 0.05
C = 128
NCH = S // C
HALF = M // 2
KS = 4
RE = 128
NE = S // RE

QSCALE = (D ** -0.5) * math.log2(math.e)
NEG = -1e30
NT = (((1,), (1,)), ((), ()))


def _dft_matrices():
    freqs = np.concatenate([np.arange(0, C, 2), np.arange(1, C, 2)])
    t = np.arange(C)
    n = ((2 * freqs[:, None] + 1) * t[None, :]) % (4 * C)
    ang = np.pi * n / (2 * C)
    fwd = np.concatenate([np.cos(ang), -np.sin(ang)], axis=0)
    inv = fwd.T / C
    return fwd.astype(np.float32), inv.astype(np.float32)


def _iota(shape, dim):
    return jax.lax.broadcasted_iota(jnp.int32, shape, dim)


def _pk(v):
    return pltpu.bitcast(v, u32)


def _un(u):
    return pltpu.bitcast(u, bf16)


def _ld(ref, r0, r1, cols=slice(None)):
    return _un(ref[r0 // 2: r1 // 2, cols])


def _zero_of(t):
    return (pltpu.bitcast(t, u32) >> 31) & jnp.uint32(2)


class Hooks:
    def __init__(self, items=(), rate=1.0):
        self.items = list(items)
        self.rate = rate
        self.credit = 0.0

    def take(self):
        self.credit += self.rate
        if self.items and self.items[0][0] <= self.credit:
            cost, thunk = self.items.pop(0)
            self.credit -= cost
            return thunk()
        return None

    def flush(self):
        for _, thunk in self.items:
            thunk()
        self.items = []

    def lhs(self, u, tiles=(0,)):
        nrow = u.shape[0] // 8
        cols = [u[:, t * T:(t + 1) * T] for t in range(u.shape[1] // T)]
        for t in tiles:
            parts, start = [], 0
            for r in range(nrow):
                z = self.take()
                if z is not None:
                    if r * 8 > start:
                        parts.append(cols[t][start:r * 8])
                    parts.append(cols[t][r * 8:(r + 1) * 8] | z)
                    start = (r + 1) * 8
            if start < nrow * 8:
                parts.append(cols[t][start:])
            cols[t] = parts[0] if len(parts) == 1 else jnp.concatenate(parts, axis=0)
        return _un(cols[0] if len(cols) == 1 else jnp.concatenate(cols, axis=1))


def _kernel(x_hbm, c_hbm, wq_hbm, wk_hbm, wv_hbm, wo_hbm, k_hbm, v_hbm, sk_hbm,
            sh_ref, sd_ref, gw_ref, fw_ref, iv_ref, o_ref,
            x_s, c_s, wo_s, q_s, k_s, v_s, ctx_s, wqb, wkb, wvb, wq_s, wk_s, wv_s,
            kb, vb, skb, xf, kf, yf, kprev, khalo, kv_s, g_s,
            big_sem, w_sem, ch_sem):
    h = pl.program_id(0)

    def big_copy(n):
        src, dst = ((c_hbm.at[0], c_s), (x_hbm.at[0], x_s), (wo_hbm, wo_s))[n]
        return pltpu.make_async_copy(src.bitcast(u32), dst, big_sem.at[n])

    def w_copies(pair, slot):
        return [
            pltpu.make_async_copy(src.bitcast(u32).at[:, pair, :], dst.at[slot], w_sem.at[slot, n])
            for n, (src, dst) in enumerate(((wq_hbm, wqb), (wk_hbm, wkb), (wv_hbm, wvb)))
        ]

    def chunk_copies(j, slot):
        rows = pl.ds(pl.multiple_of(j * (C // 2), C // 2), C // 2)
        cols = pl.ds(pl.multiple_of(j * C, C), C)
        return [
            pltpu.make_async_copy(k_hbm.at[0].bitcast(u32).at[rows, :], kb.at[slot], ch_sem.at[slot, 0]),
            pltpu.make_async_copy(v_hbm.at[0].bitcast(u32).at[rows, :], vb.at[slot], ch_sem.at[slot, 1]),
            pltpu.make_async_copy(sk_hbm.bitcast(u32).at[:, cols], skb.at[slot], ch_sem.at[slot, 2]),
        ]

    def unpack_weights(slot, parity, which=(0, 1, 2)):
        sh = (16 * (1 - parity)).astype(u32)
        for n in which:
            src, dst = ((wqb, wq_s), (wkb, wk_s), (wvb, wv_s))[n]
            u = (src[slot] << sh) & jnp.uint32(0xFFFF0000)
            dst[...] = _pk(pltpu.bitcast(u, f32).astype(bf16))

    def q_proj(r0, r1, hk):
        lhs = hk.lhs(x_s[r0 // 2: r1 // 2, :], (0, 4))
        q = jnp.dot(lhs, _un(wq_s[...]), preferred_element_type=f32)
        q_s[r0 // 2: r1 // 2, :] = _pk((q * QSCALE).astype(bf16))
        return q

    def k_proj(r0, r1, hk):
        lhs = hk.lhs(c_s[r0 // 2: r1 // 2, :])
        k = jnp.dot(lhs, _un(wk_s[...]), preferred_element_type=f32)
        k_s[r0 // 2: r1 // 2, :] = _pk(k.astype(bf16))
        return k

    def v_proj(r0, r1, hk):
        lhs = hk.lhs(c_s[r0 // 2: r1 // 2, :])
        v = jnp.dot(lhs, _un(wv_s[...]), preferred_element_type=f32)
        v_s[r0 // 2: r1 // 2, :] = _pk(v.astype(bf16))
        return v

    st = {}

    def scores(i, g, hk):
        base = i * BQ
        qu = q_s[base // 2: (base + BQ) // 2, :]
        if g < i:
            st["s", i, g] = jax.lax.dot_general(hk.lhs(qu), _ld(k_s, g * BQ, (g + 1) * BQ), NT,
                                                preferred_element_type=f32)
            return
        q = _un(qu)
        tri = _iota((T, T), 1) <= _iota((T, T), 0)
        sd = []
        for t in range(NSUB):
            s = jax.lax.dot_general(q[t * T:, :], _ld(k_s, base + t * T, base + (t + 1) * T), NT,
                                    preferred_element_type=f32)
            top = jnp.where(tri, s[:T], NEG)
            sd.append(top if t == NSUB - 1 else jnp.concatenate([top, s[T:]], axis=0))
        st["s", i, i] = sd

    def group_tiles(i, g, r0):
        s = st["s", i, g]
        if g < i:
            return [s[r0:r0 + RC, cc * T:(cc + 1) * T] for cc in range(NSUB)]
        return [s[t][r0 - t * T: r0 - t * T + RC] for t in range(r0 // T + 1)]

    def tree(op, xs):
        while len(xs) > 1:
            xs = [op(xs[n], xs[n + 1]) if n + 1 < len(xs) else xs[n] for n in range(0, len(xs), 2)]
        return xs[0]

    chunks = list(range(0, BQ, RC))

    def row_max(i):
        mel = {}
        for g in range(i + 1):
            for r0 in chunks:
                pm = tree(jnp.maximum, group_tiles(i, g, r0))
                mel[r0] = pm if g == 0 else jnp.maximum(mel[r0], pm)
        st["m", i] = {r0: jnp.broadcast_to(jnp.max(mel[r0], axis=1, keepdims=True), (RC, T))
                      for r0 in chunks}

    def context(i, gate):
        base = i * BQ
        mb = st.pop(("m", i))
        lsum = {}
        acc = None
        deps = [] if gate is None else [gate] * DEP_LAG
        for g in range(i + 1):
            ps = {}
            for r0 in chunks:
                m = mb[r0]
                if len(deps) >= DEP_LAG:
                    m = jnp.concatenate([m[:8] + deps[-DEP_LAG], m[8:]], axis=0)
                p = [jnp.exp2(t - m) for t in group_tiles(i, g, r0)]
                part = tree(jnp.add, p)
                lsum[r0] = part if g == 0 else lsum[r0] + part
                deps.append(tree(jnp.add, [lsum[r0][n:n + 8] for n in range(0, RC, 8)]) * 0.0)
                ps[r0] = p
            if g < i:
                pg = jnp.concatenate([jnp.concatenate(ps[r0], axis=1) for r0 in chunks], axis=0)
                pv = jnp.dot(pg.astype(bf16), _ld(v_s, g * BQ, (g + 1) * BQ),
                             preferred_element_type=f32)
                acc = pv if acc is None else acc + pv
            else:
                parts = [None] * NSUB
                for t in range(NSUB):
                    pt = jnp.concatenate([ps[r0][t] for r0 in chunks if r0 >= t * T], axis=0)
                    pv = jnp.dot(pt.astype(bf16), _ld(v_s, base + t * T, base + (t + 1) * T),
                                 preferred_element_type=f32)
                    for r in range(t, NSUB):
                        piece = pv[(r - t) * T:(r - t + 1) * T]
                        parts[r] = piece if parts[r] is None else parts[r] + piece
                diag = jnp.concatenate(parts, axis=0)
                acc = diag if acc is None else acc + diag
            st.pop(("s", i, g))
        for r0 in chunks:
            l = jnp.sum(lsum[r0], axis=1, keepdims=True)
            inv = pl.reciprocal(l, approx=True)
            inv = inv * (2.0 - l * inv)
            ctx_s[h, (base + r0) // 2: (base + r0 + RC) // 2, :] = _pk(
                (acc[r0:r0 + RC] * inv).astype(bf16))

    def conv_forward_x(j, slot):
        pr = pl.ds(pl.multiple_of(j * (C // 2), C // 2), C // 2)
        r = pl.ds(pl.multiple_of(j * C, C), C)
        w = sh_ref[...].astype(f32)
        kc = _un(kb[slot]).astype(f32)
        ext = jnp.concatenate([khalo[...], kc], axis=0)
        ks = kc * w[0:1]
        for lag in range(1, KS):
            ks = ks + ext[8 - lag: 8 + C - lag] * w[lag:lag + 1]
        khalo[...] = kc[C - 8:]
        kvc = (ks * _un(vb[slot]).astype(f32)).astype(bf16)
        kv_s[pr, :] = _pk(kvc)
        xs = jnp.dot(fw_ref[...], kvc, preferred_element_type=f32)
        xf[j, 0] = xs[:, :HALF]
        xf[j, 1] = xs[:, HALF:]
        xg = _un(x_s[pr, :]).astype(f32) * gw_ref[...].astype(f32).reshape(1, M)
        g_s[r, :] = jax.nn.sigmoid(jnp.sum(xg, axis=1, keepdims=True))

    def conv_forward_k(j, slot):
        kn = jax.lax.dot_general(fw_ref[...], _un(skb[slot]), NT, preferred_element_type=f32)
        q4 = C // 2
        kp = kprev[...]
        kw = jnp.concatenate([
            kn[0:q4] - kp[2 * q4:3 * q4],
            kn[q4:2 * q4] + kp[3 * q4:4 * q4],
            kn[2 * q4:3 * q4] + kp[0:q4],
            kn[3 * q4:4 * q4] - kp[q4:2 * q4],
        ], axis=0)
        kprev[...] = kn
        kf[j, 0] = kw[:, :HALF]
        kf[j, 1] = kw[:, HALF:]

    def conv_block_items(n, group):
        half = n % 2
        re = pl.ds(pl.multiple_of((n // 2) * 16, 16), 16)
        im = pl.ds(pl.multiple_of(C + (n // 2) * 16, 16), 16)
        pre = pl.ds(pl.multiple_of((n // 2) * 8, 8), 8)
        pim = pl.ds(pl.multiple_of(C // 2 + (n // 2) * 8, 8), 8)

        acc = {}

        def some(lb, i, a0, a1):
            ln = slice(lb * T, (lb + 1) * T)
            yr, yi = acc.pop((lb, i), (None, None))
            for a in range(a0, a1):
                xr, xi = xf[i - a, half, re, ln], xf[i - a, half, im, ln]
                kr, ki = kf[a, half, re, ln], kf[a, half, im, ln]
                pr = xr * kr - xi * ki
                pi = xr * ki + xi * kr
                yr = pr if yr is None else yr + pr
                yi = pi if yi is None else yi + pi
            if a1 == i + 1:
                yr, yi = _pk(yr.astype(bf16)), _pk(yi.astype(bf16))
                yf[i, half, pre, ln] = yr
                yf[i, half, pim, ln] = yi
                return _zero_of(yr | yi)
            acc[lb, i] = (yr, yi)
            ur, ui = pltpu.bitcast(yr, u32), pltpu.bitcast(yi, u32)
            return _zero_of((ur[:8] | ur[8:]) | (ui[:8] | ui[8:]))

        return [(min(a0 + group, i + 1) - a0,
                 (lambda lb=lb, i=i, a0=a0: some(lb, i, a0, min(a0 + group, i + 1))))
                for lb in range(HALF // T) for i in range(NCH) for a0 in range(0, i + 1, group)]

    def conv_inverse(j):
        dvec = sd_ref[...].astype(f32).reshape(1, M)
        pr = pl.ds(pl.multiple_of(j * (C // 2), C // 2), C // 2)
        y = jnp.concatenate(
            [jnp.dot(iv_ref[...], _un(yf[j, hh]), preferred_element_type=f32)
             for hh in range(2)], axis=1)
        y = y + _un(kv_s[pr, :]).astype(f32) * dvec
        return _un(x_s[pr, :]).astype(f32) * y

    slot = h % 2

    @pl.when(h == 0)
    def _():
        big_copy(0).start()
        first = w_copies(0, 1)
        for cp in first[1:]:
            cp.start()
        kprev[...] = jnp.zeros(kprev.shape, f32)
        khalo[...] = jnp.zeros(khalo.shape, f32)
        big_copy(0).wait()
        big_copy(1).start()
        first[0].start()
        for cp in first[1:]:
            cp.wait()
        unpack_weights(1, h * 0, (1, 2))

        def kv_body(i, carry):
            pr = pl.ds(pl.multiple_of(i * (BQ // 2), BQ // 2), BQ // 2)
            cc = _un(c_s[pr, :])
            k_s[pr, :] = _pk(jnp.dot(cc, _un(wk_s[...]), preferred_element_type=f32).astype(bf16))
            v_s[pr, :] = _pk(jnp.dot(cc, _un(wv_s[...]), preferred_element_type=f32).astype(bf16))
            return carry

        jax.lax.fori_loop(0, NQ, kv_body, 0)
        first[0].wait()
        unpack_weights(1, h * 0, (0,))
        big_copy(1).wait()
        for cp in w_copies(0, 0) + chunk_copies(0, 0):
            cp.start()
        big_copy(2).start()

        def q_body(i, carry):
            pr = pl.ds(pl.multiple_of(i * (BQ // 2), BQ // 2), BQ // 2)
            q = jnp.dot(_un(x_s[pr, :]), _un(wq_s[...]), preferred_element_type=f32)
            q_s[pr, :] = _pk((q * QSCALE).astype(bf16))
            return carry

        jax.lax.fori_loop(0, NQ, q_body, 0)

    def next_weights():
        for cp in w_copies((h + 1) // 2, slot):
            cp.wait()
        for cp in w_copies(jnp.minimum((h + 2) // 2, H // 2 - 1), 1 - slot):
            cp.start()
        unpack_weights(slot, (h + 1) % 2)

    HB = BQ // 2

    def head_step(fill, hk):
        def run(*names):
            gate = None
            for name in names:
                if name in fill:
                    res = fill[name](hk)
                    if res is not None and USE_GATE:
                        r = int(res.shape[0] * (GATE_Q if name[0] == 'Q' else GATE_K)) // 8 * 8
                        gate = pltpu.bitcast(_zero_of(res[r:r + 8]), f32)
            return gate

        for g in range(4):
            scores(3, g, hk)
        row_max(3)
        context(3, run("K3", "Q3a"))
        run("V3")
        for g in range(3):
            scores(2, g, hk)
        row_max(2)
        context(2, run("Q3b", "K2"))
        run("V2")
        for g in range(2):
            scores(1, g, hk)
        row_max(1)
        context(1, run("Q2a", "Q2b"))
        run("V1")
        scores(0, 0, hk)
        row_max(0)
        context(0, run("E0", "E1", "K1", "Q1a", "Q1b"))
        run("V0", "K0", "Q0a", "Q0b")
        hk.flush()

    def proj_fill():
        fill = {}
        for i in range(NQ):
            fill["K%d" % i] = lambda hk, i=i: k_proj(i * BQ, (i + 1) * BQ, hk)
            fill["V%d" % i] = lambda hk, i=i: v_proj(i * BQ, (i + 1) * BQ, hk)
            fill["Q%da" % i] = lambda hk, i=i: q_proj(i * BQ, i * BQ + HB, hk)
            fill["Q%db" % i] = lambda hk, i=i: q_proj(i * BQ + HB, (i + 1) * BQ, hk)
        return fill

    @pl.when(h < NCH)
    def _():
        for cp in chunk_copies(h, slot):
            cp.wait()
        for cp in chunk_copies(jnp.minimum(h + 1, NCH - 1), 1 - slot):
            cp.start()
        next_weights()
        fill = proj_fill()
        fill["E0"] = lambda hk: conv_forward_x(h, slot)
        fill["E1"] = lambda hk: conv_forward_k(h, slot)
        head_step(fill, Hooks())

    @pl.when(jnp.logical_and(h >= NCH, h < H - 1))
    def _():
        next_weights()
        head_step(proj_fill(), Hooks(conv_block_items(h - NCH, GROUP), rate=0.8))

    @pl.when(h == H - 1)
    def _():
        for cp in w_copies(H // 2 - 1, slot) + chunk_copies(NCH - 1, NCH % 2):
            cp.wait()
        big_copy(2).wait()
        head_step({}, Hooks(conv_block_items(NCH - 1, 4), rate=3.0))

    @pl.when(h >= H)
    def _():
        e = h - H
        pr = pl.ds(pl.multiple_of(e * (RE // 2), RE // 2), RE // 2)
        r = pl.ds(pl.multiple_of(e * RE, RE), RE)
        ctx = jnp.concatenate([_un(ctx_s[hh, pr, :]) for hh in range(H)], axis=1)
        b = jnp.concatenate([conv_inverse(e * (RE // C) + j) for j in range(RE // C)], axis=0)
        a = jnp.dot(ctx, _un(wo_s[...]), preferred_element_type=f32)
        g = g_s[r, :]
        o_ref[...] = (b + g * (a - b)).astype(o_ref.dtype)


@jax.jit
def pallas_gated_mix__compressed_kv_cla__ssm_conv_h3__prompt_kernel(
    A_x: jax.Array,
    A_c_kv: jax.Array,
    A_w_q: jax.Array,
    A_w_uk: jax.Array,
    A_w_uv: jax.Array,
    A_w_o: jax.Array,
    B_q: jax.Array,
    B_k: jax.Array,
    B_v: jax.Array,
    B_shift_k: jax.Array,
    B_ssm_k: jax.Array,
    B_ssm_D: jax.Array,
    gate_w: jax.Array,
):
    fwd, inv = _dft_matrices()
    fwd = jnp.asarray(fwd, bf16)
    inv = jnp.asarray(inv, bf16)

    once = pl.Buffered(1)

    def whole(shape):
        return pl.BlockSpec(shape, lambda h: (0,) * len(shape), pipeline_mode=once)

    hbm = pl.BlockSpec(memory_space=pl.ANY)
    in_specs = [hbm] * 9 + [
        whole((KS, M)),
        whole((M,)),
        whole((M,)),
        whole((2 * C, C)),
        whole((C, 2 * C)),
    ]
    scratch = [
        pltpu.VMEM((S // 2, M), u32),
        pltpu.VMEM((S // 2, DC), u32),
        pltpu.VMEM((H * D // 2, M), u32),
        pltpu.VMEM((S // 2, D), u32), pltpu.VMEM((S // 2, D), u32), pltpu.VMEM((S // 2, D), u32),
        pltpu.VMEM((H, S // 2, D), u32),
        pltpu.VMEM((2, M, D), u32), pltpu.VMEM((2, DC, D), u32), pltpu.VMEM((2, DC, D), u32),
        pltpu.VMEM((M // 2, D), u32), pltpu.VMEM((DC // 2, D), u32), pltpu.VMEM((DC // 2, D), u32),
        pltpu.VMEM((2, C // 2, M), u32), pltpu.VMEM((2, C // 2, M), u32),
        pltpu.VMEM((2, M // 2, C), u32),
        pltpu.VMEM((NCH, 2, 2 * C, HALF), f32),
        pltpu.VMEM((NCH, 2, 2 * C, HALF), f32),
        pltpu.VMEM((NCH, 2, C, HALF), u32),
        pltpu.VMEM((2 * C, M), f32),
        pltpu.VMEM((8, M), f32),
        pltpu.VMEM((S // 2, M), u32),
        pltpu.VMEM((S, 1), f32),
        pltpu.SemaphoreType.DMA((3,)),
        pltpu.SemaphoreType.DMA((2, 3)),
        pltpu.SemaphoreType.DMA((2, 3)),
    ]
    return pl.pallas_call(
        _kernel,
        grid=(H + NE,),
        in_specs=in_specs,
        out_specs=pl.BlockSpec((None, RE, M), lambda h: (0, jnp.maximum(h - H, 0), 0)),
        out_shape=jax.ShapeDtypeStruct((1, S, M), bf16),
        scratch_shapes=scratch,
        compiler_params=pltpu.CompilerParams(
            dimension_semantics=("arbitrary",),
            vmem_limit_bytes=126 * 1024 * 1024,
        ),
        name="gated_mix_kernel",
    )(A_x, A_c_kv, A_w_q, A_w_uk, A_w_uv, A_w_o.reshape(H * D, M), B_k, B_v, B_ssm_k,
      B_shift_k.T, B_ssm_D, gate_w, fwd, inv)
```

```python
import math

import jax
import jax.numpy as jnp
import numpy as np
import jax.experimental.pallas as pl
import jax.experimental.pallas.tpu as pltpu

f32 = jnp.float32
bf16 = jnp.bfloat16
u32 = jnp.uint32

S = 2048
M = 1024
DC = 512
H = 32
D = 128
T = 128
BQ = 512
NQ = S // BQ
NSUB = BQ // T
RC = 32
DEP_LAG = 1
GROUP = 2
USE_GATE = False
GATE_K = 0.5
GATE_Q = 0.05
C = 128
NCH = S // C
HALF = M // 2
KS = 4
RE = 128
NE = S // RE

QSCALE = (D ** -0.5) * math.log2(math.e)
NEG = -1e30
NT = (((1,), (1,)), ((), ()))


def _dft_matrices():
    freqs = np.concatenate([np.arange(0, C, 2), np.arange(1, C, 2)])
    t = np.arange(C)
    n = ((2 * freqs[:, None] + 1) * t[None, :]) % (4 * C)
    ang = np.pi * n / (2 * C)
    fwd = np.concatenate([np.cos(ang), -np.sin(ang)], axis=0)
    inv = fwd.T / C
    return fwd.astype(np.float32), inv.astype(np.float32)


def _iota(shape, dim):
    return jax.lax.broadcasted_iota(jnp.int32, shape, dim)


def _pk(v):
    return pltpu.bitcast(v, u32)


def _un(u):
    return pltpu.bitcast(u, bf16)


def _ld(ref, r0, r1, cols=slice(None)):
    return _un(ref[r0 // 2: r1 // 2, cols])


def _zero_of(t):
    return (pltpu.bitcast(t, u32) >> 31) & jnp.uint32(2)


class Hooks:
    def __init__(self, items=(), rate=1.0):
        self.items = list(items)
        self.rate = rate
        self.credit = 0.0

    def take(self):
        self.credit += self.rate
        if self.items and self.items[0][0] <= self.credit:
            cost, thunk = self.items.pop(0)
            self.credit -= cost
            return thunk()
        return None

    def flush(self):
        for _, thunk in self.items:
            thunk()
        self.items = []

    def lhs(self, u, tiles=(0,)):
        nrow = u.shape[0] // 8
        cols = [u[:, t * T:(t + 1) * T] for t in range(u.shape[1] // T)]
        for t in tiles:
            parts, start = [], 0
            for r in range(nrow):
                z = self.take()
                if z is not None:
                    if r * 8 > start:
                        parts.append(cols[t][start:r * 8])
                    parts.append(cols[t][r * 8:(r + 1) * 8] | z)
                    start = (r + 1) * 8
            if start < nrow * 8:
                parts.append(cols[t][start:])
            cols[t] = parts[0] if len(parts) == 1 else jnp.concatenate(parts, axis=0)
        return _un(cols[0] if len(cols) == 1 else jnp.concatenate(cols, axis=1))


def _kernel(x_hbm, c_hbm, wq_hbm, wk_hbm, wv_hbm, wo_hbm, k_hbm, v_hbm, sk_hbm,
            sh_ref, sd_ref, gw_ref, fw_ref, iv_ref, o_ref,
            x_s, c_s, wo_s, q_s, k_s, v_s, ctx_s, wqb, wkb, wvb, wq_s, wk_s, wv_s,
            kb, vb, skb, xf, kf, yf, kprev, khalo, kv_s, g_s,
            big_sem, wo_sem, w_sem, ch_sem):
    h = pl.program_id(0)

    def block_copy(n, i):
        src, dst = ((c_hbm, c_s), (x_hbm, x_s))[n]
        rows = pl.ds(pl.multiple_of(i * (BQ // 2), BQ // 2), BQ // 2)
        return pltpu.make_async_copy(src.at[0].bitcast(u32).at[rows, :], dst.at[rows, :],
                                     big_sem.at[n, i])

    def wo_copy():
        return pltpu.make_async_copy(wo_hbm.bitcast(u32), wo_s, wo_sem.at[0])

    def w_copies(pair, slot):
        return [
            pltpu.make_async_copy(src.bitcast(u32).at[:, pair, :], dst.at[slot], w_sem.at[slot, n])
            for n, (src, dst) in enumerate(((wq_hbm, wqb), (wk_hbm, wkb), (wv_hbm, wvb)))
        ]

    def chunk_copies(j, slot):
        rows = pl.ds(pl.multiple_of(j * (C // 2), C // 2), C // 2)
        cols = pl.ds(pl.multiple_of(j * C, C), C)
        return [
            pltpu.make_async_copy(k_hbm.at[0].bitcast(u32).at[rows, :], kb.at[slot], ch_sem.at[slot, 0]),
            pltpu.make_async_copy(v_hbm.at[0].bitcast(u32).at[rows, :], vb.at[slot], ch_sem.at[slot, 1]),
            pltpu.make_async_copy(sk_hbm.bitcast(u32).at[:, cols], skb.at[slot], ch_sem.at[slot, 2]),
        ]

    def unpack_weights(slot, parity, which=(0, 1, 2)):
        sh = (16 * (1 - parity)).astype(u32)
        for n in which:
            src, dst = ((wqb, wq_s), (wkb, wk_s), (wvb, wv_s))[n]
            u = (src[slot] << sh) & jnp.uint32(0xFFFF0000)
            dst[...] = _pk(pltpu.bitcast(u, f32).astype(bf16))

    def q_proj(r0, r1, hk):
        lhs = hk.lhs(x_s[r0 // 2: r1 // 2, :], (0, 4))
        q = jnp.dot(lhs, _un(wq_s[...]), preferred_element_type=f32)
        q_s[r0 // 2: r1 // 2, :] = _pk((q * QSCALE).astype(bf16))
        return q

    def k_proj(r0, r1, hk):
        lhs = hk.lhs(c_s[r0 // 2: r1 // 2, :])
        k = jnp.dot(lhs, _un(wk_s[...]), preferred_element_type=f32)
        k_s[r0 // 2: r1 // 2, :] = _pk(k.astype(bf16))
        return k

    def v_proj(r0, r1, hk):
        lhs = hk.lhs(c_s[r0 // 2: r1 // 2, :])
        v = jnp.dot(lhs, _un(wv_s[...]), preferred_element_type=f32)
        v_s[r0 // 2: r1 // 2, :] = _pk(v.astype(bf16))
        return v

    st = {}

    def scores(i, g, hk):
        base = i * BQ
        qu = q_s[base // 2: (base + BQ) // 2, :]
        if g < i:
            st["s", i, g] = jax.lax.dot_general(hk.lhs(qu), _ld(k_s, g * BQ, (g + 1) * BQ), NT,
                                                preferred_element_type=f32)
            return
        q = _un(qu)
        tri = _iota((T, T), 1) <= _iota((T, T), 0)
        sd = []
        for t in range(NSUB):
            s = jax.lax.dot_general(q[t * T:, :], _ld(k_s, base + t * T, base + (t + 1) * T), NT,
                                    preferred_element_type=f32)
            top = jnp.where(tri, s[:T], NEG)
            sd.append(top if t == NSUB - 1 else jnp.concatenate([top, s[T:]], axis=0))
        st["s", i, i] = sd

    def group_tiles(i, g, r0):
        s = st["s", i, g]
        if g < i:
            return [s[r0:r0 + RC, cc * T:(cc + 1) * T] for cc in range(NSUB)]
        return [s[t][r0 - t * T: r0 - t * T + RC] for t in range(r0 // T + 1)]

    def tree(op, xs):
        while len(xs) > 1:
            xs = [op(xs[n], xs[n + 1]) if n + 1 < len(xs) else xs[n] for n in range(0, len(xs), 2)]
        return xs[0]

    chunks = list(range(0, BQ, RC))

    def row_max(i):
        mel = {}
        for g in range(i + 1):
            for r0 in chunks:
                pm = tree(jnp.maximum, group_tiles(i, g, r0))
                mel[r0] = pm if g == 0 else jnp.maximum(mel[r0], pm)
        st["m", i] = {r0: jnp.broadcast_to(jnp.max(mel[r0], axis=1, keepdims=True), (RC, T))
                      for r0 in chunks}

    def context(i, gate):
        base = i * BQ
        mb = st.pop(("m", i))
        lsum = {}
        acc = None
        deps = [] if gate is None else [gate] * DEP_LAG
        for g in range(i + 1):
            ps = {}
            for r0 in chunks:
                m = mb[r0]
                if len(deps) >= DEP_LAG:
                    m = jnp.concatenate([m[:8] + deps[-DEP_LAG], m[8:]], axis=0)
                p = [jnp.exp2(t - m) for t in group_tiles(i, g, r0)]
                part = tree(jnp.add, p)
                lsum[r0] = part if g == 0 else lsum[r0] + part
                deps.append(tree(jnp.add, [lsum[r0][n:n + 8] for n in range(0, RC, 8)]) * 0.0)
                ps[r0] = p
            if g < i:
                pg = jnp.concatenate([jnp.concatenate(ps[r0], axis=1) for r0 in chunks], axis=0)
                pv = jnp.dot(pg.astype(bf16), _ld(v_s, g * BQ, (g + 1) * BQ),
                             preferred_element_type=f32)
                acc = pv if acc is None else acc + pv
            else:
                parts = [None] * NSUB
                for t in range(NSUB):
                    pt = jnp.concatenate([ps[r0][t] for r0 in chunks if r0 >= t * T], axis=0)
                    pv = jnp.dot(pt.astype(bf16), _ld(v_s, base + t * T, base + (t + 1) * T),
                                 preferred_element_type=f32)
                    for r in range(t, NSUB):
                        piece = pv[(r - t) * T:(r - t + 1) * T]
                        parts[r] = piece if parts[r] is None else parts[r] + piece
                diag = jnp.concatenate(parts, axis=0)
                acc = diag if acc is None else acc + diag
            st.pop(("s", i, g))
        for r0 in chunks:
            l = jnp.sum(lsum[r0], axis=1, keepdims=True)
            inv = pl.reciprocal(l, approx=True)
            inv = inv * (2.0 - l * inv)
            ctx_s[h, (base + r0) // 2: (base + r0 + RC) // 2, :] = _pk(
                (acc[r0:r0 + RC] * inv).astype(bf16))

    def conv_forward_x(j, slot):
        pr = pl.ds(pl.multiple_of(j * (C // 2), C // 2), C // 2)
        r = pl.ds(pl.multiple_of(j * C, C), C)
        w = sh_ref[...].astype(f32)
        kc = _un(kb[slot]).astype(f32)
        ext = jnp.concatenate([khalo[...], kc], axis=0)
        ks = kc * w[0:1]
        for lag in range(1, KS):
            ks = ks + ext[8 - lag: 8 + C - lag] * w[lag:lag + 1]
        khalo[...] = kc[C - 8:]
        kvc = (ks * _un(vb[slot]).astype(f32)).astype(bf16)
        kv_s[pr, :] = _pk(kvc)
        xs = jnp.dot(fw_ref[...], kvc, preferred_element_type=f32)
        xf[j, 0] = xs[:, :HALF]
        xf[j, 1] = xs[:, HALF:]
        xg = _un(x_s[pr, :]).astype(f32) * gw_ref[...].astype(f32).reshape(1, M)
        g_s[r, :] = jax.nn.sigmoid(jnp.sum(xg, axis=1, keepdims=True))

    def conv_forward_k(j, slot):
        kn = jax.lax.dot_general(fw_ref[...], _un(skb[slot]), NT, preferred_element_type=f32)
        q4 = C // 2
        kp = kprev[...]
        kw = jnp.concatenate([
            kn[0:q4] - kp[2 * q4:3 * q4],
            kn[q4:2 * q4] + kp[3 * q4:4 * q4],
            kn[2 * q4:3 * q4] + kp[0:q4],
            kn[3 * q4:4 * q4] - kp[q4:2 * q4],
        ], axis=0)
        kprev[...] = kn
        kf[j, 0] = kw[:, :HALF]
        kf[j, 1] = kw[:, HALF:]

    def conv_block_items(n, group):
        half = n % 2
        re = pl.ds(pl.multiple_of((n // 2) * 16, 16), 16)
        im = pl.ds(pl.multiple_of(C + (n // 2) * 16, 16), 16)
        pre = pl.ds(pl.multiple_of((n // 2) * 8, 8), 8)
        pim = pl.ds(pl.multiple_of(C // 2 + (n // 2) * 8, 8), 8)

        acc = {}

        def some(lb, i, a0, a1):
            ln = slice(lb * T, (lb + 1) * T)
            yr, yi = acc.pop((lb, i), (None, None))
            for a in range(a0, a1):
                xr, xi = xf[i - a, half, re, ln], xf[i - a, half, im, ln]
                kr, ki = kf[a, half, re, ln], kf[a, half, im, ln]
                pr = xr * kr - xi * ki
                pi = xr * ki + xi * kr
                yr = pr if yr is None else yr + pr
                yi = pi if yi is None else yi + pi
            if a1 == i + 1:
                yr, yi = _pk(yr.astype(bf16)), _pk(yi.astype(bf16))
                yf[i, half, pre, ln] = yr
                yf[i, half, pim, ln] = yi
                return _zero_of(yr | yi)
            acc[lb, i] = (yr, yi)
            ur, ui = pltpu.bitcast(yr, u32), pltpu.bitcast(yi, u32)
            return _zero_of((ur[:8] | ur[8:]) | (ui[:8] | ui[8:]))

        return [(min(a0 + group, i + 1) - a0,
                 (lambda lb=lb, i=i, a0=a0: some(lb, i, a0, min(a0 + group, i + 1))))
                for lb in range(HALF // T) for i in range(NCH) for a0 in range(0, i + 1, group)]

    def conv_inverse(j):
        dvec = sd_ref[...].astype(f32).reshape(1, M)
        pr = pl.ds(pl.multiple_of(j * (C // 2), C // 2), C // 2)
        y = jnp.concatenate(
            [jnp.dot(iv_ref[...], _un(yf[j, hh]), preferred_element_type=f32)
             for hh in range(2)], axis=1)
        y = y + _un(kv_s[pr, :]).astype(f32) * dvec
        return _un(x_s[pr, :]).astype(f32) * y

    slot = h % 2

    @pl.when(h == 0)
    def _():
        first = w_copies(0, 1)
        for cp in first[1:]:
            cp.start()
        for i in range(NQ):
            block_copy(0, i).start()
        first[0].start()
        for i in range(NQ):
            block_copy(1, i).start()
        for cp in chunk_copies(0, 0):
            cp.start()
        kprev[...] = jnp.zeros(kprev.shape, f32)
        khalo[...] = jnp.zeros(khalo.shape, f32)
        for cp in first[1:]:
            cp.wait()
        unpack_weights(1, h * 0, (1, 2))

        def kv_body(i, carry):
            block_copy(0, i).wait()
            pr = pl.ds(pl.multiple_of(i * (BQ // 2), BQ // 2), BQ // 2)
            cc = _un(c_s[pr, :])
            k_s[pr, :] = _pk(jnp.dot(cc, _un(wk_s[...]), preferred_element_type=f32).astype(bf16))
            v_s[pr, :] = _pk(jnp.dot(cc, _un(wv_s[...]), preferred_element_type=f32).astype(bf16))
            return carry

        jax.lax.fori_loop(0, NQ, kv_body, 0)
        first[0].wait()
        unpack_weights(1, h * 0, (0,))
        for n, buf in enumerate((wqb, wkb, wvb)):
            pltpu.make_async_copy(buf.at[1], buf.at[0], w_sem.at[0, n]).start()

        def q_body(i, carry):
            block_copy(1, i).wait()
            pr = pl.ds(pl.multiple_of(i * (BQ // 2), BQ // 2), BQ // 2)
            q = jnp.dot(_un(x_s[pr, :]), _un(wq_s[...]), preferred_element_type=f32)
            q_s[pr, :] = _pk((q * QSCALE).astype(bf16))
            return carry

        jax.lax.fori_loop(0, NQ, q_body, 0)
        wo_copy().start()

    def next_weights():
        for cp in w_copies((h + 1) // 2, slot):
            cp.wait()
        for cp in w_copies(jnp.minimum((h + 2) // 2, H // 2 - 1), 1 - slot):
            cp.start()
        unpack_weights(slot, (h + 1) % 2)

    HB = BQ // 2

    def head_step(fill, hk):
        def run(*names):
            gate = None
            for name in names:
                if name in fill:
                    res = fill[name](hk)
                    if res is not None and USE_GATE:
                        r = int(res.shape[0] * (GATE_Q if name[0] == 'Q' else GATE_K)) // 8 * 8
                        gate = pltpu.bitcast(_zero_of(res[r:r + 8]), f32)
            return gate

        for g in range(4):
            scores(3, g, hk)
        row_max(3)
        context(3, run("K3", "Q3a"))
        run("V3")
        for g in range(3):
            scores(2, g, hk)
        row_max(2)
        context(2, run("Q3b", "K2"))
        run("V2")
        for g in range(2):
            scores(1, g, hk)
        row_max(1)
        context(1, run("Q2a", "Q2b"))
        run("V1")
        scores(0, 0, hk)
        row_max(0)
        context(0, run("E0", "E1", "K1", "Q1a", "Q1b"))
        run("V0", "K0", "Q0a", "Q0b")
        hk.flush()

    def proj_fill():
        fill = {}
        for i in range(NQ):
            fill["K%d" % i] = lambda hk, i=i: k_proj(i * BQ, (i + 1) * BQ, hk)
            fill["V%d" % i] = lambda hk, i=i: v_proj(i * BQ, (i + 1) * BQ, hk)
            fill["Q%da" % i] = lambda hk, i=i: q_proj(i * BQ, i * BQ + HB, hk)
            fill["Q%db" % i] = lambda hk, i=i: q_proj(i * BQ + HB, (i + 1) * BQ, hk)
        return fill

    @pl.when(h < NCH)
    def _():
        for cp in chunk_copies(h, slot):
            cp.wait()
        for cp in chunk_copies(jnp.minimum(h + 1, NCH - 1), 1 - slot):
            cp.start()
        next_weights()
        fill = proj_fill()
        fill["E0"] = lambda hk: conv_forward_x(h, slot)
        fill["E1"] = lambda hk: conv_forward_k(h, slot)
        head_step(fill, Hooks())

    @pl.when(jnp.logical_and(h >= NCH, h < H - 1))
    def _():
        next_weights()
        head_step(proj_fill(), Hooks(conv_block_items(h - NCH, GROUP), rate=0.8))

    @pl.when(h == H - 1)
    def _():
        for cp in w_copies(H // 2 - 1, slot) + chunk_copies(NCH - 1, NCH % 2):
            cp.wait()
        wo_copy().wait()
        head_step({}, Hooks(conv_block_items(NCH - 1, 4), rate=3.0))

    @pl.when(h >= H)
    def _():
        e = h - H
        pr = pl.ds(pl.multiple_of(e * (RE // 2), RE // 2), RE // 2)
        r = pl.ds(pl.multiple_of(e * RE, RE), RE)
        ctx = jnp.concatenate([_un(ctx_s[hh, pr, :]) for hh in range(H)], axis=1)
        b = jnp.concatenate([conv_inverse(e * (RE // C) + j) for j in range(RE // C)], axis=0)
        a = jnp.dot(ctx, _un(wo_s[...]), preferred_element_type=f32)
        g = g_s[r, :]
        o_ref[...] = (b + g * (a - b)).astype(o_ref.dtype)


@jax.jit
def pallas_gated_mix__compressed_kv_cla__ssm_conv_h3__prompt_kernel(
    A_x: jax.Array,
    A_c_kv: jax.Array,
    A_w_q: jax.Array,
    A_w_uk: jax.Array,
    A_w_uv: jax.Array,
    A_w_o: jax.Array,
    B_q: jax.Array,
    B_k: jax.Array,
    B_v: jax.Array,
    B_shift_k: jax.Array,
    B_ssm_k: jax.Array,
    B_ssm_D: jax.Array,
    gate_w: jax.Array,
):
    fwd, inv = _dft_matrices()
    fwd = jnp.asarray(fwd, bf16)
    inv = jnp.asarray(inv, bf16)

    once = pl.Buffered(1)

    def whole(shape):
        return pl.BlockSpec(shape, lambda h: (0,) * len(shape), pipeline_mode=once)

    hbm = pl.BlockSpec(memory_space=pl.ANY)
    in_specs = [hbm] * 9 + [
        whole((KS, M)),
        whole((M,)),
        whole((M,)),
        whole((2 * C, C)),
        whole((C, 2 * C)),
    ]
    scratch = [
        pltpu.VMEM((S // 2, M), u32),
        pltpu.VMEM((S // 2, DC), u32),
        pltpu.VMEM((H * D // 2, M), u32),
        pltpu.VMEM((S // 2, D), u32), pltpu.VMEM((S // 2, D), u32), pltpu.VMEM((S // 2, D), u32),
        pltpu.VMEM((H, S // 2, D), u32),
        pltpu.VMEM((2, M, D), u32), pltpu.VMEM((2, DC, D), u32), pltpu.VMEM((2, DC, D), u32),
        pltpu.VMEM((M // 2, D), u32), pltpu.VMEM((DC // 2, D), u32), pltpu.VMEM((DC // 2, D), u32),
        pltpu.VMEM((2, C // 2, M), u32), pltpu.VMEM((2, C // 2, M), u32),
        pltpu.VMEM((2, M // 2, C), u32),
        pltpu.VMEM((NCH, 2, 2 * C, HALF), f32),
        pltpu.VMEM((NCH, 2, 2 * C, HALF), f32),
        pltpu.VMEM((NCH, 2, C, HALF), u32),
        pltpu.VMEM((2 * C, M), f32),
        pltpu.VMEM((8, M), f32),
        pltpu.VMEM((S // 2, M), u32),
        pltpu.VMEM((S, 1), f32),
        pltpu.SemaphoreType.DMA((2, NQ)),
        pltpu.SemaphoreType.DMA((1,)),
        pltpu.SemaphoreType.DMA((2, 3)),
        pltpu.SemaphoreType.DMA((2, 3)),
    ]
    return pl.pallas_call(
        _kernel,
        grid=(H + NE,),
        in_specs=in_specs,
        out_specs=pl.BlockSpec((None, RE, M), lambda h: (0, jnp.maximum(h - H, 0), 0)),
        out_shape=jax.ShapeDtypeStruct((1, S, M), bf16),
        scratch_shapes=scratch,
        compiler_params=pltpu.CompilerParams(
            dimension_semantics=("arbitrary",),
            vmem_limit_bytes=126 * 1024 * 1024,
        ),
        name="gated_mix_kernel",
    )(A_x, A_c_kv, A_w_q, A_w_uk, A_w_uv, A_w_o.reshape(H * D, M), B_k, B_v, B_ssm_k,
      B_shift_k.T, B_ssm_D, gate_w, fwd, inv)
```

```python
import math

import jax
import jax.numpy as jnp
import numpy as np
import jax.experimental.pallas as pl
import jax.experimental.pallas.tpu as pltpu

f32 = jnp.float32
bf16 = jnp.bfloat16
u32 = jnp.uint32

S = 2048
M = 1024
DC = 512
H = 32
D = 128
T = 128
BQ = 512
NQ = S // BQ
NSUB = BQ // T
RC = 32
DEP_LAG = 1
GROUP = 2
USE_GATE = False
GATE_K = 0.5
GATE_Q = 0.05
C = 128
NCH = S // C
HALF = M // 2
KS = 4
RE = 256
NE = S // RE

QSCALE = (D ** -0.5) * math.log2(math.e)
NEG = -1e30
NT = (((1,), (1,)), ((), ()))


def _dft_matrices():
    freqs = np.concatenate([np.arange(0, C, 2), np.arange(1, C, 2)])
    t = np.arange(C)
    n = ((2 * freqs[:, None] + 1) * t[None, :]) % (4 * C)
    ang = np.pi * n / (2 * C)
    fwd = np.concatenate([np.cos(ang), -np.sin(ang)], axis=0)
    inv = fwd.T / C
    return fwd.astype(np.float32), inv.astype(np.float32)


def _iota(shape, dim):
    return jax.lax.broadcasted_iota(jnp.int32, shape, dim)


def _pk(v):
    return pltpu.bitcast(v, u32)


def _un(u):
    return pltpu.bitcast(u, bf16)


def _ld(ref, r0, r1, cols=slice(None)):
    return _un(ref[r0 // 2: r1 // 2, cols])


def _zero_of(t):
    return (pltpu.bitcast(t, u32) >> 31) & jnp.uint32(2)


class Hooks:
    def __init__(self, items=(), rate=1.0):
        self.items = list(items)
        self.rate = rate
        self.credit = 0.0

    def take(self):
        self.credit += self.rate
        if self.items and self.items[0][0] <= self.credit:
            cost, thunk = self.items.pop(0)
            self.credit -= cost
            return thunk()
        return None

    def flush(self):
        for _, thunk in self.items:
            thunk()
        self.items = []

    def lhs(self, u, tiles=(0,)):
        nrow = u.shape[0] // 8
        cols = [u[:, t * T:(t + 1) * T] for t in range(u.shape[1] // T)]
        for t in tiles:
            parts, start = [], 0
            for r in range(nrow):
                z = self.take()
                if z is not None:
                    if r * 8 > start:
                        parts.append(cols[t][start:r * 8])
                    parts.append(cols[t][r * 8:(r + 1) * 8] | z)
                    start = (r + 1) * 8
            if start < nrow * 8:
                parts.append(cols[t][start:])
            cols[t] = parts[0] if len(parts) == 1 else jnp.concatenate(parts, axis=0)
        return _un(cols[0] if len(cols) == 1 else jnp.concatenate(cols, axis=1))


def _kernel(x_hbm, c_hbm, wq_hbm, wk_hbm, wv_hbm, wo_hbm, k_hbm, v_hbm, sk_hbm,
            sh_hbm, sd_hbm, gw_hbm, fw_hbm, iv_hbm, o_ref,
            x_s, c_s, wo_s, q_s, k_s, v_s, ctx_s, wqb, wkb, wvb, wq_s, wk_s, wv_s,
            kb, vb, skb, xf, kf, yf, kprev, khalo, kv_s, g_s,
            sh_ref, sd_ref, gw_ref, fw_ref, iv_ref, small_sem, big_sem, wo_sem, w_sem, ch_sem):
    h = pl.program_id(0)

    def block_copy(n, i):
        src, dst = ((c_hbm, c_s), (x_hbm, x_s))[n]
        rows = pl.ds(pl.multiple_of(i * (BQ // 2), BQ // 2), BQ // 2)
        return pltpu.make_async_copy(src.at[0].bitcast(u32).at[rows, :], dst.at[rows, :],
                                     big_sem.at[n, i])

    def small_copies():
        pairs = ((sh_hbm, sh_ref), (sd_hbm, sd_ref), (gw_hbm, gw_ref), (fw_hbm, fw_ref),
                 (iv_hbm, iv_ref))
        return [pltpu.make_async_copy(src, dst, small_sem.at[n])
                for n, (src, dst) in enumerate(pairs)]

    def wo_copy():
        return pltpu.make_async_copy(wo_hbm.bitcast(u32), wo_s, wo_sem.at[0])

    def w_copies(pair, slot):
        return [
            pltpu.make_async_copy(src.bitcast(u32).at[:, pair, :], dst.at[slot], w_sem.at[slot, n])
            for n, (src, dst) in enumerate(((wq_hbm, wqb), (wk_hbm, wkb), (wv_hbm, wvb)))
        ]

    def chunk_copies(j, slot):
        rows = pl.ds(pl.multiple_of(j * (C // 2), C // 2), C // 2)
        cols = pl.ds(pl.multiple_of(j * C, C), C)
        return [
            pltpu.make_async_copy(k_hbm.at[0].bitcast(u32).at[rows, :], kb.at[slot], ch_sem.at[slot, 0]),
            pltpu.make_async_copy(v_hbm.at[0].bitcast(u32).at[rows, :], vb.at[slot], ch_sem.at[slot, 1]),
            pltpu.make_async_copy(sk_hbm.bitcast(u32).at[:, cols], skb.at[slot], ch_sem.at[slot, 2]),
        ]

    def unpack_weights(slot, parity, which=(0, 1, 2)):
        sh = (16 * (1 - parity)).astype(u32)
        for n in which:
            src, dst = ((wqb, wq_s), (wkb, wk_s), (wvb, wv_s))[n]
            u = (src[slot] << sh) & jnp.uint32(0xFFFF0000)
            dst[...] = _pk(pltpu.bitcast(u, f32).astype(bf16))

    def q_proj(r0, r1, hk):
        lhs = hk.lhs(x_s[r0 // 2: r1 // 2, :], (0, 4))
        q = jnp.dot(lhs, _un(wq_s[...]), preferred_element_type=f32)
        q_s[r0 // 2: r1 // 2, :] = _pk((q * QSCALE).astype(bf16))
        return q

    def k_proj(r0, r1, hk):
        lhs = hk.lhs(c_s[r0 // 2: r1 // 2, :])
        k = jnp.dot(lhs, _un(wk_s[...]), preferred_element_type=f32)
        k_s[r0 // 2: r1 // 2, :] = _pk(k.astype(bf16))
        return k

    def v_proj(r0, r1, hk):
        lhs = hk.lhs(c_s[r0 // 2: r1 // 2, :])
        v = jnp.dot(lhs, _un(wv_s[...]), preferred_element_type=f32)
        v_s[r0 // 2: r1 // 2, :] = _pk(v.astype(bf16))
        return v

    st = {}

    def scores(i, g, hk):
        base = i * BQ
        qu = q_s[base // 2: (base + BQ) // 2, :]
        if g < i:
            st["s", i, g] = jax.lax.dot_general(hk.lhs(qu), _ld(k_s, g * BQ, (g + 1) * BQ), NT,
                                                preferred_element_type=f32)
            return
        q = _un(qu)
        tri = _iota((T, T), 1) <= _iota((T, T), 0)
        sd = []
        for t in range(NSUB):
            s = jax.lax.dot_general(q[t * T:, :], _ld(k_s, base + t * T, base + (t + 1) * T), NT,
                                    preferred_element_type=f32)
            top = jnp.where(tri, s[:T], NEG)
            sd.append(top if t == NSUB - 1 else jnp.concatenate([top, s[T:]], axis=0))
        st["s", i, i] = sd

    def group_tiles(i, g, r0):
        s = st["s", i, g]
        if g < i:
            return [s[r0:r0 + RC, cc * T:(cc + 1) * T] for cc in range(NSUB)]
        return [s[t][r0 - t * T: r0 - t * T + RC] for t in range(r0 // T + 1)]

    def tree(op, xs):
        while len(xs) > 1:
            xs = [op(xs[n], xs[n + 1]) if n + 1 < len(xs) else xs[n] for n in range(0, len(xs), 2)]
        return xs[0]

    chunks = list(range(0, BQ, RC))

    def row_max(i):
        mel = {}
        for g in range(i + 1):
            for r0 in chunks:
                pm = tree(jnp.maximum, group_tiles(i, g, r0))
                mel[r0] = pm if g == 0 else jnp.maximum(mel[r0], pm)
        st["m", i] = {r0: jnp.broadcast_to(jnp.max(mel[r0], axis=1, keepdims=True), (RC, T))
                      for r0 in chunks}

    def context(i, gate):
        base = i * BQ
        mb = st.pop(("m", i))
        lsum = {}
        acc = None
        deps = [] if gate is None else [gate] * DEP_LAG
        for g in range(i + 1):
            ps = {}
            for r0 in chunks:
                m = mb[r0]
                if len(deps) >= DEP_LAG:
                    m = jnp.concatenate([m[:8] + deps[-DEP_LAG], m[8:]], axis=0)
                p = [jnp.exp2(t - m) for t in group_tiles(i, g, r0)]
                part = tree(jnp.add, p)
                lsum[r0] = part if g == 0 else lsum[r0] + part
                deps.append(tree(jnp.add, [lsum[r0][n:n + 8] for n in range(0, RC, 8)]) * 0.0)
                ps[r0] = p
            if g < i:
                pg = jnp.concatenate([jnp.concatenate(ps[r0], axis=1) for r0 in chunks], axis=0)
                pv = jnp.dot(pg.astype(bf16), _ld(v_s, g * BQ, (g + 1) * BQ),
                             preferred_element_type=f32)
                acc = pv if acc is None else acc + pv
            else:
                parts = [None] * NSUB
                for t in range(NSUB):
                    pt = jnp.concatenate([ps[r0][t] for r0 in chunks if r0 >= t * T], axis=0)
                    pv = jnp.dot(pt.astype(bf16), _ld(v_s, base + t * T, base + (t + 1) * T),
                                 preferred_element_type=f32)
                    for r in range(t, NSUB):
                        piece = pv[(r - t) * T:(r - t + 1) * T]
                        parts[r] = piece if parts[r] is None else parts[r] + piece
                diag = jnp.concatenate(parts, axis=0)
                acc = diag if acc is None else acc + diag
            st.pop(("s", i, g))
        for r0 in chunks:
            l = jnp.sum(lsum[r0], axis=1, keepdims=True)
            inv = pl.reciprocal(l, approx=True)
            inv = inv * (2.0 - l * inv)
            ctx_s[h, (base + r0) // 2: (base + r0 + RC) // 2, :] = _pk(
                (acc[r0:r0 + RC] * inv).astype(bf16))

    def conv_forward_x(j, slot):
        pr = pl.ds(pl.multiple_of(j * (C // 2), C // 2), C // 2)
        r = pl.ds(pl.multiple_of(j * C, C), C)
        w = sh_ref[...].astype(f32)
        kc = _un(kb[slot]).astype(f32)
        ext = jnp.concatenate([khalo[...], kc], axis=0)
        ks = kc * w[0:1]
        for lag in range(1, KS):
            ks = ks + ext[8 - lag: 8 + C - lag] * w[lag:lag + 1]
        khalo[...] = kc[C - 8:]
        kvc = (ks * _un(vb[slot]).astype(f32)).astype(bf16)
        kv_s[pr, :] = _pk(kvc)
        xs = jnp.dot(fw_ref[...], kvc, preferred_element_type=f32)
        xf[j, 0] = xs[:, :HALF]
        xf[j, 1] = xs[:, HALF:]
        xg = _un(x_s[pr, :]).astype(f32) * gw_ref[...].astype(f32).reshape(1, M)
        g_s[r, :] = jax.nn.sigmoid(jnp.sum(xg, axis=1, keepdims=True))

    def conv_forward_k(j, slot):
        kn = jax.lax.dot_general(fw_ref[...], _un(skb[slot]), NT, preferred_element_type=f32)
        q4 = C // 2
        kp = kprev[...]
        kw = jnp.concatenate([
            kn[0:q4] - kp[2 * q4:3 * q4],
            kn[q4:2 * q4] + kp[3 * q4:4 * q4],
            kn[2 * q4:3 * q4] + kp[0:q4],
            kn[3 * q4:4 * q4] - kp[q4:2 * q4],
        ], axis=0)
        kprev[...] = kn
        kf[j, 0] = kw[:, :HALF]
        kf[j, 1] = kw[:, HALF:]

    def conv_block_items(n, group):
        half = n % 2
        re = pl.ds(pl.multiple_of((n // 2) * 16, 16), 16)
        im = pl.ds(pl.multiple_of(C + (n // 2) * 16, 16), 16)
        pre = pl.ds(pl.multiple_of((n // 2) * 8, 8), 8)
        pim = pl.ds(pl.multiple_of(C // 2 + (n // 2) * 8, 8), 8)

        acc = {}

        def some(lb, i, a0, a1):
            ln = slice(lb * T, (lb + 1) * T)
            yr, yi = acc.pop((lb, i), (None, None))
            for a in range(a0, a1):
                xr, xi = xf[i - a, half, re, ln], xf[i - a, half, im, ln]
                kr, ki = kf[a, half, re, ln], kf[a, half, im, ln]
                pr = xr * kr - xi * ki
                pi = xr * ki + xi * kr
                yr = pr if yr is None else yr + pr
                yi = pi if yi is None else yi + pi
            if a1 == i + 1:
                yr, yi = _pk(yr.astype(bf16)), _pk(yi.astype(bf16))
                yf[i, half, pre, ln] = yr
                yf[i, half, pim, ln] = yi
                return _zero_of(yr | yi)
            acc[lb, i] = (yr, yi)
            ur, ui = pltpu.bitcast(yr, u32), pltpu.bitcast(yi, u32)
            return _zero_of((ur[:8] | ur[8:]) | (ui[:8] | ui[8:]))

        return [(min(a0 + group, i + 1) - a0,
                 (lambda lb=lb, i=i, a0=a0: some(lb, i, a0, min(a0 + group, i + 1))))
                for lb in range(HALF // T) for i in range(NCH) for a0 in range(0, i + 1, group)]

    def conv_inverse(j):
        dvec = sd_ref[...].astype(f32).reshape(1, M)
        pr = pl.ds(pl.multiple_of(j * (C // 2), C // 2), C // 2)
        y = jnp.concatenate(
            [jnp.dot(iv_ref[...], _un(yf[j, hh]), preferred_element_type=f32)
             for hh in range(2)], axis=1)
        y = y + _un(kv_s[pr, :]).astype(f32) * dvec
        return _un(x_s[pr, :]).astype(f32) * y

    slot = h % 2

    @pl.when(h == 0)
    def _():
        first = w_copies(0, 1)
        for cp in first[1:]:
            cp.start()
        for i in range(NQ):
            block_copy(0, i).start()
        first[0].start()
        for i in range(NQ):
            block_copy(1, i).start()
        for cp in chunk_copies(0, 0) + small_copies():
            cp.start()
        kprev[...] = jnp.zeros(kprev.shape, f32)
        khalo[...] = jnp.zeros(khalo.shape, f32)
        for cp in first[1:]:
            cp.wait()
        unpack_weights(1, h * 0, (1, 2))

        def kv_body(i, carry):
            block_copy(0, i).wait()
            pr = pl.ds(pl.multiple_of(i * (BQ // 2), BQ // 2), BQ // 2)
            cc = _un(c_s[pr, :])
            k_s[pr, :] = _pk(jnp.dot(cc, _un(wk_s[...]), preferred_element_type=f32).astype(bf16))
            v_s[pr, :] = _pk(jnp.dot(cc, _un(wv_s[...]), preferred_element_type=f32).astype(bf16))
            return carry

        jax.lax.fori_loop(0, NQ, kv_body, 0)
        first[0].wait()
        unpack_weights(1, h * 0, (0,))
        for n, buf in enumerate((wqb, wkb, wvb)):
            pltpu.make_async_copy(buf.at[1], buf.at[0], w_sem.at[0, n]).start()

        def q_body(i, carry):
            block_copy(1, i).wait()
            pr = pl.ds(pl.multiple_of(i * (BQ // 2), BQ // 2), BQ // 2)
            q = jnp.dot(_un(x_s[pr, :]), _un(wq_s[...]), preferred_element_type=f32)
            q_s[pr, :] = _pk((q * QSCALE).astype(bf16))
            return carry

        jax.lax.fori_loop(0, NQ, q_body, 0)
        for cp in small_copies():
            cp.wait()
        wo_copy().start()

    def next_weights():
        for cp in w_copies((h + 1) // 2, slot):
            cp.wait()
        for cp in w_copies(jnp.minimum((h + 2) // 2, H // 2 - 1), 1 - slot):
            cp.start()
        unpack_weights(slot, (h + 1) % 2)

    HB = BQ // 2

    def head_step(fill, hk):
        def run(*names):
            gate = None
            for name in names:
                if name in fill:
                    res = fill[name](hk)
                    if res is not None and USE_GATE:
                        r = int(res.shape[0] * (GATE_Q if name[0] == 'Q' else GATE_K)) // 8 * 8
                        gate = pltpu.bitcast(_zero_of(res[r:r + 8]), f32)
            return gate

        for g in range(4):
            scores(3, g, hk)
        row_max(3)
        context(3, run("K3", "Q3a"))
        run("V3")
        for g in range(3):
            scores(2, g, hk)
        row_max(2)
        context(2, run("Q3b", "K2"))
        run("V2")
        for g in range(2):
            scores(1, g, hk)
        row_max(1)
        context(1, run("Q2a", "Q2b"))
        run("V1")
        scores(0, 0, hk)
        row_max(0)
        context(0, run("E0", "E1", "K1", "Q1a", "Q1b"))
        run("V0", "K0", "Q0a", "Q0b")
        hk.flush()

    def proj_fill():
        fill = {}
        for i in range(NQ):
            fill["K%d" % i] = lambda hk, i=i: k_proj(i * BQ, (i + 1) * BQ, hk)
            fill["V%d" % i] = lambda hk, i=i: v_proj(i * BQ, (i + 1) * BQ, hk)
            fill["Q%da" % i] = lambda hk, i=i: q_proj(i * BQ, i * BQ + HB, hk)
            fill["Q%db" % i] = lambda hk, i=i: q_proj(i * BQ + HB, (i + 1) * BQ, hk)
        return fill

    @pl.when(h < NCH)
    def _():
        for cp in chunk_copies(h, slot):
            cp.wait()
        for cp in chunk_copies(jnp.minimum(h + 1, NCH - 1), 1 - slot):
            cp.start()
        next_weights()
        fill = proj_fill()
        fill["E0"] = lambda hk: conv_forward_x(h, slot)
        fill["E1"] = lambda hk: conv_forward_k(h, slot)
        head_step(fill, Hooks())

    @pl.when(jnp.logical_and(h >= NCH, h < H - 1))
    def _():
        next_weights()
        head_step(proj_fill(), Hooks(conv_block_items(h - NCH, GROUP), rate=0.8))

    @pl.when(h == H - 1)
    def _():
        for cp in w_copies(H // 2 - 1, slot) + chunk_copies(NCH - 1, NCH % 2):
            cp.wait()
        wo_copy().wait()
        head_step({}, Hooks(conv_block_items(NCH - 1, 4), rate=3.0))

    @pl.when(h >= H)
    def _():
        e = h - H
        pr = pl.ds(pl.multiple_of(e * (RE // 2), RE // 2), RE // 2)
        r = pl.ds(pl.multiple_of(e * RE, RE), RE)
        ctx = jnp.concatenate([_un(ctx_s[hh, pr, :]) for hh in range(H)], axis=1)
        b = jnp.concatenate([conv_inverse(e * (RE // C) + j) for j in range(RE // C)], axis=0)
        a = jnp.dot(ctx, _un(wo_s[...]), preferred_element_type=f32)
        g = g_s[r, :]
        o_ref[...] = (b + g * (a - b)).astype(o_ref.dtype)


@jax.jit
def pallas_gated_mix__compressed_kv_cla__ssm_conv_h3__prompt_kernel(
    A_x: jax.Array,
    A_c_kv: jax.Array,
    A_w_q: jax.Array,
    A_w_uk: jax.Array,
    A_w_uv: jax.Array,
    A_w_o: jax.Array,
    B_q: jax.Array,
    B_k: jax.Array,
    B_v: jax.Array,
    B_shift_k: jax.Array,
    B_ssm_k: jax.Array,
    B_ssm_D: jax.Array,
    gate_w: jax.Array,
):
    fwd, inv = _dft_matrices()
    fwd = jnp.asarray(fwd, bf16)
    inv = jnp.asarray(inv, bf16)

    in_specs = [pl.BlockSpec(memory_space=pl.ANY)] * 14
    scratch = [
        pltpu.VMEM((S // 2, M), u32),
        pltpu.VMEM((S // 2, DC), u32),
        pltpu.VMEM((H * D // 2, M), u32),
        pltpu.VMEM((S // 2, D), u32), pltpu.VMEM((S // 2, D), u32), pltpu.VMEM((S // 2, D), u32),
        pltpu.VMEM((H, S // 2, D), u32),
        pltpu.VMEM((2, M, D), u32), pltpu.VMEM((2, DC, D), u32), pltpu.VMEM((2, DC, D), u32),
        pltpu.VMEM((M // 2, D), u32), pltpu.VMEM((DC // 2, D), u32), pltpu.VMEM((DC // 2, D), u32),
        pltpu.VMEM((2, C // 2, M), u32), pltpu.VMEM((2, C // 2, M), u32),
        pltpu.VMEM((2, M // 2, C), u32),
        pltpu.VMEM((NCH, 2, 2 * C, HALF), f32),
        pltpu.VMEM((NCH, 2, 2 * C, HALF), f32),
        pltpu.VMEM((NCH, 2, C, HALF), u32),
        pltpu.VMEM((2 * C, M), f32),
        pltpu.VMEM((8, M), f32),
        pltpu.VMEM((S // 2, M), u32),
        pltpu.VMEM((S, 1), f32),
        pltpu.VMEM((KS, M), bf16), pltpu.VMEM((M,), bf16), pltpu.VMEM((M,), bf16),
        pltpu.VMEM((2 * C, C), bf16), pltpu.VMEM((C, 2 * C), bf16),
        pltpu.SemaphoreType.DMA((5,)),
        pltpu.SemaphoreType.DMA((2, NQ)),
        pltpu.SemaphoreType.DMA((1,)),
        pltpu.SemaphoreType.DMA((2, 3)),
        pltpu.SemaphoreType.DMA((2, 3)),
    ]
    return pl.pallas_call(
        _kernel,
        grid=(H + NE,),
        in_specs=in_specs,
        out_specs=pl.BlockSpec((None, RE, M), lambda h: (0, jnp.maximum(h - H, 0), 0)),
        out_shape=jax.ShapeDtypeStruct((1, S, M), bf16),
        scratch_shapes=scratch,
        compiler_params=pltpu.CompilerParams(
            dimension_semantics=("arbitrary",),
            vmem_limit_bytes=126 * 1024 * 1024,
        ),
        name="gated_mix_kernel",
    )(A_x, A_c_kv, A_w_q, A_w_uk, A_w_uv, A_w_o.reshape(H * D, M), B_k, B_v, B_ssm_k,
      B_shift_k.T, B_ssm_D, gate_w, fwd, inv)
```

```python
import math

import jax
import jax.numpy as jnp
import numpy as np
import jax.experimental.pallas as pl
import jax.experimental.pallas.tpu as pltpu

f32 = jnp.float32
bf16 = jnp.bfloat16
u32 = jnp.uint32

S = 2048
M = 1024
DC = 512
H = 32
D = 128
T = 128
BQ = 512
NQ = S // BQ
NSUB = BQ // T
RC = 32
DEP_LAG = 1
GROUP = 1
URGENT_EVERY = 1000
DIAG_FIRST = True
PV_DIAG_FIRST = True
FILL_ORDER = {
    3: (("K3", "Q3a"), ("V3",)),
    2: (("Q3b", "K2"), ("V2",)),
    1: (("Q2a", "Q2b"), ("V1",)),
    0: (("K1", "Q1a", "Q1b"), ("V0", "E0", "E1", "K0", "Q0a", "Q0b")),
}
USE_GATE = False
GATE_K = 0.5
GATE_Q = 0.05
C = 128
NCH = S // C
HALF = M // 2
KS = 4
RE = 256
NE = S // RE

QSCALE = (D ** -0.5) * math.log2(math.e)
NEG = -1e30
NT = (((1,), (1,)), ((), ()))


def _dft_matrices():
    freqs = np.concatenate([np.arange(0, C, 2), np.arange(1, C, 2)])
    t = np.arange(C)
    n = ((2 * freqs[:, None] + 1) * t[None, :]) % (4 * C)
    ang = np.pi * n / (2 * C)
    fwd = np.concatenate([np.cos(ang), -np.sin(ang)], axis=0)
    inv = fwd.T / C
    return fwd.astype(np.float32), inv.astype(np.float32)


def _iota(shape, dim):
    return jax.lax.broadcasted_iota(jnp.int32, shape, dim)


def _pk(v):
    return pltpu.bitcast(v, u32)


def _un(u):
    return pltpu.bitcast(u, bf16)


def _ld(ref, r0, r1, cols=slice(None)):
    return _un(ref[r0 // 2: r1 // 2, cols])


def _zero_of(t):
    return (pltpu.bitcast(t, u32) >> 31) & jnp.uint32(2)


class Hooks:
    def __init__(self, items=(), rate=1.0):
        self.items = list(items)
        self.urgent = []
        self.rate = rate
        self.credit = 0.0
        self.count = 0

    def take(self):
        zs = []
        self.count += 1
        if self.urgent and self.count % URGENT_EVERY == 0:
            zs.append(self.urgent.pop(0)())
        self.credit += self.rate
        if self.items and self.items[0][0] <= self.credit:
            cost, thunk = self.items.pop(0)
            self.credit -= cost
            zs.append(thunk())
        if not zs:
            return None
        return zs[0] if len(zs) == 1 else zs[0] | zs[1]

    def flush_urgent(self):
        for thunk in self.urgent:
            thunk()
        self.urgent = []

    def flush(self):
        self.flush_urgent()
        for _, thunk in self.items:
            thunk()
        self.items = []

    def lhs(self, u, tiles=(0,)):
        nrow = u.shape[0] // 8
        cols = [u[:, t * T:(t + 1) * T] for t in range(u.shape[1] // T)]
        for t in tiles:
            parts, start = [], 0
            for r in range(nrow):
                z = self.take()
                if z is not None:
                    if r * 8 > start:
                        parts.append(cols[t][start:r * 8])
                    parts.append(cols[t][r * 8:(r + 1) * 8] | z)
                    start = (r + 1) * 8
            if start < nrow * 8:
                parts.append(cols[t][start:])
            cols[t] = parts[0] if len(parts) == 1 else jnp.concatenate(parts, axis=0)
        return _un(cols[0] if len(cols) == 1 else jnp.concatenate(cols, axis=1))


def _kernel(x_hbm, c_hbm, wq_hbm, wk_hbm, wv_hbm, wo_hbm, k_hbm, v_hbm, sk_hbm,
            sh_hbm, sd_hbm, gw_hbm, fw_hbm, iv_hbm, o_ref,
            x_s, c_s, wo_s, q_s, k_s, v_s, ctx_s, wqb, wkb, wvb, wq_s, wk_s, wv_s,
            kb, vb, skb, xf, kf, yf, kprev, khalo, kv_s, g_s,
            sh_ref, sd_ref, gw_ref, fw_ref, iv_ref, small_sem, big_sem, wo_sem, w_sem, ch_sem):
    h = pl.program_id(0)

    def block_copy(n, i):
        src, dst = ((c_hbm, c_s), (x_hbm, x_s))[n]
        rows = pl.ds(pl.multiple_of(i * (BQ // 2), BQ // 2), BQ // 2)
        return pltpu.make_async_copy(src.at[0].bitcast(u32).at[rows, :], dst.at[rows, :],
                                     big_sem.at[n, i])

    def small_copies():
        pairs = ((sh_hbm, sh_ref), (sd_hbm, sd_ref), (gw_hbm, gw_ref), (fw_hbm, fw_ref),
                 (iv_hbm, iv_ref))
        return [pltpu.make_async_copy(src, dst, small_sem.at[n])
                for n, (src, dst) in enumerate(pairs)]

    def wo_copy():
        return pltpu.make_async_copy(wo_hbm.bitcast(u32), wo_s, wo_sem.at[0])

    def w_copies(pair, slot):
        return [
            pltpu.make_async_copy(src.bitcast(u32).at[:, pair, :], dst.at[slot], w_sem.at[slot, n])
            for n, (src, dst) in enumerate(((wq_hbm, wqb), (wk_hbm, wkb), (wv_hbm, wvb)))
        ]

    def chunk_copies(j, slot):
        rows = pl.ds(pl.multiple_of(j * (C // 2), C // 2), C // 2)
        cols = pl.ds(pl.multiple_of(j * C, C), C)
        return [
            pltpu.make_async_copy(k_hbm.at[0].bitcast(u32).at[rows, :], kb.at[slot], ch_sem.at[slot, 0]),
            pltpu.make_async_copy(v_hbm.at[0].bitcast(u32).at[rows, :], vb.at[slot], ch_sem.at[slot, 1]),
            pltpu.make_async_copy(sk_hbm.bitcast(u32).at[:, cols], skb.at[slot], ch_sem.at[slot, 2]),
        ]

    def unpack_weights(slot, parity, which=(0, 1, 2)):
        sh = (16 * (1 - parity)).astype(u32)
        for n in which:
            src, dst = ((wqb, wq_s), (wkb, wk_s), (wvb, wv_s))[n]
            u = (src[slot] << sh) & jnp.uint32(0xFFFF0000)
            dst[...] = _pk(pltpu.bitcast(u, f32).astype(bf16))

    def q_proj(r0, r1, hk):
        lhs = hk.lhs(x_s[r0 // 2: r1 // 2, :], (0, 4))
        q = jnp.dot(lhs, _un(wq_s[...]), preferred_element_type=f32)
        q_s[r0 // 2: r1 // 2, :] = _pk((q * QSCALE).astype(bf16))
        return q

    def k_proj(r0, r1, hk):
        lhs = hk.lhs(c_s[r0 // 2: r1 // 2, :])
        k = jnp.dot(lhs, _un(wk_s[...]), preferred_element_type=f32)
        k_s[r0 // 2: r1 // 2, :] = _pk(k.astype(bf16))
        return k

    def v_proj(r0, r1, hk):
        lhs = hk.lhs(c_s[r0 // 2: r1 // 2, :])
        v = jnp.dot(lhs, _un(wv_s[...]), preferred_element_type=f32)
        v_s[r0 // 2: r1 // 2, :] = _pk(v.astype(bf16))
        return v

    st = {}

    def scores(i, g, hk):
        base = i * BQ
        qu = q_s[base // 2: (base + BQ) // 2, :]
        if g < i:
            st["s", i, g] = jax.lax.dot_general(hk.lhs(qu), _ld(k_s, g * BQ, (g + 1) * BQ), NT,
                                                preferred_element_type=f32)
            return
        q = _un(qu)
        tri = _iota((T, T), 1) <= _iota((T, T), 0)
        sd = []
        for t in range(NSUB):
            s = jax.lax.dot_general(q[t * T:, :], _ld(k_s, base + t * T, base + (t + 1) * T), NT,
                                    preferred_element_type=f32)
            top = jnp.where(tri, s[:T], NEG)
            sd.append(top if t == NSUB - 1 else jnp.concatenate([top, s[T:]], axis=0))
        st["s", i, i] = sd

    def group_tiles(i, g, r0):
        s = st["s", i, g]
        if g < i:
            return [s[r0:r0 + RC, cc * T:(cc + 1) * T] for cc in range(NSUB)]
        return [s[t][r0 - t * T: r0 - t * T + RC] for t in range(r0 // T + 1)]

    def tree(op, xs):
        while len(xs) > 1:
            xs = [op(xs[n], xs[n + 1]) if n + 1 < len(xs) else xs[n] for n in range(0, len(xs), 2)]
        return xs[0]

    chunks = list(range(0, BQ, RC))

    def partial_max_items(i, g, first):
        mel = st.setdefault(("mel", i), {})

        def one(r0):
            pm = tree(jnp.maximum, group_tiles(i, g, r0))
            mel[r0] = pm if first else jnp.maximum(mel[r0], pm)
            u = pltpu.bitcast(mel[r0], u32)
            return _zero_of(tree(jnp.bitwise_or, [u[n:n + 8] for n in range(0, RC, 8)]))

        return [(lambda r0=r0: one(r0)) for r0 in chunks]

    def row_max(i):
        mel = st.pop(("mel", i))
        st["m", i] = {r0: jnp.broadcast_to(jnp.max(mel[r0], axis=1, keepdims=True), (RC, T))
                      for r0 in chunks}

    def context(i, gate):
        base = i * BQ
        mb = st.pop(("m", i))
        lsum = {}
        acc = None
        deps = [] if gate is None else [gate] * DEP_LAG
        order = list(range(i + 1))
        if PV_DIAG_FIRST:
            order = order[-1:] + order[:-1]
        for n, g in enumerate(order):
            ps = {}
            for r0 in chunks:
                m = mb[r0]
                if len(deps) >= DEP_LAG:
                    m = jnp.concatenate([m[:8] + deps[-DEP_LAG], m[8:]], axis=0)
                p = [jnp.exp2(t - m) for t in group_tiles(i, g, r0)]
                part = tree(jnp.add, p)
                lsum[r0] = part if n == 0 else lsum[r0] + part
                deps.append(tree(jnp.add, [lsum[r0][q:q + 8] for q in range(0, RC, 8)]) * 0.0)
                ps[r0] = p
            if g < i:
                pg = jnp.concatenate([jnp.concatenate(ps[r0], axis=1) for r0 in chunks], axis=0)
                pv = jnp.dot(pg.astype(bf16), _ld(v_s, g * BQ, (g + 1) * BQ),
                             preferred_element_type=f32)
                acc = pv if acc is None else acc + pv
            else:
                parts = [None] * NSUB
                for t in range(NSUB):
                    pt = jnp.concatenate([ps[r0][t] for r0 in chunks if r0 >= t * T], axis=0)
                    pv = jnp.dot(pt.astype(bf16), _ld(v_s, base + t * T, base + (t + 1) * T),
                                 preferred_element_type=f32)
                    for r in range(t, NSUB):
                        piece = pv[(r - t) * T:(r - t + 1) * T]
                        parts[r] = piece if parts[r] is None else parts[r] + piece
                diag = jnp.concatenate(parts, axis=0)
                acc = diag if acc is None else acc + diag
            st.pop(("s", i, g))
        for r0 in chunks:
            l = jnp.sum(lsum[r0], axis=1, keepdims=True)
            inv = pl.reciprocal(l, approx=True)
            inv = inv * (2.0 - l * inv)
            ctx_s[h, (base + r0) // 2: (base + r0 + RC) // 2, :] = _pk(
                (acc[r0:r0 + RC] * inv).astype(bf16))

    def conv_forward_x(j, slot):
        pr = pl.ds(pl.multiple_of(j * (C // 2), C // 2), C // 2)
        r = pl.ds(pl.multiple_of(j * C, C), C)
        w = sh_ref[...].astype(f32)
        kc = _un(kb[slot]).astype(f32)
        ext = jnp.concatenate([khalo[...], kc], axis=0)
        ks = kc * w[0:1]
        for lag in range(1, KS):
            ks = ks + ext[8 - lag: 8 + C - lag] * w[lag:lag + 1]
        khalo[...] = kc[C - 8:]
        kvc = (ks * _un(vb[slot]).astype(f32)).astype(bf16)
        kv_s[pr, :] = _pk(kvc)
        xs = jnp.dot(fw_ref[...], kvc, preferred_element_type=f32)
        xf[j, 0] = xs[:, :HALF]
        xf[j, 1] = xs[:, HALF:]
        xg = _un(x_s[pr, :]).astype(f32) * gw_ref[...].astype(f32).reshape(1, M)
        g_s[r, :] = jax.nn.sigmoid(jnp.sum(xg, axis=1, keepdims=True))

    def conv_forward_k(j, slot):
        kn = jax.lax.dot_general(fw_ref[...], _un(skb[slot]), NT, preferred_element_type=f32)
        q4 = C // 2
        kp = kprev[...]
        kw = jnp.concatenate([
            kn[0:q4] - kp[2 * q4:3 * q4],
            kn[q4:2 * q4] + kp[3 * q4:4 * q4],
            kn[2 * q4:3 * q4] + kp[0:q4],
            kn[3 * q4:4 * q4] - kp[q4:2 * q4],
        ], axis=0)
        kprev[...] = kn
        kf[j, 0] = kw[:, :HALF]
        kf[j, 1] = kw[:, HALF:]

    def conv_block_items(n, group):
        half = n % 2
        re = pl.ds(pl.multiple_of((n // 2) * 16, 16), 16)
        im = pl.ds(pl.multiple_of(C + (n // 2) * 16, 16), 16)
        pre = pl.ds(pl.multiple_of((n // 2) * 8, 8), 8)
        pim = pl.ds(pl.multiple_of(C // 2 + (n // 2) * 8, 8), 8)

        acc = {}

        def some(lb, i, a0, a1):
            ln = slice(lb * T, (lb + 1) * T)
            yr, yi = acc.pop((lb, i), (None, None))
            for a in range(a0, a1):
                xr, xi = xf[i - a, half, re, ln], xf[i - a, half, im, ln]
                kr, ki = kf[a, half, re, ln], kf[a, half, im, ln]
                pr = xr * kr - xi * ki
                pi = xr * ki + xi * kr
                yr = pr if yr is None else yr + pr
                yi = pi if yi is None else yi + pi
            if a1 == i + 1:
                yr, yi = _pk(yr.astype(bf16)), _pk(yi.astype(bf16))
                yf[i, half, pre, ln] = yr
                yf[i, half, pim, ln] = yi
                return _zero_of(yr | yi)
            acc[lb, i] = (yr, yi)
            ur, ui = pltpu.bitcast(yr, u32), pltpu.bitcast(yi, u32)
            return _zero_of((ur[:8] | ur[8:]) | (ui[:8] | ui[8:]))

        return [(min(a0 + group, i + 1) - a0,
                 (lambda lb=lb, i=i, a0=a0: some(lb, i, a0, min(a0 + group, i + 1))))
                for lb in range(HALF // T) for i in range(NCH) for a0 in range(0, i + 1, group)]

    def conv_inverse(j):
        dvec = sd_ref[...].astype(f32).reshape(1, M)
        pr = pl.ds(pl.multiple_of(j * (C // 2), C // 2), C // 2)
        y = jnp.concatenate(
            [jnp.dot(iv_ref[...], _un(yf[j, hh]), preferred_element_type=f32)
             for hh in range(2)], axis=1)
        y = y + _un(kv_s[pr, :]).astype(f32) * dvec
        return _un(x_s[pr, :]).astype(f32) * y

    slot = h % 2

    @pl.when(h == 0)
    def _():
        first = w_copies(0, 1)
        for cp in first[1:]:
            cp.start()
        for i in range(NQ):
            block_copy(0, i).start()
        first[0].start()
        for i in range(NQ):
            block_copy(1, i).start()
        for cp in chunk_copies(0, 0) + small_copies():
            cp.start()
        kprev[...] = jnp.zeros(kprev.shape, f32)
        khalo[...] = jnp.zeros(khalo.shape, f32)
        for cp in first[1:]:
            cp.wait()
        unpack_weights(1, h * 0, (1, 2))

        def kv_body(i, carry):
            block_copy(0, i).wait()
            pr = pl.ds(pl.multiple_of(i * (BQ // 2), BQ // 2), BQ // 2)
            cc = _un(c_s[pr, :])
            k_s[pr, :] = _pk(jnp.dot(cc, _un(wk_s[...]), preferred_element_type=f32).astype(bf16))
            v_s[pr, :] = _pk(jnp.dot(cc, _un(wv_s[...]), preferred_element_type=f32).astype(bf16))
            return carry

        jax.lax.fori_loop(0, NQ, kv_body, 0)
        first[0].wait()
        unpack_weights(1, h * 0, (0,))
        for n, buf in enumerate((wqb, wkb, wvb)):
            pltpu.make_async_copy(buf.at[1], buf.at[0], w_sem.at[0, n]).start()

        def q_body(i, carry):
            block_copy(1, i).wait()
            pr = pl.ds(pl.multiple_of(i * (BQ // 2), BQ // 2), BQ // 2)
            q = jnp.dot(_un(x_s[pr, :]), _un(wq_s[...]), preferred_element_type=f32)
            q_s[pr, :] = _pk((q * QSCALE).astype(bf16))
            return carry

        jax.lax.fori_loop(0, NQ, q_body, 0)
        for cp in small_copies():
            cp.wait()
        wo_copy().start()

    def next_weights():
        for cp in w_copies((h + 1) // 2, slot):
            cp.wait()
        for cp in w_copies(jnp.minimum((h + 2) // 2, H // 2 - 1), 1 - slot):
            cp.start()
        unpack_weights(slot, (h + 1) % 2)

    HB = BQ // 2

    def head_step(fill, hk):
        def run(*names):
            gate = None
            for name in names:
                if name in fill:
                    res = fill[name](hk)
                    if res is not None and USE_GATE:
                        r = int(res.shape[0] * (GATE_Q if name[0] == 'Q' else GATE_K)) // 8 * 8
                        gate = pltpu.bitcast(_zero_of(res[r:r + 8]), f32)
            return gate

        def block(i, before, after):
            order = list(range(i + 1))
            if DIAG_FIRST:
                order = order[-1:] + order[:-1]
            for n, g in enumerate(order):
                scores(i, g, hk)
                hk.urgent += partial_max_items(i, g, n == 0)
            gate = run(*before)
            hk.flush_urgent()
            row_max(i)
            context(i, gate)
            run(*after)

        for i in range(NQ - 1, -1, -1):
            block(i, *FILL_ORDER[i])
        hk.flush()

    def proj_fill():
        fill = {}
        for i in range(NQ):
            fill["K%d" % i] = lambda hk, i=i: k_proj(i * BQ, (i + 1) * BQ, hk)
            fill["V%d" % i] = lambda hk, i=i: v_proj(i * BQ, (i + 1) * BQ, hk)
            fill["Q%da" % i] = lambda hk, i=i: q_proj(i * BQ, i * BQ + HB, hk)
            fill["Q%db" % i] = lambda hk, i=i: q_proj(i * BQ + HB, (i + 1) * BQ, hk)
        return fill

    @pl.when(h < NCH)
    def _():
        for cp in chunk_copies(h, slot):
            cp.wait()
        for cp in chunk_copies(jnp.minimum(h + 1, NCH - 1), 1 - slot):
            cp.start()
        next_weights()
        fill = proj_fill()
        fill["E0"] = lambda hk: conv_forward_x(h, slot)
        fill["E1"] = lambda hk: conv_forward_k(h, slot)
        head_step(fill, Hooks())

    @pl.when(jnp.logical_and(h >= NCH, h < H - 1))
    def _():
        next_weights()
        head_step(proj_fill(), Hooks(conv_block_items(h - NCH, GROUP), rate=0.8))

    @pl.when(h == H - 1)
    def _():
        for cp in w_copies(H // 2 - 1, slot) + chunk_copies(NCH - 1, NCH % 2):
            cp.wait()
        wo_copy().wait()
        head_step({}, Hooks(conv_block_items(NCH - 1, 4), rate=3.0))

    @pl.when(h >= H)
    def _():
        e = h - H
        pr = pl.ds(pl.multiple_of(e * (RE // 2), RE // 2), RE // 2)
        r = pl.ds(pl.multiple_of(e * RE, RE), RE)
        ctx = jnp.concatenate([_un(ctx_s[hh, pr, :]) for hh in range(H)], axis=1)
        b = jnp.concatenate([conv_inverse(e * (RE // C) + j) for j in range(RE // C)], axis=0)
        a = jnp.dot(ctx, _un(wo_s[...]), preferred_element_type=f32)
        g = g_s[r, :]
        o_ref[...] = (b + g * (a - b)).astype(o_ref.dtype)


@jax.jit
def pallas_gated_mix__compressed_kv_cla__ssm_conv_h3__prompt_kernel(
    A_x: jax.Array,
    A_c_kv: jax.Array,
    A_w_q: jax.Array,
    A_w_uk: jax.Array,
    A_w_uv: jax.Array,
    A_w_o: jax.Array,
    B_q: jax.Array,
    B_k: jax.Array,
    B_v: jax.Array,
    B_shift_k: jax.Array,
    B_ssm_k: jax.Array,
    B_ssm_D: jax.Array,
    gate_w: jax.Array,
):
    fwd, inv = _dft_matrices()
    fwd = jnp.asarray(fwd, bf16)
    inv = jnp.asarray(inv, bf16)

    in_specs = [pl.BlockSpec(memory_space=pl.ANY)] * 14
    scratch = [
        pltpu.VMEM((S // 2, M), u32),
        pltpu.VMEM((S // 2, DC), u32),
        pltpu.VMEM((H * D // 2, M), u32),
        pltpu.VMEM((S // 2, D), u32), pltpu.VMEM((S // 2, D), u32), pltpu.VMEM((S // 2, D), u32),
        pltpu.VMEM((H, S // 2, D), u32),
        pltpu.VMEM((2, M, D), u32), pltpu.VMEM((2, DC, D), u32), pltpu.VMEM((2, DC, D), u32),
        pltpu.VMEM((M // 2, D), u32), pltpu.VMEM((DC // 2, D), u32), pltpu.VMEM((DC // 2, D), u32),
        pltpu.VMEM((2, C // 2, M), u32), pltpu.VMEM((2, C // 2, M), u32),
        pltpu.VMEM((2, M // 2, C), u32),
        pltpu.VMEM((NCH, 2, 2 * C, HALF), f32),
        pltpu.VMEM((NCH, 2, 2 * C, HALF), f32),
        pltpu.VMEM((NCH, 2, C, HALF), u32),
        pltpu.VMEM((2 * C, M), f32),
        pltpu.VMEM((8, M), f32),
        pltpu.VMEM((S // 2, M), u32),
        pltpu.VMEM((S, 1), f32),
        pltpu.VMEM((KS, M), bf16), pltpu.VMEM((M,), bf16), pltpu.VMEM((M,), bf16),
        pltpu.VMEM((2 * C, C), bf16), pltpu.VMEM((C, 2 * C), bf16),
        pltpu.SemaphoreType.DMA((5,)),
        pltpu.SemaphoreType.DMA((2, NQ)),
        pltpu.SemaphoreType.DMA((1,)),
        pltpu.SemaphoreType.DMA((2, 3)),
        pltpu.SemaphoreType.DMA((2, 3)),
    ]
    return pl.pallas_call(
        _kernel,
        grid=(H + NE,),
        in_specs=in_specs,
        out_specs=pl.BlockSpec((None, RE, M), lambda h: (0, jnp.maximum(h - H, 0), 0)),
        out_shape=jax.ShapeDtypeStruct((1, S, M), bf16),
        scratch_shapes=scratch,
        compiler_params=pltpu.CompilerParams(
            dimension_semantics=("arbitrary",),
            vmem_limit_bytes=126 * 1024 * 1024,
        ),
        name="gated_mix_kernel",
    )(A_x, A_c_kv, A_w_q, A_w_uk, A_w_uv, A_w_o.reshape(H * D, M), B_k, B_v, B_ssm_k,
      B_shift_k.T, B_ssm_D, gate_w, fwd, inv)
```

```python
import math

import jax
import jax.numpy as jnp
import numpy as np
import jax.experimental.pallas as pl
import jax.experimental.pallas.tpu as pltpu

f32 = jnp.float32
bf16 = jnp.bfloat16
u32 = jnp.uint32

S = 2048
M = 1024
DC = 512
H = 32
D = 128
T = 128
BQ = 512
NQ = S // BQ
NSUB = BQ // T
RC = 32
DEP_LAG = 1
GROUP = 1
URGENT_EVERY = 1000
DIAG_FIRST = True
PV_DIAG_FIRST = True
FILL_ORDER = {
    3: (("K3", "Q3a"), ("V3",)),
    2: (("Q3b", "K2"), ("V2",)),
    1: (("Q2a", "Q2b"), ("V1",)),
    0: (("K1", "Q1a", "Q1b"), ("V0", "E0", "E1", "K0", "Q0a", "Q0b")),
}
USE_GATE = False
GATE_K = 0.5
GATE_Q = 0.05
C = 128
NCH = S // C
HALF = M // 2
KS = 4
RE = 256
NE = S // RE

QSCALE = (D ** -0.5) * math.log2(math.e)
NEG = -1e30
NT = (((1,), (1,)), ((), ()))


def _dft_matrices():
    freqs = np.concatenate([np.arange(0, C, 2), np.arange(1, C, 2)])
    t = np.arange(C)
    n = ((2 * freqs[:, None] + 1) * t[None, :]) % (4 * C)
    ang = np.pi * n / (2 * C)
    fwd = np.concatenate([np.cos(ang), -np.sin(ang)], axis=0)
    inv = fwd.T / C
    return fwd.astype(np.float32), inv.astype(np.float32)


def _iota(shape, dim):
    return jax.lax.broadcasted_iota(jnp.int32, shape, dim)


def _pk(v):
    return pltpu.bitcast(v, u32)


def _un(u):
    return pltpu.bitcast(u, bf16)


def _ld(ref, r0, r1, cols=slice(None)):
    return _un(ref[r0 // 2: r1 // 2, cols])


def _zero_of(t):
    return (pltpu.bitcast(t, u32) >> 31) & jnp.uint32(2)


class Hooks:
    def __init__(self, items=(), rate=1.0):
        self.items = list(items)
        self.urgent = []
        self.rate = rate
        self.credit = 0.0
        self.count = 0

    def take(self):
        zs = []
        self.count += 1
        if self.urgent and self.count % URGENT_EVERY == 0:
            zs.append(self.urgent.pop(0)())
        self.credit += self.rate
        if self.items and self.items[0][0] <= self.credit:
            cost, thunk = self.items.pop(0)
            self.credit -= cost
            zs.append(thunk())
        if not zs:
            return None
        return zs[0] if len(zs) == 1 else zs[0] | zs[1]

    def flush_urgent(self):
        for thunk in self.urgent:
            thunk()
        self.urgent = []

    def flush(self):
        self.flush_urgent()
        for _, thunk in self.items:
            thunk()
        self.items = []

    def lhs(self, u, tiles=(0,)):
        nrow = u.shape[0] // 8
        cols = [u[:, t * T:(t + 1) * T] for t in range(u.shape[1] // T)]
        for t in tiles:
            parts, start = [], 0
            for r in range(nrow):
                z = self.take()
                if z is not None:
                    if r * 8 > start:
                        parts.append(cols[t][start:r * 8])
                    parts.append(cols[t][r * 8:(r + 1) * 8] | z)
                    start = (r + 1) * 8
            if start < nrow * 8:
                parts.append(cols[t][start:])
            cols[t] = parts[0] if len(parts) == 1 else jnp.concatenate(parts, axis=0)
        return _un(cols[0] if len(cols) == 1 else jnp.concatenate(cols, axis=1))


def _kernel(x_hbm, c_hbm, wq_hbm, wk_hbm, wv_hbm, wo_hbm, k_hbm, v_hbm, sk_hbm,
            sh_hbm, sd_hbm, gw_hbm, fw_hbm, iv_hbm, o_hbm,
            o_s, o_sem, x_s, c_s, wo_s, q_s, k_s, v_s, ctx_s, wqb, wkb, wvb, wq_s, wk_s, wv_s,
            kb, vb, skb, xf, kf, yf, kprev, khalo, kv_s, g_s,
            sh_ref, sd_ref, gw_ref, fw_ref, iv_ref, small_sem, big_sem, wo_sem, w_sem, ch_sem):
    cur = {}

    def block_copy(n, i):
        src, dst = ((c_hbm, c_s), (x_hbm, x_s))[n]
        rows = pl.ds(pl.multiple_of(i * (BQ // 2), BQ // 2), BQ // 2)
        return pltpu.make_async_copy(src.at[0].bitcast(u32).at[rows, :], dst.at[rows, :],
                                     big_sem.at[n, i])

    def small_copies():
        pairs = ((sh_hbm, sh_ref), (sd_hbm, sd_ref), (gw_hbm, gw_ref), (fw_hbm, fw_ref),
                 (iv_hbm, iv_ref))
        return [pltpu.make_async_copy(src, dst, small_sem.at[n])
                for n, (src, dst) in enumerate(pairs)]

    def wo_copy():
        return pltpu.make_async_copy(wo_hbm.bitcast(u32), wo_s, wo_sem.at[0])

    def w_copies(pair, slot):
        return [
            pltpu.make_async_copy(src.bitcast(u32).at[:, pair, :], dst.at[slot], w_sem.at[slot, n])
            for n, (src, dst) in enumerate(((wq_hbm, wqb), (wk_hbm, wkb), (wv_hbm, wvb)))
        ]

    def chunk_copies(j, slot):
        rows = pl.ds(pl.multiple_of(j * (C // 2), C // 2), C // 2)
        cols = pl.ds(pl.multiple_of(j * C, C), C)
        return [
            pltpu.make_async_copy(k_hbm.at[0].bitcast(u32).at[rows, :], kb.at[slot], ch_sem.at[slot, 0]),
            pltpu.make_async_copy(v_hbm.at[0].bitcast(u32).at[rows, :], vb.at[slot], ch_sem.at[slot, 1]),
            pltpu.make_async_copy(sk_hbm.bitcast(u32).at[:, cols], skb.at[slot], ch_sem.at[slot, 2]),
        ]

    def unpack_weights(slot, parity, which=(0, 1, 2)):
        sh = jnp.asarray(16 * (1 - parity)).astype(u32)
        for n in which:
            src, dst = ((wqb, wq_s), (wkb, wk_s), (wvb, wv_s))[n]
            u = (src[slot] << sh) & jnp.uint32(0xFFFF0000)
            dst[...] = _pk(pltpu.bitcast(u, f32).astype(bf16))

    def q_proj(r0, r1, hk):
        lhs = hk.lhs(x_s[r0 // 2: r1 // 2, :], (0, 4))
        q = jnp.dot(lhs, _un(wq_s[...]), preferred_element_type=f32)
        q_s[r0 // 2: r1 // 2, :] = _pk((q * QSCALE).astype(bf16))
        return q

    def k_proj(r0, r1, hk):
        lhs = hk.lhs(c_s[r0 // 2: r1 // 2, :])
        k = jnp.dot(lhs, _un(wk_s[...]), preferred_element_type=f32)
        k_s[r0 // 2: r1 // 2, :] = _pk(k.astype(bf16))
        return k

    def v_proj(r0, r1, hk):
        lhs = hk.lhs(c_s[r0 // 2: r1 // 2, :])
        v = jnp.dot(lhs, _un(wv_s[...]), preferred_element_type=f32)
        v_s[r0 // 2: r1 // 2, :] = _pk(v.astype(bf16))
        return v

    st = {}

    def scores(i, g, hk):
        base = i * BQ
        qu = q_s[base // 2: (base + BQ) // 2, :]
        if g < i:
            st["s", i, g] = jax.lax.dot_general(hk.lhs(qu), _ld(k_s, g * BQ, (g + 1) * BQ), NT,
                                                preferred_element_type=f32)
            return
        q = _un(qu)
        tri = _iota((T, T), 1) <= _iota((T, T), 0)
        sd = []
        for t in range(NSUB):
            s = jax.lax.dot_general(q[t * T:, :], _ld(k_s, base + t * T, base + (t + 1) * T), NT,
                                    preferred_element_type=f32)
            top = jnp.where(tri, s[:T], NEG)
            sd.append(top if t == NSUB - 1 else jnp.concatenate([top, s[T:]], axis=0))
        st["s", i, i] = sd

    def group_tiles(i, g, r0):
        s = st["s", i, g]
        if g < i:
            return [s[r0:r0 + RC, cc * T:(cc + 1) * T] for cc in range(NSUB)]
        return [s[t][r0 - t * T: r0 - t * T + RC] for t in range(r0 // T + 1)]

    def tree(op, xs):
        while len(xs) > 1:
            xs = [op(xs[n], xs[n + 1]) if n + 1 < len(xs) else xs[n] for n in range(0, len(xs), 2)]
        return xs[0]

    chunks = list(range(0, BQ, RC))

    def partial_max_items(i, g, first):
        mel = st.setdefault(("mel", i), {})

        def one(r0):
            pm = tree(jnp.maximum, group_tiles(i, g, r0))
            mel[r0] = pm if first else jnp.maximum(mel[r0], pm)
            u = pltpu.bitcast(mel[r0], u32)
            return _zero_of(tree(jnp.bitwise_or, [u[n:n + 8] for n in range(0, RC, 8)]))

        return [(lambda r0=r0: one(r0)) for r0 in chunks]

    def row_max(i):
        mel = st.pop(("mel", i))
        st["m", i] = {r0: jnp.broadcast_to(jnp.max(mel[r0], axis=1, keepdims=True), (RC, T))
                      for r0 in chunks}

    def context(i, gate):
        base = i * BQ
        mb = st.pop(("m", i))
        lsum = {}
        acc = None
        deps = [] if gate is None else [gate] * DEP_LAG
        order = list(range(i + 1))
        if PV_DIAG_FIRST:
            order = order[-1:] + order[:-1]
        for n, g in enumerate(order):
            ps = {}
            for r0 in chunks:
                m = mb[r0]
                if len(deps) >= DEP_LAG:
                    m = jnp.concatenate([m[:8] + deps[-DEP_LAG], m[8:]], axis=0)
                p = [jnp.exp2(t - m) for t in group_tiles(i, g, r0)]
                part = tree(jnp.add, p)
                lsum[r0] = part if n == 0 else lsum[r0] + part
                deps.append(tree(jnp.add, [lsum[r0][q:q + 8] for q in range(0, RC, 8)]) * 0.0)
                ps[r0] = p
            if g < i:
                pg = jnp.concatenate([jnp.concatenate(ps[r0], axis=1) for r0 in chunks], axis=0)
                pv = jnp.dot(pg.astype(bf16), _ld(v_s, g * BQ, (g + 1) * BQ),
                             preferred_element_type=f32)
                acc = pv if acc is None else acc + pv
            else:
                parts = [None] * NSUB
                for t in range(NSUB):
                    pt = jnp.concatenate([ps[r0][t] for r0 in chunks if r0 >= t * T], axis=0)
                    pv = jnp.dot(pt.astype(bf16), _ld(v_s, base + t * T, base + (t + 1) * T),
                                 preferred_element_type=f32)
                    for r in range(t, NSUB):
                        piece = pv[(r - t) * T:(r - t + 1) * T]
                        parts[r] = piece if parts[r] is None else parts[r] + piece
                diag = jnp.concatenate(parts, axis=0)
                acc = diag if acc is None else acc + diag
            st.pop(("s", i, g))
        for r0 in chunks:
            l = jnp.sum(lsum[r0], axis=1, keepdims=True)
            inv = pl.reciprocal(l, approx=True)
            inv = inv * (2.0 - l * inv)
            ctx_s[cur["h"], (base + r0) // 2: (base + r0 + RC) // 2, :] = _pk(
                (acc[r0:r0 + RC] * inv).astype(bf16))

    def conv_forward_x(j, slot):
        pr = pl.ds(pl.multiple_of(j * (C // 2), C // 2), C // 2)
        r = pl.ds(pl.multiple_of(j * C, C), C)
        w = sh_ref[...].astype(f32)
        kc = _un(kb[slot]).astype(f32)
        ext = jnp.concatenate([khalo[...], kc], axis=0)
        ks = kc * w[0:1]
        for lag in range(1, KS):
            ks = ks + ext[8 - lag: 8 + C - lag] * w[lag:lag + 1]
        khalo[...] = kc[C - 8:]
        kvc = (ks * _un(vb[slot]).astype(f32)).astype(bf16)
        kv_s[pr, :] = _pk(kvc)
        xs = jnp.dot(fw_ref[...], kvc, preferred_element_type=f32)
        xf[j, 0] = xs[:, :HALF]
        xf[j, 1] = xs[:, HALF:]
        xg = _un(x_s[pr, :]).astype(f32) * gw_ref[...].astype(f32).reshape(1, M)
        g_s[r, :] = jax.nn.sigmoid(jnp.sum(xg, axis=1, keepdims=True))

    def conv_forward_k(j, slot):
        kn = jax.lax.dot_general(fw_ref[...], _un(skb[slot]), NT, preferred_element_type=f32)
        q4 = C // 2
        kp = kprev[...]
        kw = jnp.concatenate([
            kn[0:q4] - kp[2 * q4:3 * q4],
            kn[q4:2 * q4] + kp[3 * q4:4 * q4],
            kn[2 * q4:3 * q4] + kp[0:q4],
            kn[3 * q4:4 * q4] - kp[q4:2 * q4],
        ], axis=0)
        kprev[...] = kn
        kf[j, 0] = kw[:, :HALF]
        kf[j, 1] = kw[:, HALF:]

    def conv_block_items(n, group):
        half = n % 2
        re = pl.ds(pl.multiple_of((n // 2) * 16, 16), 16)
        im = pl.ds(pl.multiple_of(C + (n // 2) * 16, 16), 16)
        pre = pl.ds(pl.multiple_of((n // 2) * 8, 8), 8)
        pim = pl.ds(pl.multiple_of(C // 2 + (n // 2) * 8, 8), 8)

        acc = {}

        def some(lb, i, a0, a1):
            ln = slice(lb * T, (lb + 1) * T)
            yr, yi = acc.pop((lb, i), (None, None))
            for a in range(a0, a1):
                xr, xi = xf[i - a, half, re, ln], xf[i - a, half, im, ln]
                kr, ki = kf[a, half, re, ln], kf[a, half, im, ln]
                pr = xr * kr - xi * ki
                pi = xr * ki + xi * kr
                yr = pr if yr is None else yr + pr
                yi = pi if yi is None else yi + pi
            if a1 == i + 1:
                yr, yi = _pk(yr.astype(bf16)), _pk(yi.astype(bf16))
                yf[i, half, pre, ln] = yr
                yf[i, half, pim, ln] = yi
                return _zero_of(yr | yi)
            acc[lb, i] = (yr, yi)
            ur, ui = pltpu.bitcast(yr, u32), pltpu.bitcast(yi, u32)
            return _zero_of((ur[:8] | ur[8:]) | (ui[:8] | ui[8:]))

        return [(min(a0 + group, i + 1) - a0,
                 (lambda lb=lb, i=i, a0=a0: some(lb, i, a0, min(a0 + group, i + 1))))
                for lb in range(HALF // T) for i in range(NCH) for a0 in range(0, i + 1, group)]

    def conv_inverse(j):
        dvec = sd_ref[...].astype(f32).reshape(1, M)
        pr = pl.ds(pl.multiple_of(j * (C // 2), C // 2), C // 2)
        y = jnp.concatenate(
            [jnp.dot(iv_ref[...], _un(yf[j, hh]), preferred_element_type=f32)
             for hh in range(2)], axis=1)
        y = y + _un(kv_s[pr, :]).astype(f32) * dvec
        return _un(x_s[pr, :]).astype(f32) * y

    def prologue():
        first = w_copies(0, 1)
        for cp in first[1:]:
            cp.start()
        for i in range(NQ):
            block_copy(0, i).start()
        first[0].start()
        for i in range(NQ):
            block_copy(1, i).start()
        for cp in chunk_copies(0, 0) + small_copies():
            cp.start()
        kprev[...] = jnp.zeros(kprev.shape, f32)
        khalo[...] = jnp.zeros(khalo.shape, f32)
        for cp in first[1:]:
            cp.wait()
        unpack_weights(1, 0, (1, 2))

        def kv_body(i, carry):
            block_copy(0, i).wait()
            pr = pl.ds(pl.multiple_of(i * (BQ // 2), BQ // 2), BQ // 2)
            cc = _un(c_s[pr, :])
            k_s[pr, :] = _pk(jnp.dot(cc, _un(wk_s[...]), preferred_element_type=f32).astype(bf16))
            v_s[pr, :] = _pk(jnp.dot(cc, _un(wv_s[...]), preferred_element_type=f32).astype(bf16))
            return carry

        jax.lax.fori_loop(0, NQ, kv_body, 0)
        first[0].wait()
        unpack_weights(1, 0, (0,))
        for n, buf in enumerate((wqb, wkb, wvb)):
            pltpu.make_async_copy(buf.at[1], buf.at[0], w_sem.at[0, n]).start()

        def q_body(i, carry):
            block_copy(1, i).wait()
            pr = pl.ds(pl.multiple_of(i * (BQ // 2), BQ // 2), BQ // 2)
            q = jnp.dot(_un(x_s[pr, :]), _un(wq_s[...]), preferred_element_type=f32)
            q_s[pr, :] = _pk((q * QSCALE).astype(bf16))
            return carry

        jax.lax.fori_loop(0, NQ, q_body, 0)
        for cp in small_copies():
            cp.wait()
        wo_copy().start()

    def next_weights(h):
        slot = h % 2
        for cp in w_copies((h + 1) // 2, slot):
            cp.wait()
        for cp in w_copies(jnp.minimum((h + 2) // 2, H // 2 - 1), 1 - slot):
            cp.start()
        unpack_weights(slot, (h + 1) % 2)

    HB = BQ // 2

    def head_step(fill, hk):
        def run(*names):
            gate = None
            for name in names:
                if name in fill:
                    res = fill[name](hk)
                    if res is not None and USE_GATE:
                        r = int(res.shape[0] * (GATE_Q if name[0] == 'Q' else GATE_K)) // 8 * 8
                        gate = pltpu.bitcast(_zero_of(res[r:r + 8]), f32)
            return gate

        def block(i, before, after):
            order = list(range(i + 1))
            if DIAG_FIRST:
                order = order[-1:] + order[:-1]
            for n, g in enumerate(order):
                scores(i, g, hk)
                hk.urgent += partial_max_items(i, g, n == 0)
            gate = run(*before)
            hk.flush_urgent()
            row_max(i)
            context(i, gate)
            run(*after)

        for i in range(NQ - 1, -1, -1):
            block(i, *FILL_ORDER[i])
        hk.flush()

    def proj_fill():
        fill = {}
        for i in range(NQ):
            fill["K%d" % i] = lambda hk, i=i: k_proj(i * BQ, (i + 1) * BQ, hk)
            fill["V%d" % i] = lambda hk, i=i: v_proj(i * BQ, (i + 1) * BQ, hk)
            fill["Q%da" % i] = lambda hk, i=i: q_proj(i * BQ, i * BQ + HB, hk)
            fill["Q%db" % i] = lambda hk, i=i: q_proj(i * BQ + HB, (i + 1) * BQ, hk)
        return fill

    def forward_step(h, carry):
        cur["h"] = h
        slot = h % 2
        for cp in chunk_copies(h, slot):
            cp.wait()
        for cp in chunk_copies(jnp.minimum(h + 1, NCH - 1), 1 - slot):
            cp.start()
        next_weights(h)
        fill = proj_fill()
        fill["E0"] = lambda hk: conv_forward_x(h, slot)
        fill["E1"] = lambda hk: conv_forward_k(h, slot)
        head_step(fill, Hooks())
        return carry

    def product_step(h, carry):
        cur["h"] = h
        next_weights(h)
        head_step(proj_fill(), Hooks(conv_block_items(h - NCH, GROUP), rate=0.8))
        return carry

    def last_step():
        cur["h"] = H - 1
        for cp in w_copies(H // 2 - 1, (H - 1) % 2) + chunk_copies(NCH - 1, NCH % 2):
            cp.wait()
        wo_copy().wait()
        head_step({}, Hooks(conv_block_items(NCH - 1, 4), rate=3.0))

    def out_copy(e):
        r = pl.ds(pl.multiple_of(e * RE, RE), RE)
        return pltpu.make_async_copy(o_s.at[r, :], o_hbm.at[0, r, :], o_sem.at[e])

    def output_step(e, carry):
        pr = pl.ds(pl.multiple_of(e * (RE // 2), RE // 2), RE // 2)
        r = pl.ds(pl.multiple_of(e * RE, RE), RE)
        ctx = jnp.concatenate([_un(ctx_s[hh, pr, :]) for hh in range(H)], axis=1)
        b = jnp.concatenate([conv_inverse(e * (RE // C) + j) for j in range(RE // C)], axis=0)
        a = jnp.dot(ctx, _un(wo_s[...]), preferred_element_type=f32)
        g = g_s[r, :]
        o_s[r, :] = (b + g * (a - b)).astype(bf16)
        out_copy(e).start()
        return carry

    prologue()
    jax.lax.fori_loop(0, NCH, forward_step, 0)
    jax.lax.fori_loop(NCH, H - 1, product_step, 0)
    last_step()
    jax.lax.fori_loop(0, NE, output_step, 0)
    for e in range(NE):
        out_copy(e).wait()


@jax.jit
def pallas_gated_mix__compressed_kv_cla__ssm_conv_h3__prompt_kernel(
    A_x: jax.Array,
    A_c_kv: jax.Array,
    A_w_q: jax.Array,
    A_w_uk: jax.Array,
    A_w_uv: jax.Array,
    A_w_o: jax.Array,
    B_q: jax.Array,
    B_k: jax.Array,
    B_v: jax.Array,
    B_shift_k: jax.Array,
    B_ssm_k: jax.Array,
    B_ssm_D: jax.Array,
    gate_w: jax.Array,
):
    fwd, inv = _dft_matrices()
    fwd = jnp.asarray(fwd, bf16)
    inv = jnp.asarray(inv, bf16)

    in_specs = [pl.BlockSpec(memory_space=pl.ANY)] * 14
    scratch = [
        pltpu.VMEM((S, M), bf16),
        pltpu.SemaphoreType.DMA((NE,)),
        pltpu.VMEM((S // 2, M), u32),
        pltpu.VMEM((S // 2, DC), u32),
        pltpu.VMEM((H * D // 2, M), u32),
        pltpu.VMEM((S // 2, D), u32), pltpu.VMEM((S // 2, D), u32), pltpu.VMEM((S // 2, D), u32),
        pltpu.VMEM((H, S // 2, D), u32),
        pltpu.VMEM((2, M, D), u32), pltpu.VMEM((2, DC, D), u32), pltpu.VMEM((2, DC, D), u32),
        pltpu.VMEM((M // 2, D), u32), pltpu.VMEM((DC // 2, D), u32), pltpu.VMEM((DC // 2, D), u32),
        pltpu.VMEM((2, C // 2, M), u32), pltpu.VMEM((2, C // 2, M), u32),
        pltpu.VMEM((2, M // 2, C), u32),
        pltpu.VMEM((NCH, 2, 2 * C, HALF), f32),
        pltpu.VMEM((NCH, 2, 2 * C, HALF), f32),
        pltpu.VMEM((NCH, 2, C, HALF), u32),
        pltpu.VMEM((2 * C, M), f32),
        pltpu.VMEM((8, M), f32),
        pltpu.VMEM((S // 2, M), u32),
        pltpu.VMEM((S, 1), f32),
        pltpu.VMEM((KS, M), bf16), pltpu.VMEM((M,), bf16), pltpu.VMEM((M,), bf16),
        pltpu.VMEM((2 * C, C), bf16), pltpu.VMEM((C, 2 * C), bf16),
        pltpu.SemaphoreType.DMA((5,)),
        pltpu.SemaphoreType.DMA((2, NQ)),
        pltpu.SemaphoreType.DMA((1,)),
        pltpu.SemaphoreType.DMA((2, 3)),
        pltpu.SemaphoreType.DMA((2, 3)),
    ]
    return pl.pallas_call(
        _kernel,
        in_specs=in_specs,
        out_specs=pl.BlockSpec(memory_space=pl.ANY),
        out_shape=jax.ShapeDtypeStruct((1, S, M), bf16),
        scratch_shapes=scratch,
        compiler_params=pltpu.CompilerParams(
            vmem_limit_bytes=126 * 1024 * 1024,
        ),
        name="gated_mix_kernel",
    )(A_x, A_c_kv, A_w_q, A_w_uk, A_w_uv, A_w_o.reshape(H * D, M), B_k, B_v, B_ssm_k,
      B_shift_k.T, B_ssm_D, gate_w, fwd, inv)
```

```python
import math

import jax
import jax.numpy as jnp
import numpy as np
import jax.experimental.pallas as pl
import jax.experimental.pallas.tpu as pltpu

f32 = jnp.float32
bf16 = jnp.bfloat16
u32 = jnp.uint32

S = 2048
M = 1024
DC = 512
H = 32
D = 128
T = 128
BQ = 512
NQ = S // BQ
NSUB = BQ // T
NX = 8
RC = 32
DEP_LAG = 1
GROUP = 1
URGENT_EVERY = 1000
DIAG_FIRST = True
PV_DIAG_FIRST = True
FILL_ORDER = {
    3: (("K3", "Q3a"), ("V3",)),
    2: (("Q3b", "K2"), ("V2",)),
    1: (("Q2a", "Q2b"), ("V1",)),
    0: (("K1", "Q1a", "Q1b"), ("V0", "E0", "E1", "K0", "Q0a", "Q0b")),
}
USE_GATE = False
GATE_K = 0.5
GATE_Q = 0.05
C = 128
NCH = S // C
HALF = M // 2
KS = 4
RE = 256
NE = S // RE

QSCALE = (D ** -0.5) * math.log2(math.e)
NEG = -1e30
NT = (((1,), (1,)), ((), ()))


def _dft_matrices():
    freqs = np.concatenate([np.arange(0, C, 2), np.arange(1, C, 2)])
    t = np.arange(C)
    n = ((2 * freqs[:, None] + 1) * t[None, :]) % (4 * C)
    ang = np.pi * n / (2 * C)
    fwd = np.concatenate([np.cos(ang), -np.sin(ang)], axis=0)
    inv = fwd.T / C
    return fwd.astype(np.float32), inv.astype(np.float32)


def _iota(shape, dim):
    return jax.lax.broadcasted_iota(jnp.int32, shape, dim)


def _pk(v):
    return pltpu.bitcast(v, u32)


def _un(u):
    return pltpu.bitcast(u, bf16)


def _ld(ref, r0, r1, cols=slice(None)):
    return _un(ref[r0 // 2: r1 // 2, cols])


def _zero_of(t):
    return (pltpu.bitcast(t, u32) >> 31) & jnp.uint32(2)


class Hooks:
    def __init__(self, items=(), rate=1.0):
        self.items = list(items)
        self.urgent = []
        self.rate = rate
        self.credit = 0.0
        self.count = 0

    def take(self):
        zs = []
        self.count += 1
        if self.urgent and self.count % URGENT_EVERY == 0:
            zs.append(self.urgent.pop(0)())
        self.credit += self.rate
        if self.items and self.items[0][0] <= self.credit:
            cost, thunk = self.items.pop(0)
            self.credit -= cost
            zs.append(thunk())
        if not zs:
            return None
        return zs[0] if len(zs) == 1 else zs[0] | zs[1]

    def flush_urgent(self):
        for thunk in self.urgent:
            thunk()
        self.urgent = []

    def flush(self):
        self.flush_urgent()
        for _, thunk in self.items:
            thunk()
        self.items = []

    def lhs(self, u, tiles=(0,)):
        nrow = u.shape[0] // 8
        cols = [u[:, t * T:(t + 1) * T] for t in range(u.shape[1] // T)]
        for t in tiles:
            parts, start = [], 0
            for r in range(nrow):
                z = self.take()
                if z is not None:
                    if r * 8 > start:
                        parts.append(cols[t][start:r * 8])
                    parts.append(cols[t][r * 8:(r + 1) * 8] | z)
                    start = (r + 1) * 8
            if start < nrow * 8:
                parts.append(cols[t][start:])
            cols[t] = parts[0] if len(parts) == 1 else jnp.concatenate(parts, axis=0)
        return _un(cols[0] if len(cols) == 1 else jnp.concatenate(cols, axis=1))


def _kernel(x_hbm, c_hbm, wq_hbm, wk_hbm, wv_hbm, wo_hbm, k_hbm, v_hbm, sk_hbm,
            sh_hbm, sd_hbm, gw_hbm, fw_hbm, iv_hbm, o_hbm,
            o_s, o_sem, x_s, c_s, wo_s, q_s, k_s, v_s, ctx_s, wqb, wkb, wvb, wq_s, wk_s, wv_s,
            kb, vb, skb, xf, kf, yf, kprev, khalo, kv_s, g_s,
            sh_ref, sd_ref, gw_ref, fw_ref, iv_ref, small_sem, big_sem, wo_sem, w_sem, ch_sem):
    cur = {}

    def block_copy(n, i):
        src, dst = ((c_hbm, c_s), (x_hbm, x_s))[n]
        size = S // 2 // (NQ, NX)[n]
        rows = pl.ds(pl.multiple_of(i * size, size), size)
        return pltpu.make_async_copy(src.at[0].bitcast(u32).at[rows, :], dst.at[rows, :],
                                     big_sem.at[n, i])

    def small_copies():
        pairs = ((sh_hbm, sh_ref), (sd_hbm, sd_ref), (gw_hbm, gw_ref), (fw_hbm, fw_ref),
                 (iv_hbm, iv_ref))
        return [pltpu.make_async_copy(src, dst, small_sem.at[n])
                for n, (src, dst) in enumerate(pairs)]

    def wo_copy():
        return pltpu.make_async_copy(wo_hbm.bitcast(u32), wo_s, wo_sem.at[0])

    def w_copies(pair, slot):
        return [
            pltpu.make_async_copy(src.bitcast(u32).at[:, pair, :], dst.at[slot], w_sem.at[slot, n])
            for n, (src, dst) in enumerate(((wq_hbm, wqb), (wk_hbm, wkb), (wv_hbm, wvb)))
        ]

    def chunk_copies(j, slot):
        rows = pl.ds(pl.multiple_of(j * (C // 2), C // 2), C // 2)
        cols = pl.ds(pl.multiple_of(j * C, C), C)
        return [
            pltpu.make_async_copy(k_hbm.at[0].bitcast(u32).at[rows, :], kb.at[slot], ch_sem.at[slot, 0]),
            pltpu.make_async_copy(v_hbm.at[0].bitcast(u32).at[rows, :], vb.at[slot], ch_sem.at[slot, 1]),
            pltpu.make_async_copy(sk_hbm.bitcast(u32).at[:, cols], skb.at[slot], ch_sem.at[slot, 2]),
        ]

    def unpack_weights(slot, parity, which=(0, 1, 2)):
        sh = jnp.asarray(16 * (1 - parity)).astype(u32)
        for n in which:
            src, dst = ((wqb, wq_s), (wkb, wk_s), (wvb, wv_s))[n]
            u = (src[slot] << sh) & jnp.uint32(0xFFFF0000)
            dst[...] = _pk(pltpu.bitcast(u, f32).astype(bf16))

    def q_proj(r0, r1, hk):
        lhs = hk.lhs(x_s[r0 // 2: r1 // 2, :], (0, 4))
        q = jnp.dot(lhs, _un(wq_s[...]), preferred_element_type=f32)
        q_s[r0 // 2: r1 // 2, :] = _pk((q * QSCALE).astype(bf16))
        return q

    def k_proj(r0, r1, hk):
        lhs = hk.lhs(c_s[r0 // 2: r1 // 2, :])
        k = jnp.dot(lhs, _un(wk_s[...]), preferred_element_type=f32)
        k_s[r0 // 2: r1 // 2, :] = _pk(k.astype(bf16))
        return k

    def v_proj(r0, r1, hk):
        lhs = hk.lhs(c_s[r0 // 2: r1 // 2, :])
        v = jnp.dot(lhs, _un(wv_s[...]), preferred_element_type=f32)
        v_s[r0 // 2: r1 // 2, :] = _pk(v.astype(bf16))
        return v

    st = {}

    def scores(i, g, hk):
        base = i * BQ
        qu = q_s[base // 2: (base + BQ) // 2, :]
        if g < i:
            st["s", i, g] = jax.lax.dot_general(hk.lhs(qu), _ld(k_s, g * BQ, (g + 1) * BQ), NT,
                                                preferred_element_type=f32)
            return
        q = _un(qu)
        tri = _iota((T, T), 1) <= _iota((T, T), 0)
        sd = []
        for t in range(NSUB):
            s = jax.lax.dot_general(q[t * T:, :], _ld(k_s, base + t * T, base + (t + 1) * T), NT,
                                    preferred_element_type=f32)
            top = jnp.where(tri, s[:T], NEG)
            sd.append(top if t == NSUB - 1 else jnp.concatenate([top, s[T:]], axis=0))
        st["s", i, i] = sd

    def group_tiles(i, g, r0):
        s = st["s", i, g]
        if g < i:
            return [s[r0:r0 + RC, cc * T:(cc + 1) * T] for cc in range(NSUB)]
        return [s[t][r0 - t * T: r0 - t * T + RC] for t in range(r0 // T + 1)]

    def tree(op, xs):
        while len(xs) > 1:
            xs = [op(xs[n], xs[n + 1]) if n + 1 < len(xs) else xs[n] for n in range(0, len(xs), 2)]
        return xs[0]

    chunks = list(range(0, BQ, RC))

    def partial_max_items(i, g, first):
        mel = st.setdefault(("mel", i), {})

        def one(r0):
            pm = tree(jnp.maximum, group_tiles(i, g, r0))
            mel[r0] = pm if first else jnp.maximum(mel[r0], pm)
            u = pltpu.bitcast(mel[r0], u32)
            return _zero_of(tree(jnp.bitwise_or, [u[n:n + 8] for n in range(0, RC, 8)]))

        return [(lambda r0=r0: one(r0)) for r0 in chunks]

    def row_max(i):
        mel = st.pop(("mel", i))
        st["m", i] = {r0: jnp.broadcast_to(jnp.max(mel[r0], axis=1, keepdims=True), (RC, T))
                      for r0 in chunks}

    def context(i, gate):
        base = i * BQ
        mb = st.pop(("m", i))
        lsum = {}
        acc = None
        deps = [] if gate is None else [gate] * DEP_LAG
        order = list(range(i + 1))
        if PV_DIAG_FIRST:
            order = order[-1:] + order[:-1]
        for n, g in enumerate(order):
            ps = {}
            for r0 in chunks:
                m = mb[r0]
                if len(deps) >= DEP_LAG:
                    m = jnp.concatenate([m[:8] + deps[-DEP_LAG], m[8:]], axis=0)
                p = [jnp.exp2(t - m) for t in group_tiles(i, g, r0)]
                part = tree(jnp.add, p)
                lsum[r0] = part if n == 0 else lsum[r0] + part
                deps.append(tree(jnp.add, [lsum[r0][q:q + 8] for q in range(0, RC, 8)]) * 0.0)
                ps[r0] = p
            if g < i:
                pg = jnp.concatenate([jnp.concatenate(ps[r0], axis=1) for r0 in chunks], axis=0)
                pv = jnp.dot(pg.astype(bf16), _ld(v_s, g * BQ, (g + 1) * BQ),
                             preferred_element_type=f32)
                acc = pv if acc is None else acc + pv
            else:
                parts = [None] * NSUB
                for t in range(NSUB):
                    pt = jnp.concatenate([ps[r0][t] for r0 in chunks if r0 >= t * T], axis=0)
                    pv = jnp.dot(pt.astype(bf16), _ld(v_s, base + t * T, base + (t + 1) * T),
                                 preferred_element_type=f32)
                    for r in range(t, NSUB):
                        piece = pv[(r - t) * T:(r - t + 1) * T]
                        parts[r] = piece if parts[r] is None else parts[r] + piece
                diag = jnp.concatenate(parts, axis=0)
                acc = diag if acc is None else acc + diag
            st.pop(("s", i, g))
        for r0 in chunks:
            l = jnp.sum(lsum[r0], axis=1, keepdims=True)
            inv = pl.reciprocal(l, approx=True)
            inv = inv * (2.0 - l * inv)
            ctx_s[cur["h"], (base + r0) // 2: (base + r0 + RC) // 2, :] = _pk(
                (acc[r0:r0 + RC] * inv).astype(bf16))

    def conv_forward_x(j, slot):
        pr = pl.ds(pl.multiple_of(j * (C // 2), C // 2), C // 2)
        r = pl.ds(pl.multiple_of(j * C, C), C)
        w = sh_ref[...].astype(f32)
        kc = _un(kb[slot]).astype(f32)
        ext = jnp.concatenate([khalo[...], kc], axis=0)
        ks = kc * w[0:1]
        for lag in range(1, KS):
            ks = ks + ext[8 - lag: 8 + C - lag] * w[lag:lag + 1]
        khalo[...] = kc[C - 8:]
        kvc = (ks * _un(vb[slot]).astype(f32)).astype(bf16)
        kv_s[pr, :] = _pk(kvc)
        xs = jnp.dot(fw_ref[...], kvc, preferred_element_type=f32)
        xf[j, 0] = xs[:, :HALF]
        xf[j, 1] = xs[:, HALF:]
        xg = _un(x_s[pr, :]).astype(f32) * gw_ref[...].astype(f32).reshape(1, M)
        g_s[r, :] = jax.nn.sigmoid(jnp.sum(xg, axis=1, keepdims=True))

    def conv_forward_k(j, slot):
        kn = jax.lax.dot_general(fw_ref[...], _un(skb[slot]), NT, preferred_element_type=f32)
        q4 = C // 2
        kp = kprev[...]
        kw = jnp.concatenate([
            kn[0:q4] - kp[2 * q4:3 * q4],
            kn[q4:2 * q4] + kp[3 * q4:4 * q4],
            kn[2 * q4:3 * q4] + kp[0:q4],
            kn[3 * q4:4 * q4] - kp[q4:2 * q4],
        ], axis=0)
        kprev[...] = kn
        kf[j, 0] = kw[:, :HALF]
        kf[j, 1] = kw[:, HALF:]

    def conv_block_items(n, group):
        half = n % 2
        re = pl.ds(pl.multiple_of((n // 2) * 16, 16), 16)
        im = pl.ds(pl.multiple_of(C + (n // 2) * 16, 16), 16)
        pre = pl.ds(pl.multiple_of((n // 2) * 8, 8), 8)
        pim = pl.ds(pl.multiple_of(C // 2 + (n // 2) * 8, 8), 8)

        acc = {}

        def some(lb, i, a0, a1):
            ln = slice(lb * T, (lb + 1) * T)
            yr, yi = acc.pop((lb, i), (None, None))
            for a in range(a0, a1):
                xr, xi = xf[i - a, half, re, ln], xf[i - a, half, im, ln]
                kr, ki = kf[a, half, re, ln], kf[a, half, im, ln]
                pr = xr * kr - xi * ki
                pi = xr * ki + xi * kr
                yr = pr if yr is None else yr + pr
                yi = pi if yi is None else yi + pi
            if a1 == i + 1:
                yr, yi = _pk(yr.astype(bf16)), _pk(yi.astype(bf16))
                yf[i, half, pre, ln] = yr
                yf[i, half, pim, ln] = yi
                return _zero_of(yr | yi)
            acc[lb, i] = (yr, yi)
            ur, ui = pltpu.bitcast(yr, u32), pltpu.bitcast(yi, u32)
            return _zero_of((ur[:8] | ur[8:]) | (ui[:8] | ui[8:]))

        return [(min(a0 + group, i + 1) - a0,
                 (lambda lb=lb, i=i, a0=a0: some(lb, i, a0, min(a0 + group, i + 1))))
                for lb in range(HALF // T) for i in range(NCH) for a0 in range(0, i + 1, group)]

    def conv_inverse(j):
        dvec = sd_ref[...].astype(f32).reshape(1, M)
        pr = pl.ds(pl.multiple_of(j * (C // 2), C // 2), C // 2)
        y = jnp.concatenate(
            [jnp.dot(iv_ref[...], _un(yf[j, hh]), preferred_element_type=f32)
             for hh in range(2)], axis=1)
        y = y + _un(kv_s[pr, :]).astype(f32) * dvec
        return _un(x_s[pr, :]).astype(f32) * y

    def prologue():
        first = w_copies(0, 1)
        for cp in first[1:]:
            cp.start()
        for i in range(NQ):
            block_copy(0, i).start()
        for cp in small_copies():
            cp.start()
        first[0].start()
        for i in range(NX):
            block_copy(1, i).start()
        for cp in chunk_copies(0, 0):
            cp.start()
        kprev[...] = jnp.zeros(kprev.shape, f32)
        khalo[...] = jnp.zeros(khalo.shape, f32)
        for cp in first[1:]:
            cp.wait()
        unpack_weights(1, 0, (1, 2))

        def kv_body(i, carry):
            block_copy(0, i).wait()
            pr = pl.ds(pl.multiple_of(i * (BQ // 2), BQ // 2), BQ // 2)
            cc = _un(c_s[pr, :])
            k_s[pr, :] = _pk(jnp.dot(cc, _un(wk_s[...]), preferred_element_type=f32).astype(bf16))
            v_s[pr, :] = _pk(jnp.dot(cc, _un(wv_s[...]), preferred_element_type=f32).astype(bf16))
            return carry

        jax.lax.fori_loop(0, NQ, kv_body, 0)
        first[0].wait()
        unpack_weights(1, 0, (0,))
        for n, buf in enumerate((wqb, wkb, wvb)):
            pltpu.make_async_copy(buf.at[1], buf.at[0], w_sem.at[0, n]).start()

        def q_body(i, carry):
            block_copy(1, i).wait()
            pr = pl.ds(pl.multiple_of(i * (S // 2 // NX), S // 2 // NX), S // 2 // NX)
            q = jnp.dot(_un(x_s[pr, :]), _un(wq_s[...]), preferred_element_type=f32)
            q_s[pr, :] = _pk((q * QSCALE).astype(bf16))
            return carry

        jax.lax.fori_loop(0, NX, q_body, 0)
        for cp in small_copies():
            cp.wait()
        wo_copy().start()

    def next_weights(h):
        slot = h % 2
        for cp in w_copies((h + 1) // 2, slot):
            cp.wait()
        for cp in w_copies(jnp.minimum((h + 2) // 2, H // 2 - 1), 1 - slot):
            cp.start()
        unpack_weights(slot, (h + 1) % 2)

    HB = BQ // 2

    def head_step(fill, hk):
        def run(*names):
            gate = None
            for name in names:
                if name in fill:
                    res = fill[name](hk)
                    if res is not None and USE_GATE:
                        r = int(res.shape[0] * (GATE_Q if name[0] == 'Q' else GATE_K)) // 8 * 8
                        gate = pltpu.bitcast(_zero_of(res[r:r + 8]), f32)
            return gate

        def block(i, before, after):
            order = list(range(i + 1))
            if DIAG_FIRST:
                order = order[-1:] + order[:-1]
            for n, g in enumerate(order):
                scores(i, g, hk)
                hk.urgent += partial_max_items(i, g, n == 0)
            gate = run(*before)
            hk.flush_urgent()
            row_max(i)
            context(i, gate)
            run(*after)

        for i in range(NQ - 1, -1, -1):
            block(i, *FILL_ORDER[i])
        hk.flush()

    def proj_fill():
        fill = {}
        for i in range(NQ):
            fill["K%d" % i] = lambda hk, i=i: k_proj(i * BQ, (i + 1) * BQ, hk)
            fill["V%d" % i] = lambda hk, i=i: v_proj(i * BQ, (i + 1) * BQ, hk)
            fill["Q%da" % i] = lambda hk, i=i: q_proj(i * BQ, i * BQ + HB, hk)
            fill["Q%db" % i] = lambda hk, i=i: q_proj(i * BQ + HB, (i + 1) * BQ, hk)
        return fill

    def forward_step(h, carry):
        cur["h"] = h
        slot = h % 2
        for cp in chunk_copies(h, slot):
            cp.wait()
        for cp in chunk_copies(jnp.minimum(h + 1, NCH - 1), 1 - slot):
            cp.start()
        next_weights(h)
        fill = proj_fill()
        fill["E0"] = lambda hk: conv_forward_x(h, slot)
        fill["E1"] = lambda hk: conv_forward_k(h, slot)
        head_step(fill, Hooks())
        return carry

    def product_step(h, carry):
        cur["h"] = h
        next_weights(h)
        head_step(proj_fill(), Hooks(conv_block_items(h - NCH, GROUP), rate=0.8))
        return carry

    def last_step():
        cur["h"] = H - 1
        for cp in w_copies(H // 2 - 1, (H - 1) % 2) + chunk_copies(NCH - 1, NCH % 2):
            cp.wait()
        wo_copy().wait()
        head_step({}, Hooks(conv_block_items(NCH - 1, 4), rate=3.0))

    def out_copy(e):
        r = pl.ds(pl.multiple_of(e * RE, RE), RE)
        return pltpu.make_async_copy(o_s.at[r, :], o_hbm.at[0, r, :], o_sem.at[e])

    def output_step(e, carry):
        pr = pl.ds(pl.multiple_of(e * (RE // 2), RE // 2), RE // 2)
        r = pl.ds(pl.multiple_of(e * RE, RE), RE)
        ctx = jnp.concatenate([_un(ctx_s[hh, pr, :]) for hh in range(H)], axis=1)
        b = jnp.concatenate([conv_inverse(e * (RE // C) + j) for j in range(RE // C)], axis=0)
        a = jnp.dot(ctx, _un(wo_s[...]), preferred_element_type=f32)
        g = g_s[r, :]
        o_s[r, :] = (b + g * (a - b)).astype(bf16)
        out_copy(e).start()
        return carry

    prologue()
    jax.lax.fori_loop(0, NCH, forward_step, 0)
    jax.lax.fori_loop(NCH, H - 1, product_step, 0)
    last_step()
    jax.lax.fori_loop(0, NE, output_step, 0)
    for e in range(NE):
        out_copy(e).wait()


@jax.jit
def pallas_gated_mix__compressed_kv_cla__ssm_conv_h3__prompt_kernel(
    A_x: jax.Array,
    A_c_kv: jax.Array,
    A_w_q: jax.Array,
    A_w_uk: jax.Array,
    A_w_uv: jax.Array,
    A_w_o: jax.Array,
    B_q: jax.Array,
    B_k: jax.Array,
    B_v: jax.Array,
    B_shift_k: jax.Array,
    B_ssm_k: jax.Array,
    B_ssm_D: jax.Array,
    gate_w: jax.Array,
):
    fwd, inv = _dft_matrices()
    fwd = jnp.asarray(fwd, bf16)
    inv = jnp.asarray(inv, bf16)

    in_specs = [pl.BlockSpec(memory_space=pl.ANY)] * 14
    scratch = [
        pltpu.VMEM((S, M), bf16),
        pltpu.SemaphoreType.DMA((NE,)),
        pltpu.VMEM((S // 2, M), u32),
        pltpu.VMEM((S // 2, DC), u32),
        pltpu.VMEM((H * D // 2, M), u32),
        pltpu.VMEM((S // 2, D), u32), pltpu.VMEM((S // 2, D), u32), pltpu.VMEM((S // 2, D), u32),
        pltpu.VMEM((H, S // 2, D), u32),
        pltpu.VMEM((2, M, D), u32), pltpu.VMEM((2, DC, D), u32), pltpu.VMEM((2, DC, D), u32),
        pltpu.VMEM((M // 2, D), u32), pltpu.VMEM((DC // 2, D), u32), pltpu.VMEM((DC // 2, D), u32),
        pltpu.VMEM((2, C // 2, M), u32), pltpu.VMEM((2, C // 2, M), u32),
        pltpu.VMEM((2, M // 2, C), u32),
        pltpu.VMEM((NCH, 2, 2 * C, HALF), f32),
        pltpu.VMEM((NCH, 2, 2 * C, HALF), f32),
        pltpu.VMEM((NCH, 2, C, HALF), u32),
        pltpu.VMEM((2 * C, M), f32),
        pltpu.VMEM((8, M), f32),
        pltpu.VMEM((S // 2, M), u32),
        pltpu.VMEM((S, 1), f32),
        pltpu.VMEM((KS, M), bf16), pltpu.VMEM((M,), bf16), pltpu.VMEM((M,), bf16),
        pltpu.VMEM((2 * C, C), bf16), pltpu.VMEM((C, 2 * C), bf16),
        pltpu.SemaphoreType.DMA((5,)),
        pltpu.SemaphoreType.DMA((2, NX)),
        pltpu.SemaphoreType.DMA((1,)),
        pltpu.SemaphoreType.DMA((2, 3)),
        pltpu.SemaphoreType.DMA((2, 3)),
    ]
    return pl.pallas_call(
        _kernel,
        in_specs=in_specs,
        out_specs=pl.BlockSpec(memory_space=pl.ANY),
        out_shape=jax.ShapeDtypeStruct((1, S, M), bf16),
        scratch_shapes=scratch,
        compiler_params=pltpu.CompilerParams(
            vmem_limit_bytes=126 * 1024 * 1024,
        ),
        name="gated_mix_kernel",
    )(A_x, A_c_kv, A_w_q, A_w_uk, A_w_uv, A_w_o.reshape(H * D, M), B_k, B_v, B_ssm_k,
      B_shift_k.T, B_ssm_D, gate_w, fwd, inv)
```

```python
import math

import jax
import jax.numpy as jnp
import numpy as np
import jax.experimental.pallas as pl
import jax.experimental.pallas.tpu as pltpu

f32 = jnp.float32
bf16 = jnp.bfloat16
u32 = jnp.uint32

S = 2048
M = 1024
DC = 512
H = 32
D = 128
T = 128
BQ = 512
NQ = S // BQ
NSUB = BQ // T
NX = 8
RC = 32
PRODUCT_RATE = 0.8
FILL_ORDER = {
    3: (("K3", "Q3a"), ("V3",)),
    2: (("Q3b", "K2"), ("V2",)),
    1: (("Q2a", "Q2b"), ("V1",)),
    0: (("K1", "Q1a", "Q1b"), ("V0", "E0", "E1", "K0", "Q0a", "Q0b")),
}
C = 128
NCH = S // C
HALF = M // 2
KS = 4
RE = 256
NE = S // RE

QSCALE = (D ** -0.5) * math.log2(math.e)
NEG = -1e30
NT = (((1,), (1,)), ((), ()))


def _dft_matrices():
    freqs = np.concatenate([np.arange(0, C, 2), np.arange(1, C, 2)])
    t = np.arange(C)
    n = ((2 * freqs[:, None] + 1) * t[None, :]) % (4 * C)
    ang = np.pi * n / (2 * C)
    fwd = np.concatenate([np.cos(ang), -np.sin(ang)], axis=0)
    inv = fwd.T / C
    return fwd.astype(np.float32), inv.astype(np.float32)


def _iota(shape, dim):
    return jax.lax.broadcasted_iota(jnp.int32, shape, dim)


def _pk(v):
    return pltpu.bitcast(v, u32)


def _un(u):
    return pltpu.bitcast(u, bf16)


def _ld(ref, r0, r1, cols=slice(None)):
    return _un(ref[r0 // 2: r1 // 2, cols])


def _zero_of(t):
    return (pltpu.bitcast(t, u32) >> 31) & jnp.uint32(2)


class Hooks:
    def __init__(self, items=(), rate=1.0):
        self.items = list(items)
        self.rate = rate
        self.credit = 0.0

    def take(self):
        self.credit += self.rate
        if self.items and self.items[0][0] <= self.credit:
            cost, thunk = self.items.pop(0)
            self.credit -= cost
            return thunk()
        return None

    def flush(self):
        for _, thunk in self.items:
            thunk()
        self.items = []

    def lhs(self, u, tiles=(0,)):
        nrow = u.shape[0] // 8
        cols = [u[:, t * T:(t + 1) * T] for t in range(u.shape[1] // T)]
        for t in tiles:
            parts, start = [], 0
            for r in range(nrow):
                z = self.take()
                if z is not None:
                    if r * 8 > start:
                        parts.append(cols[t][start:r * 8])
                    parts.append(cols[t][r * 8:(r + 1) * 8] | z)
                    start = (r + 1) * 8
            if start < nrow * 8:
                parts.append(cols[t][start:])
            cols[t] = parts[0] if len(parts) == 1 else jnp.concatenate(parts, axis=0)
        return _un(cols[0] if len(cols) == 1 else jnp.concatenate(cols, axis=1))


def _kernel(x_hbm, c_hbm, wq_hbm, wk_hbm, wv_hbm, wo_hbm, k_hbm, v_hbm, sk_hbm,
            sh_hbm, sd_hbm, gw_hbm, fw_hbm, iv_hbm, o_hbm,
            o_s, o_sem, x_s, c_s, wo_s, q_s, k_s, v_s, ctx_s, wqb, wkb, wvb, wq_s, wk_s, wv_s,
            kb, vb, skb, xf, kf, yf, kprev, khalo, kv_s, g_s,
            sh_ref, sd_ref, gw_ref, fw_ref, iv_ref, small_sem, big_sem, wo_sem, w_sem, ch_sem):
    cur = {}

    def block_copy(n, i):
        src, dst = ((c_hbm, c_s), (x_hbm, x_s))[n]
        size = S // 2 // (NQ, NX)[n]
        rows = pl.ds(pl.multiple_of(i * size, size), size)
        return pltpu.make_async_copy(src.at[0].bitcast(u32).at[rows, :], dst.at[rows, :],
                                     big_sem.at[n, i])

    def small_copies():
        pairs = ((sh_hbm, sh_ref), (sd_hbm, sd_ref), (gw_hbm, gw_ref), (fw_hbm, fw_ref),
                 (iv_hbm, iv_ref))
        return [pltpu.make_async_copy(src, dst, small_sem.at[n])
                for n, (src, dst) in enumerate(pairs)]

    def wo_copy():
        return pltpu.make_async_copy(wo_hbm.bitcast(u32), wo_s, wo_sem.at[0])

    def w_copies(pair, slot):
        return [
            pltpu.make_async_copy(src.bitcast(u32).at[:, pair, :], dst.at[slot], w_sem.at[slot, n])
            for n, (src, dst) in enumerate(((wq_hbm, wqb), (wk_hbm, wkb), (wv_hbm, wvb)))
        ]

    def chunk_copies(j, slot):
        rows = pl.ds(pl.multiple_of(j * (C // 2), C // 2), C // 2)
        cols = pl.ds(pl.multiple_of(j * C, C), C)
        return [
            pltpu.make_async_copy(k_hbm.at[0].bitcast(u32).at[rows, :], kb.at[slot], ch_sem.at[slot, 0]),
            pltpu.make_async_copy(v_hbm.at[0].bitcast(u32).at[rows, :], vb.at[slot], ch_sem.at[slot, 1]),
            pltpu.make_async_copy(sk_hbm.bitcast(u32).at[:, cols], skb.at[slot], ch_sem.at[slot, 2]),
        ]

    def unpack_weights(slot, parity, which=(0, 1, 2)):
        sh = jnp.asarray(16 * (1 - parity)).astype(u32)
        for n in which:
            src, dst = ((wqb, wq_s), (wkb, wk_s), (wvb, wv_s))[n]
            u = (src[slot] << sh) & jnp.uint32(0xFFFF0000)
            dst[...] = _pk(pltpu.bitcast(u, f32).astype(bf16))

    def q_proj(r0, r1, hk):
        lhs = hk.lhs(x_s[r0 // 2: r1 // 2, :], (0, 4))
        q = jnp.dot(lhs, _un(wq_s[...]), preferred_element_type=f32)
        q_s[r0 // 2: r1 // 2, :] = _pk((q * QSCALE).astype(bf16))

    def k_proj(r0, r1, hk):
        lhs = hk.lhs(c_s[r0 // 2: r1 // 2, :])
        k = jnp.dot(lhs, _un(wk_s[...]), preferred_element_type=f32)
        k_s[r0 // 2: r1 // 2, :] = _pk(k.astype(bf16))

    def v_proj(r0, r1, hk):
        lhs = hk.lhs(c_s[r0 // 2: r1 // 2, :])
        v = jnp.dot(lhs, _un(wv_s[...]), preferred_element_type=f32)
        v_s[r0 // 2: r1 // 2, :] = _pk(v.astype(bf16))

    st = {}

    def scores(i, g, hk):
        base = i * BQ
        qu = q_s[base // 2: (base + BQ) // 2, :]
        if g < i:
            st["s", i, g] = jax.lax.dot_general(hk.lhs(qu), _ld(k_s, g * BQ, (g + 1) * BQ), NT,
                                                preferred_element_type=f32)
            return
        q = _un(qu)
        tri = _iota((T, T), 1) <= _iota((T, T), 0)
        sd = []
        for t in range(NSUB):
            s = jax.lax.dot_general(q[t * T:, :], _ld(k_s, base + t * T, base + (t + 1) * T), NT,
                                    preferred_element_type=f32)
            top = jnp.where(tri, s[:T], NEG)
            sd.append(top if t == NSUB - 1 else jnp.concatenate([top, s[T:]], axis=0))
        st["s", i, i] = sd

    def group_tiles(i, g, r0):
        s = st["s", i, g]
        if g < i:
            return [s[r0:r0 + RC, cc * T:(cc + 1) * T] for cc in range(NSUB)]
        return [s[t][r0 - t * T: r0 - t * T + RC] for t in range(r0 // T + 1)]

    def tree(op, xs):
        while len(xs) > 1:
            xs = [op(xs[n], xs[n + 1]) if n + 1 < len(xs) else xs[n] for n in range(0, len(xs), 2)]
        return xs[0]

    chunks = list(range(0, BQ, RC))

    def diag_first(i):
        return [i] + list(range(i))

    def row_max(i):
        mel = {}
        for n, g in enumerate(diag_first(i)):
            for r0 in chunks:
                pm = tree(jnp.maximum, group_tiles(i, g, r0))
                mel[r0] = pm if n == 0 else jnp.maximum(mel[r0], pm)
        st["m", i] = {r0: jnp.broadcast_to(jnp.max(mel[r0], axis=1, keepdims=True), (RC, T))
                      for r0 in chunks}

    def context(i):
        base = i * BQ
        mb = st.pop(("m", i))
        lsum = {}
        acc = None
        dep = None
        for n, g in enumerate(diag_first(i)):
            ps = {}
            for r0 in chunks:
                m = mb[r0]
                if dep is not None:
                    m = jnp.concatenate([m[:8] + dep, m[8:]], axis=0)
                p = [jnp.exp2(t - m) for t in group_tiles(i, g, r0)]
                part = tree(jnp.add, p)
                lsum[r0] = part if n == 0 else lsum[r0] + part
                dep = tree(jnp.add, [lsum[r0][q:q + 8] for q in range(0, RC, 8)]) * 0.0
                ps[r0] = p
            if g < i:
                pg = jnp.concatenate([jnp.concatenate(ps[r0], axis=1) for r0 in chunks], axis=0)
                pv = jnp.dot(pg.astype(bf16), _ld(v_s, g * BQ, (g + 1) * BQ),
                             preferred_element_type=f32)
                acc = pv if acc is None else acc + pv
            else:
                parts = [None] * NSUB
                for t in range(NSUB):
                    pt = jnp.concatenate([ps[r0][t] for r0 in chunks if r0 >= t * T], axis=0)
                    pv = jnp.dot(pt.astype(bf16), _ld(v_s, base + t * T, base + (t + 1) * T),
                                 preferred_element_type=f32)
                    for r in range(t, NSUB):
                        piece = pv[(r - t) * T:(r - t + 1) * T]
                        parts[r] = piece if parts[r] is None else parts[r] + piece
                diag = jnp.concatenate(parts, axis=0)
                acc = diag if acc is None else acc + diag
            st.pop(("s", i, g))
        for r0 in chunks:
            l = jnp.sum(lsum[r0], axis=1, keepdims=True)
            inv = pl.reciprocal(l, approx=True)
            inv = inv * (2.0 - l * inv)
            ctx_s[cur["h"], (base + r0) // 2: (base + r0 + RC) // 2, :] = _pk(
                (acc[r0:r0 + RC] * inv).astype(bf16))

    def conv_forward_x(j, slot):
        pr = pl.ds(pl.multiple_of(j * (C // 2), C // 2), C // 2)
        r = pl.ds(pl.multiple_of(j * C, C), C)
        w = sh_ref[...].astype(f32)
        kc = _un(kb[slot]).astype(f32)
        ext = jnp.concatenate([khalo[...], kc], axis=0)
        ks = kc * w[0:1]
        for lag in range(1, KS):
            ks = ks + ext[8 - lag: 8 + C - lag] * w[lag:lag + 1]
        khalo[...] = kc[C - 8:]
        kvc = (ks * _un(vb[slot]).astype(f32)).astype(bf16)
        kv_s[pr, :] = _pk(kvc)
        xs = jnp.dot(fw_ref[...], kvc, preferred_element_type=f32)
        xf[j, 0] = xs[:, :HALF]
        xf[j, 1] = xs[:, HALF:]
        xg = _un(x_s[pr, :]).astype(f32) * gw_ref[...].astype(f32).reshape(1, M)
        g_s[r, :] = jax.nn.sigmoid(jnp.sum(xg, axis=1, keepdims=True))

    def conv_forward_k(j, slot):
        kn = jax.lax.dot_general(fw_ref[...], _un(skb[slot]), NT, preferred_element_type=f32)
        q4 = C // 2
        kp = kprev[...]
        kw = jnp.concatenate([
            kn[0:q4] - kp[2 * q4:3 * q4],
            kn[q4:2 * q4] + kp[3 * q4:4 * q4],
            kn[2 * q4:3 * q4] + kp[0:q4],
            kn[3 * q4:4 * q4] - kp[q4:2 * q4],
        ], axis=0)
        kprev[...] = kn
        kf[j, 0] = kw[:, :HALF]
        kf[j, 1] = kw[:, HALF:]

    def conv_block_items(n, group):
        half = n % 2
        re = pl.ds(pl.multiple_of((n // 2) * 16, 16), 16)
        im = pl.ds(pl.multiple_of(C + (n // 2) * 16, 16), 16)
        pre = pl.ds(pl.multiple_of((n // 2) * 8, 8), 8)
        pim = pl.ds(pl.multiple_of(C // 2 + (n // 2) * 8, 8), 8)

        acc = {}

        def some(lb, i, a0, a1):
            ln = slice(lb * T, (lb + 1) * T)
            yr, yi = acc.pop((lb, i), (None, None))
            for a in range(a0, a1):
                xr, xi = xf[i - a, half, re, ln], xf[i - a, half, im, ln]
                kr, ki = kf[a, half, re, ln], kf[a, half, im, ln]
                pr = xr * kr - xi * ki
                pi = xr * ki + xi * kr
                yr = pr if yr is None else yr + pr
                yi = pi if yi is None else yi + pi
            if a1 == i + 1:
                yr, yi = _pk(yr.astype(bf16)), _pk(yi.astype(bf16))
                yf[i, half, pre, ln] = yr
                yf[i, half, pim, ln] = yi
                return _zero_of(yr | yi)
            acc[lb, i] = (yr, yi)
            ur, ui = pltpu.bitcast(yr, u32), pltpu.bitcast(yi, u32)
            return _zero_of((ur[:8] | ur[8:]) | (ui[:8] | ui[8:]))

        return [(min(a0 + group, i + 1) - a0,
                 (lambda lb=lb, i=i, a0=a0: some(lb, i, a0, min(a0 + group, i + 1))))
                for lb in range(HALF // T) for i in range(NCH) for a0 in range(0, i + 1, group)]

    def conv_inverse(j):
        dvec = sd_ref[...].astype(f32).reshape(1, M)
        pr = pl.ds(pl.multiple_of(j * (C // 2), C // 2), C // 2)
        y = jnp.concatenate(
            [jnp.dot(iv_ref[...], _un(yf[j, hh]), preferred_element_type=f32)
             for hh in range(2)], axis=1)
        y = y + _un(kv_s[pr, :]).astype(f32) * dvec
        return _un(x_s[pr, :]).astype(f32) * y

    def prologue():
        first = w_copies(0, 1)
        for cp in first[1:]:
            cp.start()
        for i in range(NQ):
            block_copy(0, i).start()
        first[0].start()
        for i in range(NX):
            block_copy(1, i).start()
        for cp in small_copies() + chunk_copies(0, 0):
            cp.start()
        kprev[...] = jnp.zeros(kprev.shape, f32)
        khalo[...] = jnp.zeros(khalo.shape, f32)
        for cp in first[1:]:
            cp.wait()
        unpack_weights(1, 0, (1, 2))

        def kv_body(i, carry):
            block_copy(0, i).wait()
            pr = pl.ds(pl.multiple_of(i * (BQ // 2), BQ // 2), BQ // 2)
            cc = _un(c_s[pr, :])
            k_s[pr, :] = _pk(jnp.dot(cc, _un(wk_s[...]), preferred_element_type=f32).astype(bf16))
            v_s[pr, :] = _pk(jnp.dot(cc, _un(wv_s[...]), preferred_element_type=f32).astype(bf16))
            return carry

        jax.lax.fori_loop(0, NQ, kv_body, 0)
        first[0].wait()
        unpack_weights(1, 0, (0,))
        for n, buf in enumerate((wqb, wkb, wvb)):
            pltpu.make_async_copy(buf.at[1], buf.at[0], w_sem.at[0, n]).start()

        def q_body(i, carry):
            block_copy(1, i).wait()
            pr = pl.ds(pl.multiple_of(i * (S // 2 // NX), S // 2 // NX), S // 2 // NX)
            q = jnp.dot(_un(x_s[pr, :]), _un(wq_s[...]), preferred_element_type=f32)
            q_s[pr, :] = _pk((q * QSCALE).astype(bf16))
            return carry

        jax.lax.fori_loop(0, NX, q_body, 0)
        for cp in small_copies():
            cp.wait()
        wo_copy().start()

    def next_weights(h):
        slot = h % 2
        for cp in w_copies((h + 1) // 2, slot):
            cp.wait()
        for cp in w_copies(jnp.minimum((h + 2) // 2, H // 2 - 1), 1 - slot):
            cp.start()
        unpack_weights(slot, (h + 1) % 2)

    HB = BQ // 2

    def head_step(fill, hk):
        def run(names):
            for name in names:
                if name in fill:
                    fill[name](hk)

        for i in range(NQ - 1, -1, -1):
            before, after = FILL_ORDER[i]
            for g in diag_first(i):
                scores(i, g, hk)
            run(before)
            row_max(i)
            context(i)
            run(after)
        hk.flush()

    def proj_fill():
        fill = {}
        for i in range(NQ):
            fill["K%d" % i] = lambda hk, i=i: k_proj(i * BQ, (i + 1) * BQ, hk)
            fill["V%d" % i] = lambda hk, i=i: v_proj(i * BQ, (i + 1) * BQ, hk)
            fill["Q%da" % i] = lambda hk, i=i: q_proj(i * BQ, i * BQ + HB, hk)
            fill["Q%db" % i] = lambda hk, i=i: q_proj(i * BQ + HB, (i + 1) * BQ, hk)
        return fill

    def forward_step(h, carry):
        cur["h"] = h
        slot = h % 2
        for cp in chunk_copies(h, slot):
            cp.wait()
        for cp in chunk_copies(jnp.minimum(h + 1, NCH - 1), 1 - slot):
            cp.start()
        next_weights(h)
        fill = proj_fill()
        fill["E0"] = lambda hk: conv_forward_x(h, slot)
        fill["E1"] = lambda hk: conv_forward_k(h, slot)
        head_step(fill, Hooks())
        return carry

    def product_step(h, carry):
        cur["h"] = h
        next_weights(h)
        head_step(proj_fill(), Hooks(conv_block_items(h - NCH, 1), rate=PRODUCT_RATE))
        return carry

    def last_step():
        cur["h"] = H - 1
        for cp in w_copies(H // 2 - 1, (H - 1) % 2) + chunk_copies(NCH - 1, NCH % 2):
            cp.wait()
        wo_copy().wait()
        head_step({}, Hooks(conv_block_items(NCH - 1, 4), rate=3.0))

    def out_copy(e):
        r = pl.ds(pl.multiple_of(e * RE, RE), RE)
        return pltpu.make_async_copy(o_s.at[r, :], o_hbm.at[0, r, :], o_sem.at[e])

    def output_step(e, carry):
        pr = pl.ds(pl.multiple_of(e * (RE // 2), RE // 2), RE // 2)
        r = pl.ds(pl.multiple_of(e * RE, RE), RE)
        ctx = jnp.concatenate([_un(ctx_s[hh, pr, :]) for hh in range(H)], axis=1)
        b = jnp.concatenate([conv_inverse(e * (RE // C) + j) for j in range(RE // C)], axis=0)
        a = jnp.dot(ctx, _un(wo_s[...]), preferred_element_type=f32)
        g = g_s[r, :]
        o_s[r, :] = (b + g * (a - b)).astype(bf16)
        out_copy(e).start()
        return carry

    prologue()
    jax.lax.fori_loop(0, NCH, forward_step, 0)
    jax.lax.fori_loop(NCH, H - 1, product_step, 0)
    last_step()
    jax.lax.fori_loop(0, NE, output_step, 0)
    for e in range(NE):
        out_copy(e).wait()


@jax.jit
def pallas_gated_mix__compressed_kv_cla__ssm_conv_h3__prompt_kernel(
    A_x: jax.Array,
    A_c_kv: jax.Array,
    A_w_q: jax.Array,
    A_w_uk: jax.Array,
    A_w_uv: jax.Array,
    A_w_o: jax.Array,
    B_q: jax.Array,
    B_k: jax.Array,
    B_v: jax.Array,
    B_shift_k: jax.Array,
    B_ssm_k: jax.Array,
    B_ssm_D: jax.Array,
    gate_w: jax.Array,
):
    fwd, inv = _dft_matrices()
    fwd = jnp.asarray(fwd, bf16)
    inv = jnp.asarray(inv, bf16)

    in_specs = [pl.BlockSpec(memory_space=pl.ANY)] * 14
    scratch = [
        pltpu.VMEM((S, M), bf16),
        pltpu.SemaphoreType.DMA((NE,)),
        pltpu.VMEM((S // 2, M), u32),
        pltpu.VMEM((S // 2, DC), u32),
        pltpu.VMEM((H * D // 2, M), u32),
        pltpu.VMEM((S // 2, D), u32), pltpu.VMEM((S // 2, D), u32), pltpu.VMEM((S // 2, D), u32),
        pltpu.VMEM((H, S // 2, D), u32),
        pltpu.VMEM((2, M, D), u32), pltpu.VMEM((2, DC, D), u32), pltpu.VMEM((2, DC, D), u32),
        pltpu.VMEM((M // 2, D), u32), pltpu.VMEM((DC // 2, D), u32), pltpu.VMEM((DC // 2, D), u32),
        pltpu.VMEM((2, C // 2, M), u32), pltpu.VMEM((2, C // 2, M), u32),
        pltpu.VMEM((2, M // 2, C), u32),
        pltpu.VMEM((NCH, 2, 2 * C, HALF), f32),
        pltpu.VMEM((NCH, 2, 2 * C, HALF), f32),
        pltpu.VMEM((NCH, 2, C, HALF), u32),
        pltpu.VMEM((2 * C, M), f32),
        pltpu.VMEM((8, M), f32),
        pltpu.VMEM((S // 2, M), u32),
        pltpu.VMEM((S, 1), f32),
        pltpu.VMEM((KS, M), bf16), pltpu.VMEM((M,), bf16), pltpu.VMEM((M,), bf16),
        pltpu.VMEM((2 * C, C), bf16), pltpu.VMEM((C, 2 * C), bf16),
        pltpu.SemaphoreType.DMA((5,)),
        pltpu.SemaphoreType.DMA((2, NX)),
        pltpu.SemaphoreType.DMA((1,)),
        pltpu.SemaphoreType.DMA((2, 3)),
        pltpu.SemaphoreType.DMA((2, 3)),
    ]
    return pl.pallas_call(
        _kernel,
        in_specs=in_specs,
        out_specs=pl.BlockSpec(memory_space=pl.ANY),
        out_shape=jax.ShapeDtypeStruct((1, S, M), bf16),
        scratch_shapes=scratch,
        compiler_params=pltpu.CompilerParams(
            vmem_limit_bytes=126 * 1024 * 1024,
        ),
        name="gated_mix_kernel",
    )(A_x, A_c_kv, A_w_q, A_w_uk, A_w_uv, A_w_o.reshape(H * D, M), B_k, B_v, B_ssm_k,
      B_shift_k.T, B_ssm_D, gate_w, fwd, inv)
```

```python
import math

import jax
import jax.numpy as jnp
import numpy as np
import jax.experimental.pallas as pl
import jax.experimental.pallas.tpu as pltpu

f32 = jnp.float32
bf16 = jnp.bfloat16
u32 = jnp.uint32

S = 2048
M = 1024
DC = 512
H = 32
D = 128
T = 128
BQ = 512
NQ = S // BQ
NSUB = BQ // T
NX = 8
RC = 32
PRODUCT_RATE = 0.8
FILL_ORDER = {
    3: (("K3", "Q3a"), ("V3",)),
    2: (("Q3b", "K2"), ("V2",)),
    1: (("Q2a", "Q2b"), ("V1",)),
    0: (("K1", "Q1a", "Q1b"), ("V0", "E0", "E1", "K0", "Q0a", "Q0b")),
}
C = 128
NCH = S // C
HALF = M // 2
KS = 4
RE = 256
NE = S // RE

QSCALE = (D ** -0.5) * math.log2(math.e)
NEG = -1e30
NT = (((1,), (1,)), ((), ()))


def _dft_matrices():
    freqs = np.concatenate([np.arange(0, C, 2), np.arange(1, C, 2)])
    t = np.arange(C)
    n = ((2 * freqs[:, None] + 1) * t[None, :]) % (4 * C)
    ang = np.pi * n / (2 * C)
    fwd = np.concatenate([np.cos(ang), -np.sin(ang)], axis=0)
    inv = fwd.T / C
    return fwd.astype(np.float32), inv.astype(np.float32)


def _iota(shape, dim):
    return jax.lax.broadcasted_iota(jnp.int32, shape, dim)


def _pk(v):
    return pltpu.bitcast(v, u32)


def _un(u):
    return pltpu.bitcast(u, bf16)


def _ld(ref, r0, r1, cols=slice(None)):
    return _un(ref[r0 // 2: r1 // 2, cols])


def _zero_of(t):
    return (pltpu.bitcast(t, u32) >> 31) & jnp.uint32(2)


class Hooks:
    def __init__(self, items=(), rate=1.0):
        self.items = list(items)
        self.rate = rate
        self.credit = 0.0

    def take(self):
        self.credit += self.rate
        if self.items and self.items[0][0] <= self.credit:
            cost, thunk = self.items.pop(0)
            self.credit -= cost
            return thunk()
        return None

    def flush(self):
        for _, thunk in self.items:
            thunk()
        self.items = []

    def lhs(self, u, tiles=(0,)):
        nrow = u.shape[0] // 8
        cols = [u[:, t * T:(t + 1) * T] for t in range(u.shape[1] // T)]
        for t in tiles:
            parts, start = [], 0
            for r in range(nrow):
                z = self.take()
                if z is not None:
                    if r * 8 > start:
                        parts.append(cols[t][start:r * 8])
                    parts.append(cols[t][r * 8:(r + 1) * 8] | z)
                    start = (r + 1) * 8
            if start < nrow * 8:
                parts.append(cols[t][start:])
            cols[t] = parts[0] if len(parts) == 1 else jnp.concatenate(parts, axis=0)
        return _un(cols[0] if len(cols) == 1 else jnp.concatenate(cols, axis=1))


def _kernel(x_hbm, c_hbm, wq_hbm, wk_hbm, wv_hbm, wo_hbm, k_hbm, v_hbm, sk_hbm,
            sh_hbm, sd_hbm, gw_hbm, fw_hbm, iv_hbm, o_hbm,
            o_s, o_sem, x_s, c_s, wo_s, q_s, k_s, v_s, ctx_s, wqb, wkb, wvb, wq_s, wk_s, wv_s,
            kb, vb, skb, xf, kf, yf, kprev, khalo, kv_s, g_s,
            sh_ref, sd_ref, gw_ref, fw_ref, iv_ref, small_sem, big_sem, wo_sem, w_sem, ch_sem):
    cur = {}

    def block_copy(n, i):
        src, dst = ((c_hbm, c_s), (x_hbm, x_s))[n]
        size = S // 2 // (NQ, NX)[n]
        rows = pl.ds(pl.multiple_of(i * size, size), size)
        return pltpu.make_async_copy(src.at[0].bitcast(u32).at[rows, :], dst.at[rows, :],
                                     big_sem.at[n, i])

    def small_copies():
        pairs = ((sh_hbm, sh_ref), (sd_hbm, sd_ref), (gw_hbm, gw_ref), (fw_hbm, fw_ref),
                 (iv_hbm, iv_ref))
        return [pltpu.make_async_copy(src, dst, small_sem.at[n])
                for n, (src, dst) in enumerate(pairs)]

    def wo_copy():
        return pltpu.make_async_copy(wo_hbm.bitcast(u32), wo_s, wo_sem.at[0])

    def w_copies(pair, slot):
        return [
            pltpu.make_async_copy(src.bitcast(u32).at[:, pair, :], dst.at[slot], w_sem.at[slot, n])
            for n, (src, dst) in enumerate(((wq_hbm, wqb), (wk_hbm, wkb), (wv_hbm, wvb)))
        ]

    def chunk_copies(j, slot):
        rows = pl.ds(pl.multiple_of(j * (C // 2), C // 2), C // 2)
        cols = pl.ds(pl.multiple_of(j * C, C), C)
        return [
            pltpu.make_async_copy(k_hbm.at[0].bitcast(u32).at[rows, :], kb.at[slot], ch_sem.at[slot, 0]),
            pltpu.make_async_copy(v_hbm.at[0].bitcast(u32).at[rows, :], vb.at[slot], ch_sem.at[slot, 1]),
            pltpu.make_async_copy(sk_hbm.bitcast(u32).at[:, cols], skb.at[slot], ch_sem.at[slot, 2]),
        ]

    def unpack_weights(slot, parity, which=(0, 1, 2)):
        sh = jnp.asarray(16 * (1 - parity)).astype(u32)
        for n in which:
            src, dst = ((wqb, wq_s), (wkb, wk_s), (wvb, wv_s))[n]
            u = (src[slot] << sh) & jnp.uint32(0xFFFF0000)
            dst[...] = _pk(pltpu.bitcast(u, f32).astype(bf16))

    def q_proj(r0, r1, hk):
        lhs = hk.lhs(x_s[r0 // 2: r1 // 2, :], (0, 4))
        q = jnp.dot(lhs, _un(wq_s[...]), preferred_element_type=f32)
        q_s[r0 // 2: r1 // 2, :] = _pk((q * QSCALE).astype(bf16))

    def k_proj(r0, r1, hk):
        lhs = hk.lhs(c_s[r0 // 2: r1 // 2, :])
        k = jnp.dot(lhs, _un(wk_s[...]), preferred_element_type=f32)
        k_s[r0 // 2: r1 // 2, :] = _pk(k.astype(bf16))

    def v_proj(r0, r1, hk):
        lhs = hk.lhs(c_s[r0 // 2: r1 // 2, :])
        v = jnp.dot(lhs, _un(wv_s[...]), preferred_element_type=f32)
        v_s[r0 // 2: r1 // 2, :] = _pk(v.astype(bf16))

    st = {}

    def scores(i, g, hk):
        base = i * BQ
        qu = q_s[base // 2: (base + BQ) // 2, :]
        if g < i:
            st["s", i, g] = jax.lax.dot_general(hk.lhs(qu), _ld(k_s, g * BQ, (g + 1) * BQ), NT,
                                                preferred_element_type=f32)
            return
        q = _un(qu)
        tri = _iota((T, T), 1) <= _iota((T, T), 0)
        sd = []
        for t in range(NSUB):
            s = jax.lax.dot_general(q[t * T:, :], _ld(k_s, base + t * T, base + (t + 1) * T), NT,
                                    preferred_element_type=f32)
            top = jnp.where(tri, s[:T], NEG)
            sd.append(top if t == NSUB - 1 else jnp.concatenate([top, s[T:]], axis=0))
        st["s", i, i] = sd

    def group_tiles(i, g, r0):
        s = st["s", i, g]
        if g < i:
            return [s[r0:r0 + RC, cc * T:(cc + 1) * T] for cc in range(NSUB)]
        return [s[t][r0 - t * T: r0 - t * T + RC] for t in range(r0 // T + 1)]

    def tree(op, xs):
        while len(xs) > 1:
            xs = [op(xs[n], xs[n + 1]) if n + 1 < len(xs) else xs[n] for n in range(0, len(xs), 2)]
        return xs[0]

    chunks = list(range(0, BQ, RC))

    def diag_first(i):
        return [i] + list(range(i))

    def row_max(i):
        mel = {}
        for n, g in enumerate(diag_first(i)):
            for r0 in chunks:
                pm = tree(jnp.maximum, group_tiles(i, g, r0))
                mel[r0] = pm if n == 0 else jnp.maximum(mel[r0], pm)
        st["m", i] = {r0: jnp.broadcast_to(jnp.max(mel[r0], axis=1, keepdims=True), (RC, T))
                      for r0 in chunks}

    def context(i):
        base = i * BQ
        mb = st.pop(("m", i))
        lsum = {}
        acc = None
        dep = None
        for n, g in enumerate(diag_first(i)):
            ps = {}
            for r0 in chunks:
                m = mb[r0]
                if dep is not None:
                    m = jnp.concatenate([m[:8] + dep, m[8:]], axis=0)
                p = [jnp.exp2(t - m) for t in group_tiles(i, g, r0)]
                part = tree(jnp.add, p)
                lsum[r0] = part if n == 0 else lsum[r0] + part
                dep = tree(jnp.add, [lsum[r0][q:q + 8] for q in range(0, RC, 8)]) * 0.0
                ps[r0] = p
            if g < i:
                pg = jnp.concatenate([jnp.concatenate(ps[r0], axis=1) for r0 in chunks], axis=0)
                pv = jnp.dot(pg.astype(bf16), _ld(v_s, g * BQ, (g + 1) * BQ),
                             preferred_element_type=f32)
                acc = pv if acc is None else acc + pv
            else:
                parts = [None] * NSUB
                for t in range(NSUB):
                    pt = jnp.concatenate([ps[r0][t] for r0 in chunks if r0 >= t * T], axis=0)
                    pv = jnp.dot(pt.astype(bf16), _ld(v_s, base + t * T, base + (t + 1) * T),
                                 preferred_element_type=f32)
                    for r in range(t, NSUB):
                        piece = pv[(r - t) * T:(r - t + 1) * T]
                        parts[r] = piece if parts[r] is None else parts[r] + piece
                diag = jnp.concatenate(parts, axis=0)
                acc = diag if acc is None else acc + diag
            st.pop(("s", i, g))
        for r0 in chunks:
            l = jnp.sum(lsum[r0], axis=1, keepdims=True)
            inv = pl.reciprocal(l, approx=True)
            inv = inv * (2.0 - l * inv)
            ctx_s[cur["h"], (base + r0) // 2: (base + r0 + RC) // 2, :] = _pk(
                (acc[r0:r0 + RC] * inv).astype(bf16))

    def conv_forward_x(j, slot):
        pr = pl.ds(pl.multiple_of(j * (C // 2), C // 2), C // 2)
        r = pl.ds(pl.multiple_of(j * C, C), C)
        w = sh_ref[...].astype(f32)
        kc = _un(kb[slot]).astype(f32)
        ext = jnp.concatenate([khalo[...], kc], axis=0)
        ks = kc * w[0:1]
        for lag in range(1, KS):
            ks = ks + ext[8 - lag: 8 + C - lag] * w[lag:lag + 1]
        khalo[...] = kc[C - 8:]
        kvc = (ks * _un(vb[slot]).astype(f32)).astype(bf16)
        kv_s[pr, :] = _pk(kvc)
        xs = jnp.dot(fw_ref[...], kvc, preferred_element_type=f32)
        xf[j, 0] = xs[:, :HALF]
        xf[j, 1] = xs[:, HALF:]
        xg = _un(x_s[pr, :]).astype(f32) * gw_ref[...].astype(f32).reshape(1, M)
        g_s[r, :] = jax.nn.sigmoid(jnp.sum(xg, axis=1, keepdims=True))

    def conv_forward_k(j, slot):
        kn = jax.lax.dot_general(fw_ref[...], _un(skb[slot]), NT, preferred_element_type=f32)
        q4 = C // 2
        kp = kprev[...]
        kw = jnp.concatenate([
            kn[0:q4] - kp[2 * q4:3 * q4],
            kn[q4:2 * q4] + kp[3 * q4:4 * q4],
            kn[2 * q4:3 * q4] + kp[0:q4],
            kn[3 * q4:4 * q4] - kp[q4:2 * q4],
        ], axis=0)
        kprev[...] = kn
        kf[j, 0] = kw[:, :HALF]
        kf[j, 1] = kw[:, HALF:]

    def conv_block_items(n, group):
        half = n % 2
        re = pl.ds(pl.multiple_of((n // 2) * 16, 16), 16)
        im = pl.ds(pl.multiple_of(C + (n // 2) * 16, 16), 16)
        pre = pl.ds(pl.multiple_of((n // 2) * 8, 8), 8)
        pim = pl.ds(pl.multiple_of(C // 2 + (n // 2) * 8, 8), 8)

        acc = {}

        def some(lb, i, a0, a1):
            ln = slice(lb * T, (lb + 1) * T)
            yr, yi = acc.pop((lb, i), (None, None))
            for a in range(a0, a1):
                xr, xi = xf[i - a, half, re, ln], xf[i - a, half, im, ln]
                kr, ki = kf[a, half, re, ln], kf[a, half, im, ln]
                pr = xr * kr - xi * ki
                pi = xr * ki + xi * kr
                yr = pr if yr is None else yr + pr
                yi = pi if yi is None else yi + pi
            if a1 == i + 1:
                yr, yi = _pk(yr.astype(bf16)), _pk(yi.astype(bf16))
                yf[i, half, pre, ln] = yr
                yf[i, half, pim, ln] = yi
                return _zero_of(yr | yi)
            acc[lb, i] = (yr, yi)
            ur, ui = pltpu.bitcast(yr, u32), pltpu.bitcast(yi, u32)
            return _zero_of((ur[:8] | ur[8:]) | (ui[:8] | ui[8:]))

        return [(min(a0 + group, i + 1) - a0,
                 (lambda lb=lb, i=i, a0=a0: some(lb, i, a0, min(a0 + group, i + 1))))
                for lb in range(HALF // T) for i in range(NCH) for a0 in range(0, i + 1, group)]

    def conv_inverse(j):
        dvec = sd_ref[...].astype(f32).reshape(1, M)
        pr = pl.ds(pl.multiple_of(j * (C // 2), C // 2), C // 2)
        y = jnp.concatenate(
            [jnp.dot(iv_ref[...], _un(yf[j, hh]), preferred_element_type=f32)
             for hh in range(2)], axis=1)
        y = y + _un(kv_s[pr, :]).astype(f32) * dvec
        return _un(x_s[pr, :]).astype(f32) * y

    def prologue():
        first = w_copies(0, 1)
        for cp in first[1:]:
            cp.start()
        for i in range(NQ):
            block_copy(0, i).start()
        first[0].start()
        for i in range(NX):
            block_copy(1, i).start()
        for cp in small_copies() + chunk_copies(0, 0):
            cp.start()
        kprev[...] = jnp.zeros(kprev.shape, f32)
        khalo[...] = jnp.zeros(khalo.shape, f32)
        for cp in first[1:]:
            cp.wait()
        unpack_weights(1, 0, (1, 2))

        def kv_body(i, carry):
            block_copy(0, i).wait()
            pr = pl.ds(pl.multiple_of(i * (BQ // 2), BQ // 2), BQ // 2)
            cc = _un(c_s[pr, :])
            k_s[pr, :] = _pk(jnp.dot(cc, _un(wk_s[...]), preferred_element_type=f32).astype(bf16))
            v_s[pr, :] = _pk(jnp.dot(cc, _un(wv_s[...]), preferred_element_type=f32).astype(bf16))
            return carry

        jax.lax.fori_loop(0, NQ, kv_body, 0)
        first[0].wait()
        unpack_weights(1, 0, (0,))
        for n, buf in enumerate((wqb, wkb, wvb)):
            pltpu.make_async_copy(buf.at[1], buf.at[0], w_sem.at[0, n]).start()

        def q_body(i, carry):
            block_copy(1, i).wait()
            pr = pl.ds(pl.multiple_of(i * (S // 2 // NX), S // 2 // NX), S // 2 // NX)
            q = jnp.dot(_un(x_s[pr, :]), _un(wq_s[...]), preferred_element_type=f32)
            q_s[pr, :] = _pk((q * QSCALE).astype(bf16))
            return carry

        jax.lax.fori_loop(0, NX, q_body, 0)
        for cp in small_copies():
            cp.wait()
        wo_copy().start()

    def next_weights(h):
        slot = h % 2
        for cp in w_copies((h + 1) // 2, slot):
            cp.wait()
        for cp in w_copies(jnp.minimum((h + 2) // 2, H // 2 - 1), 1 - slot):
            cp.start()
        unpack_weights(slot, (h + 1) % 2)

    HB = BQ // 2

    def head_step(fill, hk):
        def run(names):
            for name in names:
                if name in fill:
                    fill[name](hk)

        for i in range(NQ - 1, -1, -1):
            before, after = FILL_ORDER[i]
            for g in diag_first(i):
                scores(i, g, hk)
            run(before)
            row_max(i)
            context(i)
            run(after)
        hk.flush()

    def proj_fill():
        fill = {}
        for i in range(NQ):
            fill["K%d" % i] = lambda hk, i=i: k_proj(i * BQ, (i + 1) * BQ, hk)
            fill["V%d" % i] = lambda hk, i=i: v_proj(i * BQ, (i + 1) * BQ, hk)
            fill["Q%da" % i] = lambda hk, i=i: q_proj(i * BQ, i * BQ + HB, hk)
            fill["Q%db" % i] = lambda hk, i=i: q_proj(i * BQ + HB, (i + 1) * BQ, hk)
        return fill

    def forward_step(h, carry):
        cur["h"] = h
        slot = h % 2
        for cp in chunk_copies(h, slot):
            cp.wait()
        for cp in chunk_copies(jnp.minimum(h + 1, NCH - 1), 1 - slot):
            cp.start()
        next_weights(h)
        fill = proj_fill()
        fill["E0"] = lambda hk: conv_forward_x(h, slot)
        fill["E1"] = lambda hk: conv_forward_k(h, slot)
        head_step(fill, Hooks())
        return carry

    def product_step(h, carry):
        cur["h"] = h
        next_weights(h)
        head_step(proj_fill(), Hooks(conv_block_items(h - NCH, 1), rate=PRODUCT_RATE))
        return carry

    def last_step():
        cur["h"] = H - 1
        for cp in w_copies(H // 2 - 1, (H - 1) % 2) + chunk_copies(NCH - 1, NCH % 2):
            cp.wait()
        wo_copy().wait()
        head_step({}, Hooks(conv_block_items(NCH - 1, 4), rate=3.0))

    def out_copy(e, n):
        r = pl.ds(pl.multiple_of(e * RE, RE), RE)
        cols = slice(n * HALF, (n + 1) * HALF)
        return pltpu.make_async_copy(o_s.at[r, cols], o_hbm.at[0, r, cols], o_sem.at[e, n])

    def output_step(e, carry):
        pr = pl.ds(pl.multiple_of(e * (RE // 2), RE // 2), RE // 2)
        r = pl.ds(pl.multiple_of(e * RE, RE), RE)
        ctx = jnp.concatenate([_un(ctx_s[hh, pr, :]) for hh in range(H)], axis=1)
        b = jnp.concatenate([conv_inverse(e * (RE // C) + j) for j in range(RE // C)], axis=0)
        g = g_s[r, :]
        for n in range(2):
            cols = slice(n * HALF, (n + 1) * HALF)
            a = jnp.dot(ctx, _un(wo_s[:, cols]), preferred_element_type=f32)
            bn = b[:, cols]
            o_s[r, cols] = (bn + g * (a - bn)).astype(bf16)
            out_copy(e, n).start()
        return carry

    prologue()
    jax.lax.fori_loop(0, NCH, forward_step, 0)
    jax.lax.fori_loop(NCH, H - 1, product_step, 0)
    last_step()
    jax.lax.fori_loop(0, NE, output_step, 0)
    for e in range(NE):
        for n in range(2):
            out_copy(e, n).wait()


@jax.jit
def pallas_gated_mix__compressed_kv_cla__ssm_conv_h3__prompt_kernel(
    A_x: jax.Array,
    A_c_kv: jax.Array,
    A_w_q: jax.Array,
    A_w_uk: jax.Array,
    A_w_uv: jax.Array,
    A_w_o: jax.Array,
    B_q: jax.Array,
    B_k: jax.Array,
    B_v: jax.Array,
    B_shift_k: jax.Array,
    B_ssm_k: jax.Array,
    B_ssm_D: jax.Array,
    gate_w: jax.Array,
):
    fwd, inv = _dft_matrices()
    fwd = jnp.asarray(fwd, bf16)
    inv = jnp.asarray(inv, bf16)

    in_specs = [pl.BlockSpec(memory_space=pl.ANY)] * 14
    scratch = [
        pltpu.VMEM((S, M), bf16),
        pltpu.SemaphoreType.DMA((NE, 2)),
        pltpu.VMEM((S // 2, M), u32),
        pltpu.VMEM((S // 2, DC), u32),
        pltpu.VMEM((H * D // 2, M), u32),
        pltpu.VMEM((S // 2, D), u32), pltpu.VMEM((S // 2, D), u32), pltpu.VMEM((S // 2, D), u32),
        pltpu.VMEM((H, S // 2, D), u32),
        pltpu.VMEM((2, M, D), u32), pltpu.VMEM((2, DC, D), u32), pltpu.VMEM((2, DC, D), u32),
        pltpu.VMEM((M // 2, D), u32), pltpu.VMEM((DC // 2, D), u32), pltpu.VMEM((DC // 2, D), u32),
        pltpu.VMEM((2, C // 2, M), u32), pltpu.VMEM((2, C // 2, M), u32),
        pltpu.VMEM((2, M // 2, C), u32),
        pltpu.VMEM((NCH, 2, 2 * C, HALF), f32),
        pltpu.VMEM((NCH, 2, 2 * C, HALF), f32),
        pltpu.VMEM((NCH, 2, C, HALF), u32),
        pltpu.VMEM((2 * C, M), f32),
        pltpu.VMEM((8, M), f32),
        pltpu.VMEM((S // 2, M), u32),
        pltpu.VMEM((S, 1), f32),
        pltpu.VMEM((KS, M), bf16), pltpu.VMEM((M,), bf16), pltpu.VMEM((M,), bf16),
        pltpu.VMEM((2 * C, C), bf16), pltpu.VMEM((C, 2 * C), bf16),
        pltpu.SemaphoreType.DMA((5,)),
        pltpu.SemaphoreType.DMA((2, NX)),
        pltpu.SemaphoreType.DMA((1,)),
        pltpu.SemaphoreType.DMA((2, 3)),
        pltpu.SemaphoreType.DMA((2, 3)),
    ]
    return pl.pallas_call(
        _kernel,
        in_specs=in_specs,
        out_specs=pl.BlockSpec(memory_space=pl.ANY),
        out_shape=jax.ShapeDtypeStruct((1, S, M), bf16),
        scratch_shapes=scratch,
        compiler_params=pltpu.CompilerParams(
            vmem_limit_bytes=126 * 1024 * 1024,
        ),
        name="gated_mix_kernel",
    )(A_x, A_c_kv, A_w_q, A_w_uk, A_w_uv, A_w_o.reshape(H * D, M), B_k, B_v, B_ssm_k,
      B_shift_k.T, B_ssm_D, gate_w, fwd, inv)
```
